```python
import jax
import jax.numpy as jnp

def _softmax(x, axis=-1):
    return jax.nn.softmax(x, axis=axis)

def _gelu(x):
    return jax.nn.gelu(x, approximate=True)

def _silu(x):
    return jax.nn.silu(x)

def _sigmoid(x):
    return jax.nn.sigmoid(x)

def _layernorm(x, axis=-1, eps=1e-05):
    m = jnp.mean(x, axis=axis, keepdims=True)
    v = jnp.var(x, axis=axis, keepdims=True)
    return (x - m) / jnp.sqrt(v + eps)

def _scatter_add(tgt, idx, src, axis=0):
    return tgt.at[idx].add(src)

def _segment_sum(src, seg, n):
    return jax.ops.segment_sum(src, seg, n)

class _Rng:

    def __init__(self, key):
        self._k = key

    def _next(self):
        self._k, sub = jax.random.split(self._k)
        return sub

    def normal(self, shape):
        return jax.random.normal(self._next(), shape, dtype=jnp.bfloat16)

    def randint(self, lo, hi, shape):
        return jax.random.randint(self._next(), shape, lo, hi, dtype=jnp.int32)

    def uniform(self, shape, lo=0.0, hi=1.0):
        return jax.random.uniform(self._next(), shape, jnp.bfloat16, lo, hi)

    def permutation(self, n):
        return jax.random.permutation(self._next(), n)
kernel_name = 'interleave_layers__memory_aug_recurrent_mem_tr__glu_gated_swiglu__prompt'

def setup_inputs():
    _rng = _Rng(jax.random.key(int.from_bytes(__import__("os").urandom(4), "little")))
    _w = lambda a: (lambda t: t.astype(jnp.bfloat16) if jnp.issubdtype(t.dtype, jnp.floating) else t)(jnp.asarray(a))

    def _A_setup():
        B, S, Dm = (1, 2048, 576)
        H, Dh = (32, 128)
        M, seg = (8, 32)
        seg = min(seg, S)
        S = S // seg * seg
        return {'x': _w((lambda *s: _rng.normal(s) * 0.05)(B, S, Dm)), 'mem0': _w((lambda *s: _rng.normal(s) * 0.05)(B, M, Dm)), 'Wq': _w((lambda *s: _rng.normal(s) * 0.05)(Dm, H, Dh) * Dm ** (-0.5)), 'Wk': _w((lambda *s: _rng.normal(s) * 0.05)(Dm, H, Dh) * Dm ** (-0.5)), 'Wv': _w((lambda *s: _rng.normal(s) * 0.05)(Dm, H, Dh) * Dm ** (-0.5)), 'Wo': _w((lambda *s: _rng.normal(s) * 0.05)(H, Dh, Dm) * (H * Dh) ** (-0.5)), 'seg_len': seg}
    _A_in = _A_setup()

    def _B_setup():
        B, S, D, F = (1, 2048, 576, 4608)
        return {'x': _w((lambda *s: _rng.normal(s) * 0.05)(B, S, D)), 'w1': _w((lambda *s: _rng.normal(s) * 0.05)(D, F) * (2.0 / D) ** 0.5), 'w3': _w((lambda *s: _rng.normal(s) * 0.05)(D, F) * (2.0 / D) ** 0.5), 'w2': _w((lambda *s: _rng.normal(s) * 0.05)(F, D) * (2.0 / F) ** 0.5)}
    _B_in = _B_setup()
    return {'A_x': _A_in['x'], 'A_mem0': _A_in['mem0'], 'A_Wq': _A_in['Wq'], 'A_Wk': _A_in['Wk'], 'A_Wv': _A_in['Wv'], 'A_Wo': _A_in['Wo'], 'A_seg_len': _A_in['seg_len'], 'B_x': _B_in['x'], 'B_w1': _B_in['w1'], 'B_w3': _B_in['w3'], 'B_w2': _B_in['w2']}

def reference(A_x, A_mem0, A_Wq, A_Wk, A_Wv, A_Wo, A_seg_len, B_x, B_w1, B_w3, B_w2):

    def _A_ref(x, mem0, Wq, Wk, Wv, Wo, seg_len):
        B, S, Dm = x.shape
        H, Dh = (Wq.shape[1], Wq.shape[2])
        M = mem0.shape[1]
        scale = Dh ** (-0.5)
        n_seg = S // seg_len
        L = M + seg_len
        idx = jnp.arange(L)
        mask = (idx[:, None] < M) | (idx[:, None] >= idx[None, :])
        mem = mem0
        outs = []
        for s in range(n_seg):
            xs = x[:, s * seg_len:(s + 1) * seg_len, :].copy()
            h = jnp.concatenate([mem, xs], axis=1)
            q = jnp.einsum('btd,dhe->bhte', h, Wq)
            k = jnp.einsum('btd,dhe->bhte', h, Wk)
            v = jnp.einsum('btd,dhe->bhte', h, Wv)
            scores = jnp.einsum('bhqe,bhke->bhqk', q, k) * scale
            scores = jnp.where(mask[None, None], scores, -1000000000.0)
            p = _softmax(scores, axis=-1)
            o = jnp.einsum('bhqk,bhke->bhqe', p, v)
            o = jnp.einsum('bhte,hed->btd', o, Wo)
            mem = o[:, :M, :].copy()
            outs.append(o[:, M:, :])
        return jnp.concatenate(outs, axis=1)

    def _B_ref(x, w1, w3, w2):
        gate = jnp.einsum('bsd,df->bsf', x, w1)
        up = jnp.einsum('bsd,df->bsf', x, w3)
        h = _silu(gate) * up
        out = jnp.einsum('bsf,fd->bsd', h, w2)
        return out
    x = A_x
    x = x + _A_ref(_layernorm(x, axis=-1), A_mem0, A_Wq, A_Wk, A_Wv, A_Wo, A_seg_len)
    x = x + _B_ref(_layernorm(x, axis=-1), B_w1, B_w3, B_w2)
    x = x + _A_ref(_layernorm(x, axis=-1), A_mem0, A_Wq, A_Wk, A_Wv, A_Wo, A_seg_len)
    x = x + _B_ref(_layernorm(x, axis=-1), B_w1, B_w3, B_w2)
    return x
```

```python
import functools
import math

import jax
import jax.numpy as jnp
import jax.experimental.pallas as pl
import jax.experimental.pallas.tpu as pltpu

_EPS = 1e-05
_MASKED = -1000000000.0
_LOG2E = math.log2(math.e)
_LANES = 128
_HALF = _LANES // 2
_SLAB = 16
_UNIT = 6
_SLOTS = 3
_PLAIN_HEADS = 2
_MODEL, _WIDE = 0, 2
_PRODUCTS = (
    (((1, 1, 0),), ((1, 0, 0), (1, 0, 1), (-1, 2, 0)), ((1, 1, 0),)),
    (((1, 2, 0),), ((1, 0, 0), (1, 0, 2), (-1, 1, 0)), ((1, 2, 0),)),
    (((1, 2, 0), (1, 2, 1)), ((1, 1, 0),), ((1, 3, 0), (-1, 3, 1))),
    (((1, 1, 0), (1, 1, 2)), ((1, 2, 0),), ((1, 3, 0), (-1, 3, 2))),
    (((1, 3, 0), (1, 3, 1)), ((1, 0, 1),), ((-1, 1, 0), (1, 1, 1))),
    (((-1, 2, 0), (1, 3, 1)), ((1, 0, 1), (1, 1, 0)), ((1, 1, 0), (-1, 3, 1))),
    (((1, 3, 0), (1, 3, 2)), ((1, 0, 2),), ((1, 2, 0), (-1, 2, 2))),
    (((1, 1, 0), (1, 3, 2)), ((1, 0, 2), (1, 2, 0)), ((-1, 2, 0), (1, 3, 2))),
    (((1, 1, 1),), ((1, 1, 0), (1, 1, 1), (-1, 2, 1)), ((1, 3, 1),)),
    (((1, 2, 2),), ((1, 2, 0), (1, 2, 2), (-1, 1, 2)), ((1, 3, 2),)),
    (((1, 1, 1), (1, 1, 2)), ((1, 2, 1),), ((1, 1, 1), (-1, 1, 2))),
    (((1, 2, 1), (1, 2, 2)), ((1, 1, 2),), ((-1, 2, 1), (1, 2, 2))),
    (((1, 1, 1), (1, 2, 2)), ((1, 1, 2), (1, 2, 1)), ((1, 2, 1), (1, 1, 2))),
    (((1, 3, 1),), ((1, 0, 1), (-1, 1, 1), (-1, 1, 2)), ((1, 2, 1),)),
    (((1, 3, 2),), ((1, 2, 1), (1, 2, 2), (-1, 0, 2)), ((1, 1, 2),)),
)
_N_PRODUCTS = len(_PRODUCTS)
_CLOSE = "A D13 D14 D15 D16 D17 E"
_OPEN = (
    "G0 G1 P0 P1 S0 P2 S1 V0 G2 P3 S2 V1 L D0 P4 S3 V2 D1 G3 P5 S4 V3 O0 D2 P6 S5 V4 O1 G4 D3 "
    "P7 S6 V5 O2 G5 D4 P8 S7 V6 O3 D5 P9 S8 V7 O4 G6 D6 P10 S9 V8 O5 G7 D7 P11 S10 V9 O6 D8 "
    "P12 S11 V10 O7 G8 D9 P13 S12 V11 O8 G9 D10 P14 S13 V12 O9 D11 P15 S14 V13 O10 G10 S15 "
    "V14 O11 G11 V15 D12 O12 O13 O14")
_ATTENTION = (
    "P0 P1 S0 P2 S1 P3 S2 V0 P4 S3 V1 P5 S4 V2 L P6 S5 V3 P7 S6 V4 O0 P8 S7 V5 O1 P9 S8 V6 O2 "
    "P10 S9 V7 O3 P11 S10 V8 O4 P12 S11 V9 O5 P13 S12 V10 O6 P14 S13 V11 O7 P15 S14 V12 O8 S15 "
    "O9 V13 O10 V14 O11 V15 O12 O13 O14")
_SWIGLU = (
    "G0 G1 G2 D0 D1 G3 D2 G4 D3 D4 G5 D5 G6 D6 D7 G7 D8 G8 D9 G9 D10 G10 D11 G11 D12 D13 D14 "
    "D15 D16 D17")


def _layernorm(x):
    m = jnp.mean(x, axis=-1, keepdims=True)
    d = x - m
    v = jnp.mean(d * d, axis=-1, keepdims=True)
    return d * jax.lax.rsqrt(v + _EPS)


def _silu(x):
    return x * pltpu.reciprocal(1.0 + jnp.exp2(x * -_LOG2E), approx=True)


def _dot(a, b):
    return jnp.dot(a, b, preferred_element_type=jnp.float32)


def _dot_nt(a, b):
    return jax.lax.dot_general(a, b, (((1,), (1,)), ((), ())),
                               preferred_element_type=jnp.float32)


def _load_packed(ref, *index):
    return pltpu.bitcast(ref.bitcast(jnp.uint32)[index], jnp.bfloat16)


def _accumulate(total, sign, value):
    if total is None:
        return sign, value
    if total[0] == sign:
        return sign, total[1] + value
    return 1, (total[1] - value if sign < 0 else value - total[1])


def _value(total):
    return total[1] if total[0] > 0 else -total[1]


def _signed_sum(terms):
    return _value(functools.reduce(lambda total, term: _accumulate(total, *term), terms, None))


def _products(groups):
    if groups == 2:
        return list(enumerate(_PRODUCTS))

    def upper(terms):
        return tuple((sign, 1, i) for sign, f, i in terms if f != 2)

    kept = [(r, (upper(model), weight, upper(wide)))
            for r, (model, weight, wide) in enumerate(_PRODUCTS)]
    return [(r, product) for r, product in kept if product[_MODEL] and product[_WIDE]]


def _operands(blocks, side):
    forms = dict(enumerate(blocks, 1))
    if len(blocks) == 2:
        forms[3] = [a - b if side == _MODEL else a + b for a, b in zip(*blocks)]
    return {r: _signed_sum((sign, forms[f][i]) for sign, f, i in product[side])
            for r, product in _products(len(blocks))}


def _collect(multiply, side, groups, start=None):
    total = {}
    for f, tiles in enumerate(start or (), 1):
        for i, tile in enumerate(tiles):
            total[f, i] = (1, tile)
    products = _products(groups)
    shared = [i for _, product in products for _, f, i in product[side] if f == 3]
    for r, product in products:
        result = multiply(r)
        for sign, f, i in product[side]:
            total[f, i] = _accumulate(total.get((f, i)), sign, result)
            if f == 3:
                shared.remove(i)
                if i not in shared:
                    sign, value = total.pop((3, i))
                    total[1, i] = _accumulate(total.get((1, i)), sign, value)
                    total[2, i] = _accumulate(total.get((2, i)),
                                              -sign if side == _MODEL else sign, value)
    return [[_value(total[f, i]) for i in range(3)] for f in range(1, groups + 1)]


def _split(x):
    t0, t1, t2, t3 = (x[:, i * _LANES:(i + 1) * _LANES] for i in range(4))
    rest = x[:, 4 * _LANES:]
    return ([t0, t1, t3], [t0, t2, jnp.concatenate([t3[:, :_HALF], rest], axis=1)],
            [t1, t2, jnp.concatenate([rest, t3[:, _HALF:]], axis=1)])


def _merge(a, b, c):
    low = jax.lax.broadcasted_iota(jnp.int32, a[0].shape, 1) < _HALF
    return jnp.concatenate(
        [a[0] + b[0], a[1] + c[0], b[1] + c[1], a[2] + jnp.where(low, b[2], c[2]),
         b[2][:, _HALF:] + c[2][:, :_HALF]], axis=1)


def _weight_blocks(part, row, w1, w2):
    t0, t1, t2, t3 = (i * _LANES + row for i in range(4))
    rest = 4 * _LANES + row % _HALF
    if part == 0:
        return [w1(t0), w1(t1) - w2(t1), w1(t3) if row < _HALF else w1(t3) - w2(t3)]
    if part == 1:
        return [w2(t0), w2(t2) - w1(t2), w2(t3) if row < _HALF else w2(rest) - w1(rest)]
    return [w2(t1), w1(t2), w1(rest) if row < _HALF else w2(t3)]


def _combine_weights(out_ref, part, row, load):
    blocks = [_weight_blocks(part, row, functools.partial(load, 0, j),
                             functools.partial(load, 1, j)) for j in range(3)]
    for r, (_, terms, _) in enumerate(_PRODUCTS):
        value = _signed_sum((sign, blocks[j][i]) for sign, i, j in terms)
        out_ref[part * _N_PRODUCTS + r, row:row + _SLAB, :] = value.astype(out_ref.dtype)


def _expand(operand, weight, groups):
    def multiply(part):
        first = part * _N_PRODUCTS
        return lambda r: _dot(operand(first + r), weight(first + r))

    shared = _collect(multiply(2), _WIDE, groups)
    return [_collect(multiply(part), _WIDE, groups, shared) for part in range(2)]


def _contract(part, tile, weight, groups, start, dtype):
    if part < 2:
        blocks = [[tile(f, 3 * part + j) for j in range(3)] for f in range(groups)]
    else:
        blocks = [[tile(f, j) + tile(f, 3 + j) for j in range(3)] for f in range(groups)]
    operands = _operands(blocks, _WIDE)
    return _collect(
        lambda r: _dot(operands[r].astype(dtype), weight(part * _N_PRODUCTS + r)),
        _MODEL, groups, start)


def _store_operands(ref, rows):
    for part, blocks in enumerate(zip(*map(_split, rows))):
        for r, value in _operands(blocks, _MODEL).items():
            ref[part * _N_PRODUCTS + r] = value.astype(ref.dtype)


def _attention_masks(n_mem, seg):
    size = n_mem + seg
    shape = (2 * size, 2 * size)

    def position(axis):
        r = jax.lax.broadcasted_iota(jnp.int32, shape, axis)
        return r < size, jnp.where(r < seg, r + n_mem, jnp.where(r < size, r - seg, r - size))

    (first_i, i), (first_j, j) = position(0), position(1)
    same = first_i == first_j
    fill = jnp.where(same, _MASKED * _LOG2E, -jnp.inf).astype(jnp.float32)
    return same & ((i < n_mem) | (i >= j)), fill


def _kernel(xt_hbm, mem0_hbm, wq_hbm, wk_hbm, wv_hbm, wot_hbm, w1_hbm, w3_hbm, w2t_hbm,
            outt_hbm, mem0_ref, tile_ref, x_ref, res_ref, early_in_ref, early_ref,
            pair_in_ref, solo_in_ref, ffn_in_ref, attn_sum_ref, ffn_sum_ref, hidden_ref,
            qkv_stage, up_stage, down_stage, plain_stage, turn_ref,
            wqkv_ref, wup_ref, wdown_ref, wplain_ref, stage_sem, misc_sem, tile_sem, *, seg):
    n_tok = xt_hbm.shape[1]
    n_mem = mem0_ref.shape[0]
    _, n_heads, d_head = wq_hbm.shape
    n_pairs = n_heads // 2
    n_attn_units = n_heads // _UNIT
    n_up, n_down = wup_ref.shape[0], wdown_ref.shape[0]
    n_ffn_units = n_down - n_attn_units
    n_seg = n_tok // seg
    n_io = n_tok // _LANES
    size = n_mem + seg
    ahead = seg // 2
    score_scale = d_head ** -0.5 * _LOG2E
    carried = hidden_ref.shape[0]

    def segment(s):
        return pl.ds(pl.multiple_of(s * seg, seg), seg)

    def transpose_out(i):
        rows = pl.ds(pl.multiple_of(i * _LANES, _LANES), _LANES)
        tile_ref[i] = x_ref[rows, :].astype(tile_ref.dtype).T

    def run(order, sums, hidden, t=None):
        groups = 1 if t is None else 2
        visible, fill = _attention_masks(n_mem, seg)
        qkv, probs, heads, gate = {}, {}, {}, None
        for name in order:
            stage, g = name[0], int(name[1:] or 0)
            if stage == "P" and groups == 2:
                both = _expand(functools.partial(_load_packed, pair_in_ref),
                               functools.partial(_load_packed, wqkv_ref, g), 2)
                qkv[g] = [[
                    jnp.concatenate(
                        [_load_packed(early_ref, g, t, 3 * n + w).astype(jnp.float32),
                         upper[w][n_mem:n_mem + ahead], upper[w][:n_mem], lower[w][:n_mem],
                         upper[w][n_mem + ahead:], lower[w][n_mem:]],
                        axis=0).astype(jnp.bfloat16)
                    for w in range(3)] for n, (upper, lower) in enumerate(both)]
            elif stage == "P":
                (first,), (second,) = _expand(lambda r: solo_in_ref[r],
                                              functools.partial(_load_packed, wqkv_ref, g), 1)
                qkv[g] = [[
                    jnp.concatenate([a[n_mem:], a[:n_mem], b], axis=0).astype(jnp.bfloat16)
                    for a, b in zip(first, second)]]
            elif stage == "S":
                probs[g] = []
                for q, k, _ in qkv[g]:
                    s = jnp.where(visible, _dot_nt(q, k) * score_scale, fill)
                    p = jnp.exp2(s - jnp.max(s, axis=-1, keepdims=True))
                    inv = pltpu.reciprocal(jnp.sum(p, axis=-1, keepdims=True), approx=True)
                    probs[g].append((p.astype(jnp.bfloat16), inv))
            elif stage == "V":
                for n, ((p, inv), (_, _, v)) in enumerate(zip(probs[g], qkv[g])):
                    o = _dot(p, v) * inv
                    halves = [jnp.concatenate([o[seg:size], o[:seg]], axis=0), o[size:]]
                    if groups == 2:
                        heads[2 * g + n] = halves
                    else:
                        heads[2 * g], heads[2 * g + 1] = halves[:1], halves[1:]
            elif stage == "L":
                a, b = (jnp.concatenate(heads[h], axis=0) for h in range(_PLAIN_HEADS))
                dtype = jnp.bfloat16 if groups == 2 else jnp.float32
                for part, rows in enumerate((a, b, a + b)):
                    tiles = [_dot(rows.astype(dtype), _load_packed(wplain_ref, 3 * part + i))
                             for i in range(3)]
                    sums["O", part] = [[tile[f * size:(f + 1) * size] for tile in tiles]
                                       for f in range(groups)]
            elif stage == "O":
                unit, part = divmod(g, 3)
                sums["O", part] = _contract(
                    part, lambda f, j: heads[_PLAIN_HEADS + _UNIT * unit + j][f],
                    functools.partial(_load_packed, wdown_ref, unit), groups,
                    sums["O", part], jnp.float32)
            elif stage == "G":
                first, second = _expand(functools.partial(_load_packed, ffn_in_ref),
                                        functools.partial(_load_packed, wup_ref, g), 2)
                tiles = [a + b for a, b in zip(first, second)]
                if g % 2:
                    hidden[g // 2] = [[_silu(a) * b for a, b in zip(*rows)]
                                      for rows in zip(gate, tiles)]
                gate = tiles
            elif stage == "D":
                unit, part = divmod(g, 3)
                sums["D", part] = _contract(
                    part, lambda f, j: hidden[unit][f][j],
                    functools.partial(_load_packed, wdown_ref, n_attn_units + unit), 2,
                    sums.get(("D", part)), jnp.bfloat16)

    def merged(sums, kind):
        return [_merge(*parts) for parts in zip(*(sums[kind, part] for part in range(3)))]

    def save(ref, nested):
        for a, rows in enumerate(nested):
            for b, tiles in enumerate(rows):
                for c, tile in enumerate(tiles):
                    ref[a, b, c] = tile

    def restore(ref, groups=2):
        return [[[ref[a, b, c] for c in range(ref.shape[2])] for b in range(groups)]
                for a in range(ref.shape[0])]

    def open_step(order, t=None):
        sums, hidden = {}, {}
        run(order.split(), sums, hidden, t)
        save(attn_sum_ref, [sums["O", part] for part in range(3)])
        if hidden:
            save(ffn_sum_ref, [sums["D", part] for part in range(3)])
            save(hidden_ref, [hidden[n_ffn_units - carried + u] for u in range(carried)])

    def close_step(groups, attention_done):
        sums = {("O", part): rows for part, rows in enumerate(restore(attn_sum_ref, groups))}
        sums.update({("D", part): rows for part, rows in enumerate(restore(ffn_sum_ref))})
        hidden = dict(enumerate(restore(hidden_ref), n_ffn_units - carried))
        for name in _CLOSE.split():
            if name == "A":
                attention_done(merged(sums, "O"))
            elif name != "E":
                run([name], sums, hidden)
        return merged(sums, "D")

    def solo_attention(mem, x):
        _store_operands(solo_in_ref, [jnp.concatenate([mem, _layernorm(x)], axis=0)])
        sums = {}
        run(_ATTENTION.split(), sums, None)
        out, = merged(sums, "O")
        return out[:n_mem], x + out[n_mem:]

    def solo_swiglu(rows):
        _store_operands(ffn_in_ref, [_layernorm(x) for x in rows])
        sums = {}
        run(_SWIGLU.split(), sums, {})
        return [x + y for x, y in zip(rows, merged(sums, "D"))]

    def store_pair_operands(t, mems, x2):
        late = x_ref[pl.ds(pl.multiple_of(t * seg + ahead, ahead), seg - ahead), :]
        h2 = _layernorm(x2)
        cut = ahead // 2
        _store_operands(pair_in_ref, [
            jnp.concatenate([mems[0], _layernorm(late), h2[:cut]], axis=0),
            jnp.concatenate([mems[1], h2[cut:]], axis=0)])

    def close_pair_step(t):
        state = {}

        def attention_done(outs):
            state["mems"] = [out[:n_mem] for out in outs]
            state["rows"] = [x_ref[segment(t), :] + outs[0][n_mem:], res_ref[0] + outs[1][n_mem:]]
            _store_operands(ffn_in_ref, [_layernorm(x) for x in state["rows"]])

        updates = close_step(2, attention_done)
        x2 = res_ref[1] + updates[0]
        x_ref[segment(jnp.maximum(t - 3, 0)), :] = res_ref[2] + updates[1]
        res_ref[0] = x2
        res_ref[1], res_ref[2] = state["rows"]
        return state["mems"], x2

    def qkv_copies(g):
        slot = g % _SLOTS
        return [pltpu.make_async_copy(w.bitcast(jnp.uint32).at[:, g, :], qkv_stage.at[slot, i],
                                      stage_sem.at[slot])
                for i, w in enumerate((wq_hbm, wk_hbm, wv_hbm))]

    def unit_columns(u):
        return pl.ds(pl.multiple_of(u * (_UNIT * _LANES), _LANES), _UNIT * _LANES)

    def up_copy(w_hbm, u):
        slot = u % _SLOTS
        return pltpu.make_async_copy(w_hbm.bitcast(jnp.uint32).at[:, unit_columns(u // 2)],
                                     up_stage.at[slot], stage_sem.at[_SLOTS + slot])

    def head_copies(u):
        slot = u % _SLOTS
        return [pltpu.make_async_copy(
            wot_hbm.bitcast(jnp.uint32).at[_PLAIN_HEADS + _UNIT * u + j],
            down_stage.at[slot, :, pl.ds(j * _LANES, _LANES)], stage_sem.at[2 * _SLOTS + slot])
                for j in range(_UNIT)]

    def down_copy(u):
        slot = u % _SLOTS
        return pltpu.make_async_copy(
            w2t_hbm.bitcast(jnp.uint32).at[:, unit_columns(u - n_attn_units)],
            down_stage.at[slot], stage_sem.at[2 * _SLOTS + slot])

    def each(copies, method):
        for copy in copies:
            copy.start() if method == "start" else copy.wait()

    def when(condition, function):
        if isinstance(condition, bool):
            if condition:
                function()
        else:
            pl.when(condition)(function)

    def unit_copies(u, method):
        when((u < n_up) & (u % 2 == 0), lambda: each([up_copy(w1_hbm, u)], method))
        when((u < n_up) & (u % 2 == 1), lambda: each([up_copy(w3_hbm, u)], method))
        when(u < n_attn_units, lambda: each(head_copies(u), method))
        when((u >= n_attn_units) & (u < n_down), lambda: each([down_copy(u)], method))

    def x_copy(i):
        cols = pl.ds(i * _LANES, _LANES)
        return pltpu.make_async_copy(xt_hbm.at[:, cols], tile_ref.at[i], tile_sem.at[i])

    misc_copies = [
        pltpu.make_async_copy(wot_hbm.bitcast(jnp.uint32).at[pl.ds(0, _PLAIN_HEADS)],
                              plain_stage, misc_sem.at[0]),
        pltpu.make_async_copy(mem0_hbm, mem0_ref, misc_sem.at[1])]
    out_copies = [
        pltpu.make_async_copy(tile_ref.at[i], outt_hbm.at[:, pl.ds(i * _LANES, _LANES)],
                              tile_sem.at[i]) for i in range(n_io)]

    def unpack_rows(words):
        return pltpu.bitcast(words, jnp.bfloat16).astype(jnp.float32)

    def qkv_jobs(g):
        def load(n, j, r):
            words = qkv_stage[g % _SLOTS, j, r:r + _SLAB, :]
            words = words & jnp.uint32(0xFFFF0000) if n else words << 16
            return pltpu.bitcast(words, jnp.float32)

        return [functools.partial(_combine_weights, wqkv_ref.at[g], part, row, load)
                for part in (2, 0, 1) for row in range(0, _LANES, _SLAB)]

    def unit_jobs(u):
        def load(stage, unit, n, j, r):
            cols = pl.ds((3 * n + j) * _LANES, _LANES)
            return unpack_rows(stage[unit % _SLOTS, r // 2:(r + _SLAB) // 2, cols])

        down = jnp.minimum(u, n_down - 1)

        def turn(r):
            wdown_ref[down, r] = _load_packed(turn_ref, r).T

        jobs = []
        for part in range(3):
            for out, stage, unit in ((turn_ref, down_stage, down), (wup_ref.at[u], up_stage, u)):
                jobs += [functools.partial(_combine_weights, out, part, row,
                                           functools.partial(load, stage, unit))
                         for row in range(0, _LANES, _SLAB)]
            jobs += [functools.partial(turn, part * _N_PRODUCTS + r) for r in range(_N_PRODUCTS)]
        return jobs

    def prepare_tile(i):
        x = tile_ref[i].T.astype(jnp.float32)
        x_ref[i * _LANES:(i + 1) * _LANES, :] = x
        rows = [_layernorm(jnp.concatenate([x[s * seg:s * seg + ahead] for s in (f, f + 1)],
                                           axis=0)) for f in ((0, 2) if i else (2,))]
        _store_operands(early_in_ref.at[i], rows)

    def project_tile(g, i):
        first = 4 * i if i else 2
        both = _expand(functools.partial(_load_packed, early_in_ref, i),
                       functools.partial(_load_packed, wqkv_ref, g), 2 if i else 1)
        for n, rows in enumerate(both):
            for f, tiles in enumerate(rows):
                for w, tile in enumerate(tiles):
                    for s in range(2):
                        early_ref[g, first + 2 * f + s, 3 * n + w] = (
                            tile[s * ahead:(s + 1) * ahead].astype(early_ref.dtype))

    def project_pair(g, jobs):
        for i in range(n_io):
            project_tile(g, i)
            for job in jobs[len(jobs) * i // n_io:len(jobs) * (i + 1) // n_io]:
                job()

    first_unit = n_pairs - n_up

    def load_step(g, with_units):
        following = jnp.minimum(g + 1, n_pairs - 1)
        when(g + _SLOTS < n_pairs, lambda: each(qkv_copies(g + _SLOTS), "start"))
        u = g - first_unit
        when(u + _SLOTS - 1 >= 0, lambda: unit_copies(u + _SLOTS - 1, "start"))
        when(g + 1 < n_pairs, lambda: each(qkv_copies(following), "wait"))
        jobs = qkv_jobs(following)
        if with_units:
            unit_copies(u, "wait")
            jobs += unit_jobs(u)
        project_pair(g, jobs)

    each(qkv_copies(0), "start")
    each([x_copy(i) for i in range(n_io)], "start")
    each(qkv_copies(0), "wait")
    for g in range(1, _SLOTS):
        each(qkv_copies(g), "start")
    each(misc_copies, "start")
    for job in qkv_jobs(0):
        job()
    for i in range(n_io):
        x_copy(i).wait()
        prepare_tile(i)
    pl.loop(0, first_unit)(functools.partial(load_step, with_units=False))
    pl.loop(first_unit, n_pairs)(functools.partial(load_step, with_units=True))
    each(misc_copies, "wait")
    for part in range(3):
        tiles = [
            _weight_blocks(part, row, *(
                lambda r, h=h: unpack_rows(plain_stage[h, r // 2:(r + _SLAB) // 2, :])
                for h in range(_PLAIN_HEADS)))
            for row in range(0, _LANES, _SLAB)]
        for i, slabs in enumerate(zip(*tiles)):
            wplain_ref[3 * part + i] = jnp.concatenate(slabs, axis=0).astype(jnp.bfloat16).T

    def first_steps(s, mem):
        mem, res_ref[1 + s] = solo_attention(mem, x_ref[segment(s), :])
        return mem

    mem0 = mem0_ref[...].astype(jnp.float32)
    mem1 = jax.lax.fori_loop(0, 2, first_steps, mem0)
    x2, res_ref[1] = solo_swiglu([res_ref[1], res_ref[2]])
    res_ref[0] = x2
    store_pair_operands(2, [mem1, mem0], x2)
    open_step(_ATTENTION, 2)
    ffn_sum_ref[...] = jnp.zeros_like(ffn_sum_ref)
    hidden_ref[...] = jnp.zeros_like(hidden_ref)

    @pl.loop(3, n_seg)
    def _step(t):
        transpose_out(jnp.maximum(t - 8, 0) * seg // _LANES)
        store_pair_operands(t, *close_pair_step(t - 1))
        open_step(_OPEN, t)

    each(out_copies[:n_io - 2], "start")
    mems, x2 = close_pair_step(n_seg - 1)
    transpose_out(n_io - 2)
    _store_operands(solo_in_ref, [jnp.concatenate([mems[1], _layernorm(x2)], axis=0)])
    open_step(_OPEN)
    out_copies[n_io - 2].start()
    outs = []
    updates = close_step(1, outs.extend)
    x_ref[segment(n_seg - 3), :] = res_ref[2] + updates[1]
    _, last = solo_attention(outs[0][:n_mem], res_ref[1] + updates[0])
    rows = solo_swiglu([res_ref[0] + outs[0][n_mem:], last])
    for s, x in enumerate(rows):
        x_ref[segment(n_seg - 2 + s), :] = x
    transpose_out(n_io - 1)
    out_copies[n_io - 1].start()
    each(out_copies, "wait")


@functools.partial(jax.jit, static_argnames=("A_seg_len",))
def pallas_interleave_layers__memory_aug_recurrent_mem_tr__glu_gated_swiglu__prompt_kernel(
    A_x: jax.Array,
    A_mem0: jax.Array,
    A_Wq: jax.Array,
    A_Wk: jax.Array,
    A_Wv: jax.Array,
    A_Wo: jax.Array,
    A_seg_len: int,
    B_x: jax.Array,
    B_w1: jax.Array,
    B_w3: jax.Array,
    B_w2: jax.Array,
):
    del B_x
    _, n_tok, d_model = A_x.shape
    n_mem = A_mem0.shape[1]
    _, n_heads, d_head = A_Wq.shape
    seg = A_seg_len
    assert A_x.shape[0] == 1 and 4 * seg == d_head == _LANES and 4 * n_mem == seg
    assert n_heads == 32 and B_w1.shape[1] == 36 * _LANES and 2 * d_model == 9 * _LANES
    n_ffn_units = B_w1.shape[1] // (_UNIT * _LANES)
    n_tiles = 3 * _N_PRODUCTS
    f32, bf16, words = jnp.float32, jnp.bfloat16, jnp.uint32
    hbm = pl.BlockSpec(memory_space=pltpu.HBM)
    out_t = pl.pallas_call(
        functools.partial(_kernel, seg=seg),
        out_shape=jax.ShapeDtypeStruct((d_model, n_tok), A_x.dtype),
        in_specs=[hbm] * 9,
        out_specs=hbm,
        scratch_shapes=[
            pltpu.VMEM((n_mem, d_model), A_mem0.dtype),
            pltpu.VMEM((n_tok // _LANES, d_model, _LANES), A_x.dtype),
            pltpu.VMEM((n_tok, d_model), f32),
            pltpu.VMEM((3, seg, d_model), f32),
            pltpu.VMEM((n_tok // _LANES, n_tiles, seg, _LANES), bf16),
            pltpu.VMEM((n_heads // 2, n_tok // seg, _UNIT, seg // 2, _LANES), bf16),
            pltpu.VMEM((n_tiles, seg, _LANES), bf16),
            pltpu.VMEM((n_tiles, n_mem + seg, _LANES), f32),
            pltpu.VMEM((n_tiles, seg, _LANES), bf16),
            pltpu.VMEM((3, 2, 3, n_mem + seg, _LANES), f32),
            pltpu.VMEM((3, 2, 3, seg, _LANES), f32),
            pltpu.VMEM((2, 2, _UNIT, seg, _LANES), f32),
            pltpu.VMEM((_SLOTS, 3, d_model, d_head), words),
            pltpu.VMEM((_SLOTS, d_model // 2, _UNIT * _LANES), words),
            pltpu.VMEM((_SLOTS, d_model // 2, _UNIT * _LANES), words),
            pltpu.VMEM((_PLAIN_HEADS, d_model // 2, d_head), words),
            pltpu.VMEM((n_tiles, _LANES, _LANES), bf16),
            pltpu.VMEM((n_heads // 2, n_tiles, _LANES, _LANES), bf16),
            pltpu.VMEM((2 * n_ffn_units, n_tiles, _LANES, _LANES), bf16),
            pltpu.VMEM((n_heads // _UNIT + n_ffn_units, n_tiles, _LANES, _LANES), bf16),
            pltpu.VMEM((9, _LANES, _LANES), bf16),
            pltpu.SemaphoreType.DMA((3 * _SLOTS,)),
            pltpu.SemaphoreType.DMA((2,)),
            pltpu.SemaphoreType.DMA((n_tok // _LANES,)),
        ],
        compiler_params=pltpu.CompilerParams(vmem_limit_bytes=124 * 1024 * 1024),
    )(A_x.reshape(n_tok, d_model).T, A_mem0.reshape(n_mem, d_model), A_Wq, A_Wk, A_Wv,
      A_Wo.transpose(0, 2, 1), B_w1, B_w3, B_w2.T)
    return out_t.T.reshape(A_x.shape)
```

```python
import functools
import math

import jax
import jax.numpy as jnp
import jax.experimental.pallas as pl
import jax.experimental.pallas.tpu as pltpu

_EPS = 1e-05
_MASKED = -1000000000.0
_LOG2E = math.log2(math.e)
_LANES = 128
_CHUNK = _LANES // 2
_SLAB = 16
_TILES = 4
_PARTS = 2 * _TILES
_EARLY_ROWS = 48
_SLACK = 0.7
_UNROLL = True
_TURN_PAUSE = 1
_LAG = 4
_MODEL, _WEIGHT, _WIDE = range(3)
_HOPCROFT_KERR = (
    (((1, 1, 2),), ((1, 2, 0), (1, 2, 2), (1, 2, 3), (-1, 1, 2)), ((1, 2, 2),)),
    (((1, 2, 2),), ((1, 2, 1), (1, 2, 2), (-1, 0, 2), (-1, 3, 2)), ((1, 0, 2),)),
    (((1, 0, 2), (1, 0, 3)), ((1, 2, 3),), ((-1, 2, 2), (1, 2, 3))),
    (((1, 2, 2), (1, 0, 3)), ((1, 2, 3), (1, 3, 2)), ((1, 2, 2), (-1, 1, 3))),
    (((1, 2, 2), (1, 2, 3)), ((1, 3, 2),), ((-1, 1, 2), (1, 1, 3))),
    (((1, 0, 0), (1, 0, 2)), ((1, 2, 0),), ((1, 2, 0), (-1, 2, 2))),
    (((1, 0, 0), (1, 2, 2)), ((1, 0, 2), (1, 2, 0)), ((-1, 1, 0), (1, 2, 2))),
    (((1, 2, 0), (1, 2, 2)), ((1, 0, 2),), ((1, 1, 0), (-1, 1, 2))),
    (((1, 0, 1), (1, 0, 2)), ((1, 2, 1),), ((1, 0, 1), (-1, 0, 2))),
    (((1, 0, 1), (1, 1, 2)), ((1, 1, 2), (1, 2, 1)), ((1, 1, 1), (1, 0, 2))),
    (((1, 1, 1), (1, 1, 2)), ((1, 1, 2),), ((-1, 1, 1), (1, 1, 2))),
    (((1, 1, 1), (1, 1, 3)), ((1, 0, 3), (-1, 1, 3)), ((1, 2, 1), (-1, 2, 3))),
    (((1, 0, 0), (1, 0, 1), (1, 0, 3)), ((1, 0, 3),), ((1, 2, 1), (-1, 2, 0), (1, 2, 3))),
    (((1, 2, 0), (1, 2, 1), (1, 0, 3)), ((1, 0, 3), (1, 3, 0)),
     ((1, 2, 0), (-1, 2, 1), (-1, 1, 3))),
    (((1, 2, 0), (1, 2, 1), (1, 2, 3)), ((1, 3, 0),), ((1, 1, 1), (-1, 1, 0), (1, 1, 3))),
    (((1, 1, 3),), ((1, 0, 3), (-1, 1, 3), (1, 3, 0), (1, 3, 2), (1, 3, 3)), ((1, 1, 3),)),
    (((1, 2, 1), (1, 2, 3)), ((1, 3, 0), (1, 3, 1)), ((1, 0, 1), (-1, 0, 3))),
    (((1, 1, 3), (-1, 2, 1)), ((1, 3, 0), (1, 3, 1), (-1, 0, 3), (1, 1, 3)),
     ((1, 2, 1), (-1, 0, 3))),
    (((1, 0, 3),), ((1, 3, 0), (1, 3, 1), (-1, 0, 3), (-1, 2, 3), (1, 3, 3)), ((1, 0, 3),)),
    (((1, 1, 0), (1, 1, 1)), ((1, 0, 3), (1, 1, 0)), ((1, 2, 0), (-1, 2, 1))),
    (((1, 2, 1), (-1, 1, 0)), ((1, 0, 1), (1, 1, 0)), ((1, 0, 0), (-1, 2, 1))),
    (((1, 0, 1),), ((1, 1, 0), (1, 1, 1), (1, 1, 3), (-1, 0, 3), (-1, 2, 1)), ((1, 2, 1),)),
    (((1, 2, 0), (1, 2, 1)), ((1, 0, 1), (1, 3, 0)), ((-1, 0, 0), (1, 0, 1))),
    (((1, 2, 1),), ((1, 3, 0), (1, 3, 1), (1, 0, 1), (-1, 1, 1), (-1, 1, 2)), ((1, 1, 1),)),
    (((1, 0, 0),), ((1, 0, 0), (1, 0, 1), (-1, 2, 0)), ((1, 0, 0),)),
    (((1, 1, 0),), ((1, 0, 0), (1, 0, 2), (-1, 1, 0)), ((1, 1, 0),)),
)
_BATCHES = (0, 5, 11, 19, 24, 24)
_STRASSEN = (
    (((1, 1, 0), (1, 1, 1)), ((1, 0, 0),), ((1, 1, 0), (-1, 1, 1))),
    (((1, 1, 1),), ((1, 1, 0), (-1, 0, 0)), ((1, 2, 0),)),
    (((1, 0, 0), (1, 0, 1)), ((1, 1, 1),), ((-1, 0, 0), (1, 0, 1))),
    (((1, 0, 0),), ((1, 0, 1), (-1, 1, 1)), ((1, 2, 1),)),
    (((1, 0, 0), (1, 1, 1)), ((1, 0, 0), (1, 1, 1)), ((1, 0, 0), (1, 1, 1))),
    (((1, 2, 1),), ((1, 1, 0), (1, 1, 1)), ((1, 0, 0),)),
    (((1, 2, 0),), ((-1, 0, 0), (-1, 0, 1)), ((1, 1, 1),)),
)
_ATTENTION = (
    "P24 P25 P26 P0 P1 P2 S0 S1 P3 S2 S3 P4 V0 V1 P5 V2 V3 S4 S5 P6 S6 S7 O0 P7 V4 V5 P8 V6 V7 "
    "S8 S9 P9 S10 S11 O1 P10 V8 V9 P11 V10 V11 S12 S13 P12 S14 S15 O2 P13 V12 V13 P14 V14 V15 "
    "S16 S17 P15 S18 S19 O3 P16 V16 V17 P17 V18 V19 S20 S21 P18 S22 S23 O4 P19 V20 V21 P20 V22 "
    "V23 P21 S24 S25 P22 S26 S27 P23 S28 S29 V24 V25 S30 S31 V26 V27 O5 V28 V29 V30 V31 O6 O7 "
    "O8")
_SWIGLU = (
    "F4 X F0 F1 F2 F3 J W1000 G19 G20 G0 G1 G2 D0 G3 G4 D1 G5 G6 D2 G7 G8 D3 G9 G10 D4 G11 G12 "
    "G13 G14 D5 X G15 G18 G16 D6 G17 D7 D9 D8 D10")
_CLOSE = "A M1 M3 W20 D6 F4 W80 D7 D9 E"
_OPEN = (
    "F0 W98 G18 G19 N W200 G20 G16 G17 P24 P25 P26 G0 P0 P1 P2 S0 S1 S2 S3 P3 P4 V0 V1 V2 V3 "
    "P5 D8 D10 S4 S5 S6 S7 O0 G1 P6 P7 V4 V5 V6 V7 P8 S8 S9 S10 S11 O1 F1 W98 G2 P9 P10 V8 V9 "
    "V10 V11 P11 S12 S13 S14 S15 O2 D0 P12 P13 V12 V13 V14 V15 P14 S16 S17 S18 S19 O3 G3 P15 "
    "P16 V16 V17 V18 V19 P17 S20 S21 S22 S23 O4 G4 P18 P19 V20 V21 V22 V23 P20 S24 S25 S26 "
    "S27 O5 D1 P21 P22 V24 V25 V26 V27 P23 S28 S29 S30 S31 O6 G5 V28 V29 V30 V31 G6 O7 O8 A N "
    "W200 D2 F2 G7 G8 P24 P25 P26 D3 P0 P1 P2 S0 S1 S2 S3 P3 P4 V0 V1 V2 V3 P5 G9 S4 S5 S6 S7 "
    "O0 F3 W98 G10 P6 P7 V4 V5 V6 V7 P8 S8 S9 S10 S11 O1 D4 P9 P10 V8 V9 V10 V11 P11 S12 S13 "
    "S14 S15 O2 G11 P12 P13 V12 V13 V14 V15 P14 S16 S17 S18 S19 O3 G12 P15 P16 V16 V17 V18 "
    "V19 P17 S20 S21 S22 S23 O4 M0 M2 T W98 G13 P18 P19 V20 V21 V22 V23 P20 S24 S25 S26 S27 "
    "O5 G14 P21 P22 V24 V25 V26 V27 P23 S28 S29 S30 S31 O6 D5 V28 V29 V30 V31 G15 O7 O8")
_NORMALIZE_FIRST = False
_KEEP_P = False


def _layernorm(x):
    m = jnp.mean(x, axis=-1, keepdims=True)
    d = x - m
    v = jnp.mean(d * d, axis=-1, keepdims=True)
    return d * jax.lax.rsqrt(v + _EPS)


def _silu(x):
    return x * pltpu.reciprocal(1.0 + jnp.exp2(x * -_LOG2E), approx=True)


def _dot(a, b):
    return jnp.dot(a, b, preferred_element_type=jnp.float32)


def _dot_nt(a, b):
    return jax.lax.dot_general(a, b, (((1,), (1,)), ((), ())),
                               preferred_element_type=jnp.float32)


def _load_words(ref, *index):
    return ref[index] if ref.dtype == jnp.float32 else ref.bitcast(jnp.uint32)[index]


def _load_packed(ref, *index):
    return pltpu.bitcast(_load_words(ref, *index), ref.dtype)


def _low_lanes(shape):
    return jax.lax.broadcasted_iota(jnp.int32, shape, 1) < _CHUNK


def _accumulate(total, sign, value):
    if total is None:
        return sign, value
    if total[0] == sign:
        return sign, total[1] + value
    return 1, (total[1] - value if sign < 0 else value - total[1])


def _value(total):
    return total[1] if total[0] > 0 else -total[1]


def _upper_rows_only(level):
    def upper(terms):
        return tuple((sign, 0, i) for sign, f, i in terms if f != 1)

    kept = {r: (upper(model), weight, upper(wide))
            for r, (model, weight, wide) in enumerate(level)}
    return {r: product for r, product in kept.items() if product[_MODEL] and product[_WIDE]}


def _levels(groups):
    if groups == 1:
        return [_upper_rows_only(_HOPCROFT_KERR)]
    return [dict(enumerate(_HOPCROFT_KERR))] if groups == 2 else [dict(enumerate(_STRASSEN))] * 2


def _combination(terms, side, block):
    def term(a, b):
        if side == _WEIGHT or a < 2:
            return block(a, b)
        return block(0, b) - block(1, b) if side == _MODEL else block(0, b) + block(1, b)

    total = None
    for sign, a, b in terms:
        total = _accumulate(total, sign, term(a, b))
    return _value(total)


def _operands(levels, side, block):
    level, *inner = levels
    if not inner:
        block = functools.cache(block)
        return {r: functools.partial(_combination, product[side], side, block)
                for r, product in level.items()}
    operands = {}
    for r, product in level.items():
        def sub_block(a, b, terms=product[side]):
            return _combination(terms, side, lambda f, i: block(2 * f + a, 2 * i + b))

        for n, operand in _operands(inner, side, sub_block).items():
            operands[r * len(inner[0]) + n] = operand
    return operands


def _collect(levels, side, multiply, start, finish, partial_ref=None):
    level, *inner = levels
    terms = [term for product in level.values() for term in product[side]]
    left = {}
    for _, f, i in terms:
        left[f, i] = left.get((f, i), 0) + 1
    for i in sorted({i for _, f, i in terms if f == 2}):
        for f in range(2):
            left[f, i] = left.get((f, i), 0) + 1
    total = {}

    def add(f, i, sign, result):
        left[f, i] -= 1
        if f == 2:
            total[f, i] = _accumulate(total.get((f, i)), sign, result)
            if not left[f, i]:
                sign, result = total[f, i]
                add(0, i, sign, result)
                add(1, i, -sign if side == _MODEL else sign, result)
            return
        for (a, b), tile in result.items() if inner else [((0, 0), result)]:
            index = (2 * f + a, 2 * i + b) if inner else (f, i)
            key = f, i, a, b
            if key not in total:
                first = start(*index)
                before = None if first is None else (1, first)
            else:
                before = (total[key][0], partial_ref[index]) if inner else total[key]
            total[key] = _accumulate(before, sign, tile)
            if not left[f, i]:
                finish(*index, _value(total[key]))
            elif inner:
                partial_ref[index] = total[key][1]

    for r, product in level.items():
        if inner:
            result = {}
            _collect(inner, side, lambda n: multiply(r * len(inner[0]) + n), lambda f, i: None,
                     lambda f, i, tile: result.update({(f, i): tile}))
        else:
            result = multiply(r)
        for sign, f, i in product[side]:
            add(f, i, sign, result)


@functools.cache
def _operand_slots(groups):
    slots = {}
    for r in _operands(_levels(groups), _MODEL, lambda f, i: 0):
        used = set()
        _operands(_levels(groups), _MODEL, lambda f, i: used.add(i) or 0)[r]()
        for tile in [None] + sorted(used):
            slots[r, tile] = len(slots)
    return slots


class _SideJobs:
    def __init__(self, zero):
        self.zero, self.jobs, self.pace, self.due = zero, [], 0.0, 0.0

    def add(self, source_ref, job, key=None):
        self.jobs.append((key, source_ref, job))

    def spread(self, products):
        self.pace = len(self.jobs) / products

    def finish(self, *keys):
        while self.jobs and (not keys or any(key in keys for key, _, _ in self.jobs)):
            _, ref, job = self.jobs.pop(0)
            if ref is not None:
                job()

    def dot(self, a, b):
        result = _dot(a, b)
        self.due = self.due + self.pace if self.jobs else 0.0
        while self.jobs and self.due >= 1.0:
            self.due -= 1.0
            _, ref, job = self.jobs.pop(0)
            if ref is None:
                continue
            rows = 32 // ref.dtype.itemsize
            index = (self.zero,) * (ref.ndim - 2) + (
                slice(ref.shape[-2] - rows, None), slice(0, _LANES))
            ref[index] = (pltpu.bitcast(result[:rows], ref.dtype) if ref.dtype == jnp.uint32
                          else result[:rows].astype(ref.dtype))
            job()
        return result


def _store_rows(ref, f, first, x):
    rows = slice(first, first + x.shape[0])
    for i in range(_TILES):
        ref[f, i, rows] = x[:, i * _LANES:(i + 1) * _LANES]
    ref[f, _TILES, rows] = jnp.concatenate([x[:, _TILES * _LANES:]] * 2, axis=1)


def _combination_jobs(ref, groups, side, block, slots, n_rows):
    def job(batch, rows):
        operands = _operands(_levels(groups), side, lambda a, b: block(a, b, rows))
        for r, slot in batch:
            ref[slot, rows] = operands[r]().astype(ref.dtype)

    batches = {}
    for r, slot in slots.items():
        key = r // len(_STRASSEN) if groups == 4 else sum(r >= cut for cut in _BATCHES) % 4
        batches.setdefault(key, []).append((r, slot))
    step = _SLAB if groups > 1 else 8
    return [functools.partial(job, batch, slice(first, first + step))
            for batch in batches.values() for first in range(0, n_rows, step)]


def _operand_jobs(ref, rows_ref, groups, tile):
    return _combination_jobs(
        ref, groups, _MODEL, lambda f, i, rows: rows_ref[f, _TILES if i == tile else i, rows],
        {r: slot for (r, replaced), slot in _operand_slots(groups).items() if replaced == tile},
        ref.shape[1])


def _operand_loader(ref, groups, part):
    slots = _operand_slots(groups)
    rows = ref.shape[-2] * ref.dtype.itemsize // 4
    lanes = jax.lax.broadcasted_iota(jnp.int32, (rows, _LANES), 1)
    replaced = (lanes & _CHUNK) == (part & 1) * _CHUNK
    if isinstance(part, int):
        others = {r: slot for (r, tile), slot in slots.items() if tile == part // 2}
    else:
        others = {}
        for (r, tile), slot in slots.items():
            others[r] = slot if tile is None else jnp.where(part >> 1 == tile, slot, others[r])

    def load(r, *index):
        words = _load_words(ref, *index, slots[r, None])
        if r in others:
            words = jax.lax.select(replaced, _load_words(ref, *index, others[r]), words)
        return pltpu.bitcast(words, ref.dtype) if words.dtype != ref.dtype else words

    return load


def _store_packed(ref, index, value):
    ref.bitcast(jnp.uint32)[index] = pltpu.bitcast(value, jnp.uint32)


def _merge(ref, f):
    low = _low_lanes(ref.shape[-2:])
    tiles, rest = [], None
    for i in range(_TILES):
        a, b = ref[f, _TILES + 2 * i], ref[f, _TILES + 2 * i + 1]
        tiles.append(ref[f, i] + jnp.where(low, b, a))
        rest = _accumulate(rest, 1, jnp.where(low, a, b))
    for i in range(_TILES + _PARTS, ref.shape[1]):
        rest = _accumulate(rest, 1, ref[f, i])
    return jnp.concatenate(tiles + [rest[1][:, :_CHUNK] + rest[1][:, _CHUNK:]], axis=1)


def _attention_masks(n_mem, seg):
    size = n_mem + seg
    shape = (2 * size, 2 * size)

    def position(axis):
        r = jax.lax.broadcasted_iota(jnp.int32, shape, axis)
        return r < size, jnp.where(r < seg, r + n_mem, jnp.where(r < size, r - seg, r - size))

    (first_i, i), (first_j, j) = position(0), position(1)
    same = first_i == first_j
    fill = jnp.where(same, _MASKED * _LOG2E, -jnp.inf).astype(jnp.float32)
    return same & ((i < n_mem) | (i >= j)), fill


def _when(condition, function):
    if not isinstance(condition, bool):
        pl.when(condition)(function)
    elif condition:
        function()


def _start(copies):
    for copy in copies:
        copy.start()


def _wait(copies):
    for copy in copies:
        copy.wait()


def _kernel(xt_hbm, mem0_hbm, wq_hbm, wk_hbm, wv_hbm, wot_hbm, w1_hbm, w3_hbm, w2t_hbm,
            outt_hbm, mem0_ref, tile_ref, x_ref, early_ref, wq_ref, wk_ref, wv_ref, stage_ref,
            wide_ref, stage_sem, mem_sem, tile_sem, *, seg):
    d_model, n_tok = xt_hbm.shape
    n_mem = mem0_ref.shape[0]
    _, n_heads, d_head = wq_hbm.shape
    n_seg = n_tok // seg
    n_io = n_tok // _LANES
    size = n_mem + seg
    ahead = seg // 2
    width = _TILES * _LANES
    score_scale = d_head ** -0.5 * _LOG2E
    f32, bf16, words = jnp.float32, jnp.bfloat16, jnp.uint32
    attn_tiles, ffn_tiles = len(_HOPCROFT_KERR), len(_STRASSEN) ** 2
    weight_refs = wq_ref, wk_ref, wv_ref
    behind = (_PARTS + 1) * attn_tiles
    stitched = 6

    side = _SideJobs(jax.lax.fori_loop(0, 3, lambda i, total: total - i, 3))

    def combine_weights(out_ref, groups, source_ref, block, n_rows, n_tiles):
        def widen(first, tiles):
            rows = range(first, first + n_rows)
            for j, tile in [(j, block(rows, j)) for j in tiles]:
                wide_ref[first // _LANES, j, pl.ds(first % _LANES, n_rows)] = tile

        for j in range(0, _TILES, n_tiles):
            for first in range(0, width, n_rows):
                side.add(source_ref, functools.partial(widen, first, range(j, j + n_tiles)))
                for _ in range(_TURN_PAUSE if n_rows == _LANES else 0):
                    side.add(None, None)
        for job in _combination_jobs(out_ref, groups, _WEIGHT,
                                     lambda i, j, rows: wide_ref[i, j, rows],
                                     {r: r for r in range(out_ref.shape[0])}, _LANES):
            side.add(wide_ref, job)

    def staged_rows(part, rows, packing):
        count = min(len(rows), _CHUNK)
        for first in rows[::count]:
            c, offset = divmod(first, _CHUNK)
            if isinstance(part, int):
                first = ((_PARTS if c == part else c) * _CHUNK + offset) // packing
            else:
                first = pl.multiple_of(
                    jnp.where(part == c, _PARTS, c) * (_CHUNK // packing) + offset // packing,
                    count // packing)
            yield pl.ds(first, count // packing)

    def block_copies(m, part, slot, rows=pl.ds(0, d_model // 2)):
        dst, sem = stage_ref.at[slot], stage_sem.at[slot]
        if m == 0:
            return [pltpu.make_async_copy(wot_hbm.bitcast(words).at[_TILES * part + j, rows],
                                          dst.at[rows, pl.ds(j * _LANES, _LANES)], sem)
                    for j in range(_TILES)]
        first = part * width if isinstance(part, int) else pl.multiple_of(part * width, width)
        src = (w1_hbm, w3_hbm, w2t_hbm)[m - 1].bitcast(words)
        return [pltpu.make_async_copy(src.at[rows, pl.ds(first, width)], dst.at[rows], sem)]

    def stitch_copies(m):
        return [copy for c in range(_PARTS) for copy in block_copies(
            m, c, stitched + m, pl.ds(c * _CHUNK // 2, _CHUNK // 2))]

    def staged(slot, part, rows, j):
        tile = pltpu.bitcast(jnp.concatenate(
            [stage_ref[slot, piece, j * _LANES:(j + 1) * _LANES]
             for piece in staged_rows(part, rows, 2)], axis=0), bf16)
        return (tile.T if len(rows) == _LANES else tile).astype(f32)

    def store_block(m, out_ref, unit, block):
        tiles = ffn_tiles if m else attn_tiles
        out_ref = out_ref.at[pl.ds(unit * tiles + (behind if m < 3 else 0), tiles)]
        combine_weights(out_ref, 4 if m else 2, stage_ref, block,
                        _CHUNK if m in (1, 2) else _LANES, 1)

    def store_part(m, out_ref, part, slot):
        store_block(m, out_ref, part, lambda rows, j: (
            staged(slot, part, rows, j) - staged(stitched + m, part, rows, j)))

    def store_shared(m, out_ref):
        store_block(m, out_ref, _PARTS + 1 if m else _PARTS,
                    functools.partial(staged, stitched + m, _PARTS))

    def load_weights(early_in_ref, early_shared_ref, head_ref, head_sem, *rows_refs):
        n_chunks, _, rows_per_group, _ = early_in_ref.shape
        per_group = rows_per_group // ahead

        def head_copies(w, part, slot, rows=pl.ds(0, d_model)):
            src = (wq_hbm, wk_hbm, wv_hbm)[w].bitcast(words)
            return [pltpu.make_async_copy(src.at[rows, 2 * part + n, :],
                                          head_ref.at[slot, n, rows], head_sem.at[slot])
                    for n in range(2)]

        def head_stitch_copies(w):
            return [copy for c in range(_PARTS)
                    for copy in head_copies(w, c, stitched + w, pl.ds(c * _CHUNK, _CHUNK))]

        def store_heads(w, part, slot=None):
            def head(slot, rows, j):
                pair = head_ref[slot, j // 2, next(staged_rows(part, rows, 1)), :]
                return pltpu.bitcast(pair & words(0xFFFF0000) if j % 2 else pair << 16, f32)

            def block(rows, j):
                shared = head(stitched + w, rows, j)
                return shared if slot is None else head(slot, rows, j) - shared

            combine_weights(weight_refs[w].at[pl.ds(part * attn_tiles, attn_tiles)], 2,
                            head_ref, block, _CHUNK // 2, 2)

        def x_copy(i):
            cols = pl.ds(i * _LANES, _LANES)
            return pltpu.make_async_copy(xt_hbm.at[:, cols], tile_ref.at[i, :d_model],
                                         tile_sem.at[i])

        def transpose_in(i):
            x_ref[i // 2, i % 2 * _LANES:(i % 2 + 1) * _LANES, :] = _load_packed(
                tile_ref, i, slice(0, d_model // 2)).T

        def normalize(c):
            def job(s):
                block, first = divmod((_LAG + 2 * per_group * c + s) * seg, 2 * _LANES)
                _store_rows(rows_refs[c % 3], s // per_group, s % per_group * ahead,
                            _layernorm(x_ref[block, first:first + ahead, :].astype(f32)))

            for s in range(2 * per_group):
                side.add(x_ref, functools.partial(job, s))

        def prepare(c, tiles=(None, *range(_TILES))):
            for tile in tiles:
                for job in _operand_jobs(early_in_ref.at[c], rows_refs[c % 3], 2, tile):
                    side.add(rows_refs[c % 3], job)

        def project(w, part, c, operand):
            def keep(f, j, tile):
                early_shared_ref[w, c, f, j] = tile

            def store(f, j, tile):
                for s in range(per_group):
                    early_ref[part, (2 * c + f) * per_group + s, _TILES * w + j] = (
                        tile[s * ahead:(s + 1) * ahead].astype(bf16))

            shared = isinstance(part, int) and part == _PARTS
            unit_ref = weight_refs[w].at[pl.ds(part * attn_tiles, attn_tiles)]
            _collect(_levels(2), _WIDE,
                     lambda r: side.dot(operand(r, c), _load_packed(unit_ref, r)),
                     lambda f, j: None if shared else early_shared_ref[w, c, f, j],
                     keep if shared else store)

        def copies_for(part):
            slot = 3 * (part & 1)
            following = min(part + 1, _PARTS - 1) if isinstance(part, int) else jnp.minimum(part + 1, _PARTS - 1)
            return [copy for w in (1, 2, 0) for copy in (
                head_copies(w, part if w else following, slot + w) + block_copies(w, part, slot + w))]

        def last_tile(c):
            return ((_LAG + 2 * per_group * (c + 1)) * seg - 1) // _LANES

        def tiles_for(c):
            first = last_tile(c - 1) + 1 if c else 1
            return [i % n_io for i in range(first, min(last_tile(c), n_io) + 1)]

        def x_copies(first, last):
            return [x_copy(i) for c in range(first, last) for i in tiles_for(c)]

        _start(x_copies(0, 2) + head_stitch_copies(0))
        for w in range(3):
            head_ref[stitched + w, :, width:d_model, :] = jnp.zeros((2, _CHUNK, d_head), words)
        for m in range(4):
            stage_ref[stitched + m, width // 2:d_model // 2, :] = jnp.zeros(
                (_CHUNK // 2, width), words)
        for ref in (early_in_ref, early_shared_ref):
            ref[(side.zero,) * (ref.ndim - 2)] = jnp.zeros(ref.shape[-2:], ref.dtype)
        _start(head_stitch_copies(1) + x_copies(2, 4) + head_stitch_copies(2))
        _wait(x_copies(0, 2))
        for c in range(2):
            for i in tiles_for(c):
                transpose_in(i)
            normalize(c)
            prepare(c, [None])
        side.finish()
        later = x_copies(4, n_chunks + 1) + head_copies(0, 0, 3) + stitch_copies(0)
        _start(later)
        _wait(head_stitch_copies(0))
        store_heads(0, _PARTS)
        side.finish()
        _wait(head_stitch_copies(1) + x_copies(2, 4) + head_stitch_copies(2))
        operand = _operand_loader(early_in_ref, 2, _PARTS)
        for w in range(3):
            if w < 2:
                for i in tiles_for(w + 2):
                    side.add(tile_ref, functools.partial(transpose_in, i))
                store_heads(w + 1, _PARTS)
            else:
                normalize(2)
                prepare(0, range(_TILES))
                normalize(3)
                prepare(2, [None])
            side.spread(1.5 * attn_tiles)
            for c in range(2):
                project(w, _PARTS, c, operand)
            side.finish()
        _wait(later)
        _start(stitch_copies(1) + stitch_copies(2) + copies_for(0))
        for c in range(2, n_chunks):
            for i in tiles_for(c + 2):
                side.add(tile_ref, functools.partial(transpose_in, i))
            if c + 1 < n_chunks:
                prepare(c + 1, [None])
            prepare(c - 1, range(_TILES))
            if c + 2 < n_chunks:
                normalize(c + 2)
            if c + 2 == n_chunks:
                store_heads(0, 0, 3)
            if c + 1 == n_chunks:
                prepare(c, range(_TILES))
                store_shared(0, wq_ref)
            side.spread(3 * attn_tiles)
            for w in range(3):
                project(w, _PARTS, c, operand)
            side.finish()
        _wait(stitch_copies(1) + stitch_copies(2))

        def project_part(part):
            _when(part + 1 < _PARTS, lambda: _start(copies_for(part + 1)))
            _when(part + 1 == _PARTS, lambda: _start(
                stitch_copies(3) + block_copies(3, 0, 0) + block_copies(3, 1, 1)))
            _wait(copies_for(part))
            operand = _operand_loader(early_in_ref, 2, part)
            for w in range(3):
                m = (w + 1) % 3
                slot = 3 * (part & 1) + m
                store_part(m, weight_refs[m], part, slot)
                if m or not isinstance(part, int):
                    store_heads(m, part if m else jnp.minimum(part + 1, _PARTS - 1), slot)
                elif part + 1 < _PARTS:
                    store_heads(m, part + 1, slot)
                side.spread((n_chunks - _SLACK) * attn_tiles)
                for c in range(n_chunks):
                    project(w, part, c, operand)
                side.finish()

        if _UNROLL:
            for part in range(_PARTS):
                project_part(part)
        else:
            pl.loop(0, _PARTS)(project_part)

    def run_layers(wdown_ref, wplain_ref, pair_rows_ref, pair_in_ref, solo_rows_ref, solo_in_ref,
                   ffn_rows_ref, ffn_in_ref, attn_shared_ref, ffn_shared_ref, partial_ref, qkv_ref,
                   heads_ref, hidden_ref, attn_sum_ref, ffn_sum_ref, mem_ref, block_ref,
                   second_ref):
        def store_last(m):
            slot = 3 + m if m < 3 else 0
            part = m - 1 if m < 3 else _PARTS

            def block(rows, j):
                own = staged(slot, part, rows, j)
                if m < 3 and rows[0] == (2 - m) * _CHUNK:
                    return own - staged(6 - m, part, rows, j)
                return own

            store_block(m, wdown_ref if m == 3 else weight_refs[m], _PARTS, block)
            for j in range(_TILES):
                rows = range(part * _CHUNK, (part + 1) * _CHUNK)
                tile = staged(slot, _PARTS, rows, j)
                if m < 3:
                    wplain_ref[j, rows.start:rows.stop, :] = tile.astype(bf16)
                else:
                    _store_packed(wplain_ref, _TILES + j, jnp.concatenate(
                        [tile, jnp.zeros_like(tile)], axis=0).astype(bf16).T)

        def segment(s):
            first = (s & 7) * seg
            return s >> 3, pl.ds(first if isinstance(s, int) else pl.multiple_of(first, seg), seg)

        def transpose_out(i):
            first = (i & 1) * _LANES
            rows = pl.ds(first if isinstance(i, int) else pl.multiple_of(first, _LANES), _LANES)
            _store_packed(tile_ref, (i, slice(0, d_model // 2)), x_ref[i >> 1, rows].T)

        def contract(groups, part, tile_of, weight_ref, first, sum_ref, begun, dtype, slot):
            operands = _operands(_levels(groups), _WIDE, tile_of)

            def target(i):
                return _TILES + part if i == part // 2 else i

            def start(f, i):
                return sum_ref[f, i] if target(i) in begun else None

            def finish(f, i, tile):
                sum_ref[f, target(i)] = tile

            _collect(_levels(groups), _MODEL,
                     lambda r: side.dot(operands[r]().astype(dtype), _load_packed(weight_ref, first + r)),
                     start, finish, partial_ref.at[slot])
            begun.update(map(target, range(_TILES)))

        def keep_and_add(ref, part, total, f, j, tile):
            ref[part, f, j] = tile
            if part < _PARTS:
                ref[total, f, j] = ref[total if part > 1 else 0, f, j] + tile if part else tile

        def attention_stage(stage, g, step):
            t, groups = step["t"], step["groups"]
            in_ref, rows_ref = (pair_in_ref, pair_rows_ref) if groups == 2 else (
                solo_in_ref, solo_rows_ref)
            rows = slice(0, in_ref.shape[1])
            if stage == "P":
                part, w = divmod(g, 3)
                side.finish(("P", None), ("P", part // 2))
                operand = _operand_loader(in_ref, groups, part)
                done = {}

                def finish(f, j, tile):
                    done[f, j] = tile
                    n = (_TILES * part + j) % qkv_ref.shape[0]
                    if part == _PARTS:
                        attn_shared_ref[w, f, j, rows] = tile
                    elif groups == 2 and (1 - f, j) in done:
                        upper, lower = done[0, j], done[1, j]
                        qkv_ref[n, w, :2 * size - ahead] = jnp.concatenate(
                            [upper[n_mem:n_mem + ahead], upper[:n_mem], lower[:n_mem],
                             upper[n_mem + ahead:], lower[n_mem:]], axis=0).astype(bf16)
                    elif groups == 1 and (0, j ^ 1) in done:
                        a, b = done[0, j & ~1], done[0, j | 1]
                        qkv_ref[n | 1, w] = jnp.concatenate(
                            [a[n_mem:], a[:n_mem], b], axis=0).astype(bf16)

                _collect(_levels(groups), _WIDE,
                         lambda r: side.dot(operand(r),
                                        _load_packed(weight_refs[w], part * attn_tiles + r)),
                         lambda f, j: attn_shared_ref[w, f, j, rows] if part < _PARTS else None,
                         finish)
            elif stage == "O":
                contract(groups, g, lambda f, j: heads_ref[g, f, j], wq_ref,
                         behind + g * attn_tiles, attn_sum_ref,
                         step["begun"], f32, 0)
            elif groups == 2 or g % 2:
                part, j = divmod(g, _TILES)

                def projected(w):
                    if groups == 1:
                        return _load_packed(qkv_ref, g % qkv_ref.shape[0], w)
                    return pltpu.bitcast(jnp.concatenate(
                        [_load_words(early_ref, part, t - _LAG, _TILES * w + j),
                         _load_words(qkv_ref, g % qkv_ref.shape[0], w, slice(0, size - ahead // 2))], axis=0), bf16)

                if stage == "S":
                    visible, fill = step["masks"]
                    s = jnp.where(visible, _dot_nt(projected(0), projected(1)) * score_scale, fill)
                    p = jnp.exp2(s - jnp.max(s, axis=-1, keepdims=True))
                    inv = pltpu.reciprocal(jnp.sum(p, axis=-1, keepdims=True), approx=True)
                    if _NORMALIZE_FIRST:
                        p, inv = p * inv, None
                    if _KEEP_P:
                        qkv_ref[g, 0, :, :2 * size] = p.astype(bf16)
                    step[g] = p.astype(bf16), inv
                else:
                    p, inv = step[g]
                    if _KEEP_P:
                        p = _load_packed(qkv_ref, g, 0, slice(None), slice(0, 2 * size))
                    o = _dot(p, projected(2))
                    if inv is not None:
                        o = o * inv
                    halves = jnp.concatenate([o[seg:size], o[:seg]], axis=0), o[size:]
                    for f, half in enumerate(halves):
                        index = (f, j) if groups == 2 else (0, j - 1 + f)
                        keep_and_add(heads_ref, part, _PARTS, *index, half)

        def swiglu_stage(stage, g, state):
            plain = 2 * _PARTS + 2
            if stage == "G" and g == plain:
                side.finish("M")
                x = jnp.concatenate([ffn_rows_ref[f, 0, :seg] for f in range(4)], axis=0).astype(bf16)
                for j in range(_TILES):
                    tile = _dot(x, _load_packed(wplain_ref, j))
                    for f in range(4):
                        ffn_shared_ref[2, f, j] = tile[f * seg:(f + 1) * seg]
            elif stage == "G":
                part, up = divmod(g, 2) if g < plain else (None, g - plain - 1)
                chunk = _PARTS if part is None else part if part < _PARTS else up
                side.finish(("G", None), ("G", chunk // 2))
                operand = _operand_loader(ffn_in_ref, 4, chunk)
                first = behind + (_PARTS + 1 if part is None else part) * ffn_tiles

                def finish(f, j, tile):
                    if part is None:
                        ffn_shared_ref[up, f, j] = tile
                    elif up:
                        keep_and_add(hidden_ref, part, _PARTS + 1, f, j,
                                     hidden_ref[part, f, j] * tile)
                    else:
                        hidden_ref[part, f, j] = _silu(tile)

                _collect(_levels(4), _WIDE,
                         lambda r: side.dot(operand(r), _load_packed(weight_refs[1 + up], first + r)),
                         lambda f, j: None if part is None else ffn_shared_ref[
                             up if part < _PARTS else 2, f, j],
                         finish, partial_ref.at[g % 2])
            elif g == _PARTS + 2:
                tile = sum(
                    _dot(jnp.concatenate([hidden_ref[_PARTS, f, j] for f in range(4)],
                                         axis=0).astype(bf16),
                         _load_packed(wplain_ref, _TILES + j)) for j in range(_TILES))
                for f in range(4):
                    ffn_sum_ref[f, _TILES + _PARTS] = tile[f * seg:(f + 1) * seg]
            else:
                contract(4, g, lambda f, j: hidden_ref[g, f, j], wdown_ref, g * ffn_tiles, ffn_sum_ref,
                         state["begun"], bf16, g % 2)

        def run(order, t, layers, *, resumed=False, queue=lambda: None):
            state = dict(stored=set(), begun=set(range(_TILES)) if resumed else set())
            step = None
            masks = _attention_masks(n_mem, seg)
            for name in order.split():
                stage, g = name[0], int(name[1:] or 0)
                if stage == "N":
                    begin_step(t, layers)
                    step = dict(t=t, groups=len(layers), begun=set(), stored=set(), masks=masks)
                    t = t + 1
                elif stage == "A":
                    close_step(t - 1, layers)
                elif stage == "M":
                    if len(layers) == 2:
                        normalize(((t - 1) // 2 + 1) % 2, g)
                elif stage == "F":
                    tile = g if g < _TILES else None
                    for job in _operand_jobs(ffn_in_ref, ffn_rows_ref, 4, tile):
                        side.add(ffn_rows_ref, job, ("G", tile))
                elif stage == "J":
                    queue()
                elif stage == "W":
                    side.spread(g)
                elif stage == "X":
                    side.finish()
                elif stage == "E":
                    done = close_swiglu((t // 2 + 1) % 2)
                    first = jnp.maximum(t - 2 * _LAG, 0)
                    for s in range(2):
                        second_ref[s, :seg] = done[s]
                        x_ref[segment(first + s)] = done[2 + s].astype(bf16)
                elif stage == "T":
                    side.add(x_ref, functools.partial(
                        transpose_out, jnp.maximum(t - 11, 0) >> 2))
                elif stage in "GD":
                    swiglu_stage(stage, g, state)
                else:
                    attention_stage(stage, g, step)
            side.finish()

        def layer_input(t, layer):
            return x_ref[segment(t)].astype(f32) if layer == 0 else second_ref[(t & 1), :seg]

        def begin_step(t, layers):
            cut = ahead // 2
            if len(layers) == 1:
                rows_ref, in_ref = solo_rows_ref, solo_in_ref
                pieces = [(0, n_mem, layers[0], slice(0, seg))]
            else:
                rows_ref, in_ref = pair_rows_ref, pair_in_ref
                pieces = [(0, n_mem, 0, slice(ahead, seg)), (0, seg - cut, 1, slice(0, cut)),
                          (1, n_mem, 1, slice(cut, ahead)), (1, ahead, 1, slice(ahead, seg))]

            def normalize(f, first, layer, rows):
                _store_rows(rows_ref, f, first, _layernorm(layer_input(t, layer)[rows]))

            for piece in pieces:
                side.add(second_ref if piece[2] else x_ref, functools.partial(normalize, *piece),
                         ("P", None))
            for f, layer in enumerate(layers):
                _store_rows(rows_ref, f, 0, mem_ref[layer])
            for tile in [None, *range(_TILES)]:
                for job in _operand_jobs(in_ref, rows_ref, len(layers), tile):
                    side.add(rows_ref, job, ("P", tile))

        def close_step(t, layers):
            for f, layer in enumerate(layers):
                out = _merge(attn_sum_ref, f)
                mem_ref[layer] = out[:n_mem]
                index = (((t >> 1) + 1) & 1, 2 * layer + (t & 1)) if len(layers) == 2 else (
                    layer, t & 3)
                block_ref[(*index, slice(0, seg))] = layer_input(t, layer) + out[n_mem:]

        def normalize(block, f):
            def job(first):
                _store_rows(ffn_rows_ref, f, first,
                            _layernorm(block_ref[block, f, first:first + _SLAB]))

            for first in range(0, seg, _SLAB):
                side.add(block_ref, functools.partial(job, first), "M")

        def close_swiglu(block):
            return [block_ref[block, f, :seg] + _merge(ffn_sum_ref, f) for f in range(4)]

        def solo_swiglu(block, queue=lambda: None):
            for f in range(4):
                normalize(block, f)
            run(_SWIGLU, None, None, queue=queue)
            return close_swiglu(block)

        for ref in (pair_in_ref, solo_rows_ref, solo_in_ref, ffn_in_ref, attn_shared_ref,
                    ffn_shared_ref, partial_ref, qkv_ref, heads_ref, hidden_ref, attn_sum_ref,
                    ffn_sum_ref):
            ref[(side.zero,) * (ref.ndim - 2)] = jnp.zeros(ref.shape[-2:], ref.dtype)

        mem_copy.wait()
        for layer in range(2):
            mem_ref[layer] = mem0_ref[...].astype(f32)

        last_copies = block_copies(1, _PARTS, 4) + block_copies(2, _PARTS, 5)
        _start(last_copies)
        _wait(stitch_copies(3))

        @pl.loop(0, _LAG)
        def _first_steps(t):
            for part in (2 * t + 2, 2 * t + 3):
                _when(part <= _PARTS, lambda: _start(block_copies(3, part, part & 3)))
            for part in (2 * t, 2 * t + 1):
                _wait(block_copies(3, part, part & 3))
            def queue():
                for part in (2 * t, 2 * t + 1):
                    store_part(3, wdown_ref, part, part & 3)

            run("N J W540 " + _ATTENTION + " A", t, (0,), queue=queue)

        _wait(block_copies(3, _PARTS, 0) + last_copies)
        for m in (1, 2):
            store_shared(m, weight_refs[m])

        def queue():
            for m in (1, 2, 3):
                store_last(m)
            store_shared(3, wdown_ref)

        done = solo_swiglu(0, queue)
        for s in range(2):
            second_ref[s, :seg] = done[s]
            block_ref[0, s, :seg] = done[2 + s]
        run("N W200 " + _ATTENTION + " A N M0 M2 W200 " + _ATTENTION, _LAG, (0, 1))
        ffn_sum_ref[...] = jnp.zeros_like(ffn_sum_ref)
        for name in _CLOSE.split():
            if name[0] == "D":
                hidden_ref[int(name[1:])] = jnp.zeros(hidden_ref.shape[1:], f32)

        @pl.loop(_LAG // 2 + 1, n_seg // 2)
        def _steps(b):
            run(_CLOSE, 2 * b, (0, 1), resumed=True)
            run(_OPEN, 2 * b, (0, 1))

        out_copies = [
            pltpu.make_async_copy(tile_ref.at[i, :d_model], outt_hbm.at[:, pl.ds(i * _LANES, _LANES)],
                                  tile_sem.at[i]) for i in range(n_io)]
        _start(out_copies[:n_io - 3])
        run(_CLOSE, n_seg, (0, 1), resumed=True)
        run(_OPEN, n_seg, (1,))
        run(_CLOSE, n_seg + 2, (1,), resumed=True)
        transpose_out(n_io - 2)
        _start(out_copies[n_io - 3:n_io - 1])
        pl.loop(n_seg + 2, n_seg + _LAG)(lambda t: run("N W200 " + _ATTENTION + " A", t, (1,)))
        for s, x in enumerate(solo_swiglu(1)):
            x_ref[segment(n_seg - _LAG + s)] = x.astype(bf16)
        transpose_out(n_io - 1)
        out_copies[n_io - 1].start()
        _wait(out_copies)

    mem_copy = pltpu.make_async_copy(mem0_hbm, mem0_ref, mem_sem)
    mem_copy.start()
    n_chunks = (n_seg - _LAG) * ahead // (2 * _EARLY_ROWS)
    pl.run_scoped(
        load_weights,
        pltpu.VMEM((n_chunks, len(_operand_slots(2)), _EARLY_ROWS, _LANES), bf16),
        pltpu.VMEM((3, n_chunks, 2, _TILES, _EARLY_ROWS, _LANES), f32),
        pltpu.VMEM((stitched + 3, 2, d_model + 8, d_head), words),
        pltpu.SemaphoreType.DMA((stitched + 3,)),
        *[pltpu.VMEM((2, _TILES + 1, _EARLY_ROWS + 8, _LANES), f32)] * 3)
    pl.run_scoped(
        run_layers,
        pltpu.VMEM(((_PARTS + 2) * ffn_tiles, _LANES, _LANES), bf16),
        pltpu.VMEM((2 * _TILES, _LANES, _LANES), bf16),
        pltpu.VMEM((2, _TILES + 1, seg + 8, _LANES), f32),
        pltpu.VMEM((len(_operand_slots(2)), seg, _LANES), bf16),
        pltpu.VMEM((1, _TILES + 1, size + 8, _LANES), f32),
        pltpu.VMEM((len(_operand_slots(1)), size, _LANES), f32),
        pltpu.VMEM((4, _TILES + 1, seg + 8, _LANES), f32),
        pltpu.VMEM((len(_operand_slots(4)), seg, _LANES), bf16),
        pltpu.VMEM((3, 2, _TILES, size, _LANES), f32),
        pltpu.VMEM((3, 4, _TILES, seg, _LANES), f32),
        pltpu.VMEM((2, 4, _TILES, seg, _LANES), f32),
        pltpu.VMEM((12, 3, 2 * size, _LANES), bf16),
        pltpu.VMEM((_PARTS + 1, 2, _TILES, size, _LANES), f32),
        pltpu.VMEM((_PARTS + 2, 4, _TILES, seg, _LANES), f32),
        pltpu.VMEM((2, _TILES + _PARTS, size, _LANES), f32),
        pltpu.VMEM((4, _TILES + _PARTS + 1, seg, _LANES), f32),
        pltpu.VMEM((2, n_mem, d_model), f32),
        pltpu.VMEM((2, 4, seg + 8, d_model), f32),
        pltpu.VMEM((2, seg + 8, d_model), f32))


@functools.partial(jax.jit, static_argnames=("A_seg_len",))
def pallas_interleave_layers__memory_aug_recurrent_mem_tr__glu_gated_swiglu__prompt_kernel(
    A_x: jax.Array,
    A_mem0: jax.Array,
    A_Wq: jax.Array,
    A_Wk: jax.Array,
    A_Wv: jax.Array,
    A_Wo: jax.Array,
    A_seg_len: int,
    B_x: jax.Array,
    B_w1: jax.Array,
    B_w3: jax.Array,
    B_w2: jax.Array,
):
    del B_x
    _, n_tok, d_model = A_x.shape
    n_mem = A_mem0.shape[1]
    _, n_heads, d_head = A_Wq.shape
    seg = A_seg_len
    assert A_x.shape[0] == 1 and _LAG * seg == d_head == _LANES and 4 * n_mem == seg
    assert n_heads == _PARTS * _TILES and d_model == (_PARTS + 1) * _CHUNK
    assert B_w1.shape[1] == (_PARTS + 1) * _TILES * _LANES
    bf16 = jnp.bfloat16
    attn_tiles = (_PARTS + 1) * len(_HOPCROFT_KERR)
    ffn_tiles = (_PARTS + 2) * len(_STRASSEN) ** 2
    hbm = pl.BlockSpec(memory_space=pltpu.HBM)
    out_t = pl.pallas_call(
        functools.partial(_kernel, seg=seg),
        out_shape=jax.ShapeDtypeStruct((d_model, n_tok), A_x.dtype),
        in_specs=[hbm] * 9,
        out_specs=hbm,
        scratch_shapes=[
            pltpu.VMEM((n_mem, d_model), bf16),
            pltpu.VMEM((n_tok // _LANES, d_model + 16, _LANES), bf16),
            pltpu.VMEM((n_tok // (2 * _LANES), 2 * _LANES + 16, d_model), bf16),
            pltpu.VMEM((_PARTS, n_tok // seg - _LAG, 3 * _TILES, seg // 2, _LANES), bf16),
            pltpu.VMEM((2 * attn_tiles, _LANES, _LANES), bf16),
            pltpu.VMEM((attn_tiles + ffn_tiles, _LANES, _LANES), bf16),
            pltpu.VMEM((attn_tiles + ffn_tiles, _LANES, _LANES), bf16),
            pltpu.VMEM((10, d_model // 2 + 8, _TILES * _LANES), jnp.uint32),
            pltpu.VMEM((_TILES, _TILES, _LANES + 8, _LANES), jnp.float32),
            pltpu.SemaphoreType.DMA((10,)),
            pltpu.SemaphoreType.DMA(()),
            pltpu.SemaphoreType.DMA((n_tok // _LANES,)),
        ],
        compiler_params=pltpu.CompilerParams(
            vmem_limit_bytes=127 * 1024 * 1024, disable_bounds_checks=True,
            flags={"XLA_TPU_FORCE_LP_LLO_SCHEDULER": True}),
    )(A_x.reshape(n_tok, d_model).T, A_mem0.reshape(n_mem, d_model), A_Wq, A_Wk, A_Wv,
      A_Wo.transpose(0, 2, 1), B_w1, B_w3, B_w2.T)
    return out_t.T.reshape(A_x.shape)
```

```python
import functools
import math

import jax
import jax.numpy as jnp
import jax.experimental.pallas as pl
import jax.experimental.pallas.tpu as pltpu

_EPS = 1e-05
_MASKED = -1000000000.0
_LOG2E = math.log2(math.e)
_LANES = 128
_CHUNK = _LANES // 2
_SLAB = 16
_TILES = 4
_PARTS = 2 * _TILES
_EARLY_ROWS = 32
_SLACK = 0.7
_UNROLL = 8
_TURN_PAUSE = 1
_WEAVE = True
_MIDDLE = 8
_LAG = 4
_MODEL, _WEIGHT, _WIDE = range(3)
_HOPCROFT_KERR = (
    (((1, 1, 2),), ((1, 2, 0), (1, 2, 2), (1, 2, 3), (-1, 1, 2)), ((1, 2, 2),)),
    (((1, 2, 2),), ((1, 2, 1), (1, 2, 2), (-1, 0, 2), (-1, 3, 2)), ((1, 0, 2),)),
    (((1, 0, 2), (1, 0, 3)), ((1, 2, 3),), ((-1, 2, 2), (1, 2, 3))),
    (((1, 2, 2), (1, 0, 3)), ((1, 2, 3), (1, 3, 2)), ((1, 2, 2), (-1, 1, 3))),
    (((1, 2, 2), (1, 2, 3)), ((1, 3, 2),), ((-1, 1, 2), (1, 1, 3))),
    (((1, 0, 0), (1, 0, 2)), ((1, 2, 0),), ((1, 2, 0), (-1, 2, 2))),
    (((1, 0, 0), (1, 2, 2)), ((1, 0, 2), (1, 2, 0)), ((-1, 1, 0), (1, 2, 2))),
    (((1, 2, 0), (1, 2, 2)), ((1, 0, 2),), ((1, 1, 0), (-1, 1, 2))),
    (((1, 0, 1), (1, 0, 2)), ((1, 2, 1),), ((1, 0, 1), (-1, 0, 2))),
    (((1, 0, 1), (1, 1, 2)), ((1, 1, 2), (1, 2, 1)), ((1, 1, 1), (1, 0, 2))),
    (((1, 1, 1), (1, 1, 2)), ((1, 1, 2),), ((-1, 1, 1), (1, 1, 2))),
    (((1, 1, 1), (1, 1, 3)), ((1, 0, 3), (-1, 1, 3)), ((1, 2, 1), (-1, 2, 3))),
    (((1, 0, 0), (1, 0, 1), (1, 0, 3)), ((1, 0, 3),), ((1, 2, 1), (-1, 2, 0), (1, 2, 3))),
    (((1, 2, 0), (1, 2, 1), (1, 0, 3)), ((1, 0, 3), (1, 3, 0)),
     ((1, 2, 0), (-1, 2, 1), (-1, 1, 3))),
    (((1, 2, 0), (1, 2, 1), (1, 2, 3)), ((1, 3, 0),), ((1, 1, 1), (-1, 1, 0), (1, 1, 3))),
    (((1, 1, 3),), ((1, 0, 3), (-1, 1, 3), (1, 3, 0), (1, 3, 2), (1, 3, 3)), ((1, 1, 3),)),
    (((1, 2, 1), (1, 2, 3)), ((1, 3, 0), (1, 3, 1)), ((1, 0, 1), (-1, 0, 3))),
    (((1, 1, 3), (-1, 2, 1)), ((1, 3, 0), (1, 3, 1), (-1, 0, 3), (1, 1, 3)),
     ((1, 2, 1), (-1, 0, 3))),
    (((1, 0, 3),), ((1, 3, 0), (1, 3, 1), (-1, 0, 3), (-1, 2, 3), (1, 3, 3)), ((1, 0, 3),)),
    (((1, 1, 0), (1, 1, 1)), ((1, 0, 3), (1, 1, 0)), ((1, 2, 0), (-1, 2, 1))),
    (((1, 2, 1), (-1, 1, 0)), ((1, 0, 1), (1, 1, 0)), ((1, 0, 0), (-1, 2, 1))),
    (((1, 0, 1),), ((1, 1, 0), (1, 1, 1), (1, 1, 3), (-1, 0, 3), (-1, 2, 1)), ((1, 2, 1),)),
    (((1, 2, 0), (1, 2, 1)), ((1, 0, 1), (1, 3, 0)), ((-1, 0, 0), (1, 0, 1))),
    (((1, 2, 1),), ((1, 3, 0), (1, 3, 1), (1, 0, 1), (-1, 1, 1), (-1, 1, 2)), ((1, 1, 1),)),
    (((1, 0, 0),), ((1, 0, 0), (1, 0, 1), (-1, 2, 0)), ((1, 0, 0),)),
    (((1, 1, 0),), ((1, 0, 0), (1, 0, 2), (-1, 1, 0)), ((1, 1, 0),)),
)
_BATCHES = (0, 5, 11, 19, 24, 24)
_STRASSEN = (
    (((1, 1, 0), (1, 1, 1)), ((1, 0, 0),), ((1, 1, 0), (-1, 1, 1))),
    (((1, 1, 1),), ((1, 1, 0), (-1, 0, 0)), ((1, 2, 0),)),
    (((1, 0, 0), (1, 0, 1)), ((1, 1, 1),), ((-1, 0, 0), (1, 0, 1))),
    (((1, 0, 0),), ((1, 0, 1), (-1, 1, 1)), ((1, 2, 1),)),
    (((1, 0, 0), (1, 1, 1)), ((1, 0, 0), (1, 1, 1)), ((1, 0, 0), (1, 1, 1))),
    (((1, 2, 1),), ((1, 1, 0), (1, 1, 1)), ((1, 0, 0),)),
    (((-1, 2, 0),), ((1, 0, 0), (1, 0, 1)), ((1, 1, 1),)),
)
_ATTENTION = (
    "P24 P25 P26 P0 P1 P2 S0 S1 S2 S3 P3 P4 V0 V1 V2 V3 P5 S4 S5 S6 S7 O0 P6 P7 V4 V5 V6 V7 "
    "P8 S8 S9 S10 S11 O1 P9 P10 V8 V9 V10 V11 P11 S12 S13 S14 S15 O2 P12 P13 V12 V13 V14 V15 "
    "P14 S16 S17 S18 S19 O3 P15 P16 V16 V17 V18 V19 P17 S20 S21 S22 S23 O4 P18 P19 V20 V21 "
    "V22 V23 P20 S24 S25 S26 S27 P21 P22 V24 V25 V26 V27 P23 S28 S29 S30 S31 O5 V28 V29 V30 "
    "V31 O6 O7 O8")
_SWIGLU = (
    "F4 X F0 F1 F2 F3 W500 G18 G19 G20 G16 G17 G0 D8 D10 G1 G2 D0 G3 G4 D1 G5 G6 D2 G7 G8 D3 G9 "
    "G10 D4 G11 G12 G13 G14 D5 G15 D6 D7 D9")
_CLOSE = "M0 M2 A M1 M3 D10 D6 Z0 F4 W80 D7 D9 E"
_OPEN = (
    "F0 W98 G18 G19 Z3 N W200 G20 G16 G17 P24 P25 P26 G0 P0 P1 P2 S0 S1 S2 S3 P3 P4 V0 V1 V2 V3 "
    "P5 D8 S4 S5 S6 S7 O0 G1 P6 P7 V4 V5 V6 V7 P8 S8 S9 S10 S11 O1 F1 W98 G2 P9 P10 V8 V9 "
    "V10 V11 P11 S12 S13 S14 S15 O2 D0 P12 P13 V12 V13 V14 V15 P14 S16 S17 S18 S19 O3 G3 P15 "
    "P16 V16 V17 V18 V19 P17 S20 S21 S22 S23 O4 G4 P18 P19 V20 V21 V22 V23 P20 S24 S25 S26 "
    "S27 O5 D1 P21 P22 V24 V25 V26 V27 P23 S28 S29 S30 S31 O6 G5 V28 V29 V30 V31 G6 O7 O8 A N "
    "W200 D2 F2 G7 G8 P24 P25 P26 D3 P0 P1 P2 S0 S1 S2 S3 P3 P4 V0 V1 V2 V3 P5 G9 S4 S5 S6 S7 "
    "O0 F3 W98 G10 P6 P7 V4 V5 V6 V7 P8 S8 S9 S10 S11 O1 D4 P9 P10 V8 V9 V10 V11 P11 S12 S13 "
    "S14 S15 O2 G11 P12 P13 V12 V13 V14 V15 P14 S16 S17 S18 S19 O3 G12 P15 P16 V16 V17 V18 "
    "V19 P17 S20 S21 S22 S23 O4 T W98 G13 P18 P19 V20 V21 V22 V23 P20 S24 S25 S26 S27 "
    "O5 G14 P21 P22 V24 V25 V26 V27 P23 S28 S29 S30 S31 O6 D5 V28 V29 V30 V31 G15 O7 O8")


def _layernorm(x):
    m = jnp.mean(x, axis=-1, keepdims=True)
    d = x - m
    v = jnp.mean(d * d, axis=-1, keepdims=True)
    return d * jax.lax.rsqrt(v + _EPS)


def _silu(x):
    return x * pltpu.reciprocal(1.0 + jnp.exp2(x * -_LOG2E), approx=True)


def _dot(a, b):
    return jnp.dot(a, b, preferred_element_type=jnp.float32)


def _dot_nt(a, b):
    return jax.lax.dot_general(a, b, (((1,), (1,)), ((), ())),
                               preferred_element_type=jnp.float32)


def _load_words(ref, *index):
    return ref[index] if ref.dtype == jnp.float32 else ref.bitcast(jnp.uint32)[index]


def _load_packed(ref, *index):
    return pltpu.bitcast(_load_words(ref, *index), ref.dtype)


def _low_lanes(shape):
    return jax.lax.broadcasted_iota(jnp.int32, shape, 1) < _CHUNK


def _accumulate(total, sign, value):
    if total is None:
        return sign, value
    if total[0] == sign:
        return sign, total[1] + value
    return 1, (total[1] - value if sign < 0 else value - total[1])


def _value(total):
    return total[1] if total[0] > 0 else -total[1]


def _upper_rows_only(level):
    def upper(terms):
        return tuple((sign, 0, i) for sign, f, i in terms if f != 1)

    kept = {r: (upper(model), weight, upper(wide))
            for r, (model, weight, wide) in enumerate(level)}
    return {r: product for r, product in kept.items() if product[_MODEL] and product[_WIDE]}


def _levels(groups):
    if groups == 1:
        return [_upper_rows_only(_HOPCROFT_KERR)]
    return [dict(enumerate(_HOPCROFT_KERR))] if groups == 2 else [dict(enumerate(_STRASSEN))] * 2


def _combination(terms, side, block):
    total = None
    for sign, a, b in terms:
        if side == _WEIGHT or a < 2:
            total = _accumulate(total, sign, block(a, b))
        else:
            total = _accumulate(total, *_accumulate(
                (sign, block(0, b)), -sign if side == _MODEL else sign, block(1, b)))
    return _value(total)


def _operands(levels, side, block):
    level, *inner = levels
    if not inner:
        block = functools.cache(block)
        return {r: functools.partial(_combination, product[side], side, block)
                for r, product in level.items()}
    operands = {}
    for r, product in level.items():
        def sub_block(a, b, terms=product[side]):
            return _combination(terms, side, lambda f, i: block(2 * f + a, 2 * i + b))

        for n, operand in _operands(inner, side, sub_block).items():
            operands[r * len(inner[0]) + n] = operand
    return operands


def _collect(levels, side, multiply, start, finish, partial_ref=None):
    level, *inner = levels
    terms = [term for product in level.values() for term in product[side]]
    left = {}
    for _, f, i in terms:
        left[f, i] = left.get((f, i), 0) + 1
    for i in sorted({i for _, f, i in terms if f == 2}):
        for f in range(2):
            left[f, i] = left.get((f, i), 0) + 1
    total = {}

    def add(f, i, sign, result):
        left[f, i] -= 1
        if f == 2:
            total[f, i] = _accumulate(total.get((f, i)), sign, result)
            if not left[f, i]:
                sign, result = total[f, i]
                add(0, i, sign, result)
                add(1, i, -sign if side == _MODEL else sign, result)
            return
        for (a, b), tile in result.items() if inner else [((0, 0), result)]:
            index = (2 * f + a, 2 * i + b) if inner else (f, i)
            key = f, i, a, b
            if key not in total:
                first = start(*index)
                before = None if first is None else (1, first)
            else:
                before = (total[key][0], partial_ref[index]) if inner else total[key]
            total[key] = _accumulate(before, sign, tile)
            if not left[f, i]:
                finish(*index, _value(total[key]))
            elif inner:
                partial_ref[index] = total[key][1]

    for r, product in level.items():
        if inner:
            result = {}
            _collect(inner, side, lambda n: multiply(r * len(inner[0]) + n), lambda f, i: None,
                     lambda f, i, tile: result.update({(f, i): tile}))
        else:
            result = multiply(r)
        for sign, f, i in product[side]:
            add(f, i, sign, result)


@functools.cache
def _operand_slots(groups):
    slots = {}
    for r in _operands(_levels(groups), _MODEL, lambda f, i: 0):
        used = set()
        _operands(_levels(groups), _MODEL, lambda f, i: used.add(i) or 0)[r]()
        for tile in [None] + sorted(used):
            slots[r, tile] = len(slots)
    return slots


class _SideJobs:
    def __init__(self, zero):
        self.zero, self.jobs, self.pace, self.due, self.count = zero, [], 0.0, 0.0, -1

    def add(self, source_ref, job, key=None):
        self.jobs.append((key, source_ref, job))

    def spread(self, products):
        self.pace = len(self.jobs) / products

    def finish(self, *keys):
        while self.jobs and (not keys or any(key in keys for key, _, _ in self.jobs)):
            _, ref, job = self.jobs.pop(0)
            if ref is not None:
                job()

    def dot(self, a, b):
        result = _dot(a, b)
        self.count += 1
        self.due = self.due + self.pace if self.jobs else 0.0
        while self.jobs and self.due >= 1.0:
            self.due -= 1.0
            _, ref, job = self.jobs.pop(0)
            if ref is None:
                continue
            rows = 32 // ref.dtype.itemsize
            first = self.count % 4 * (result.shape[0] // rows) // 4 * rows
            value = result[first:first + rows]
            index = (self.zero,) * (ref.ndim - 2) + (
                slice(ref.shape[-2] - rows, None), slice(0, _LANES))
            ref[index] = (pltpu.bitcast(value, ref.dtype) if ref.dtype == jnp.uint32
                          else value.astype(ref.dtype))
            job()
        return result


def _store_rows(ref, f, first, x):
    rows = slice(first, first + x.shape[0])
    for i in range(_TILES):
        ref[f, i, rows] = x[:, i * _LANES:(i + 1) * _LANES]
    ref[f, _TILES, rows] = jnp.concatenate([x[:, _TILES * _LANES:]] * 2, axis=1)


def _combination_jobs(ref, groups, side, block, slots, n_rows):
    def job(batch, rows):
        operands = _operands(_levels(groups), side, lambda a, b: block(a, b, rows))
        for r, slot in batch:
            ref[slot, rows] = operands[r]().astype(ref.dtype)

    batches = {}
    for r, slot in slots.items():
        key = r // len(_STRASSEN) if groups == 4 else sum(r >= cut for cut in _BATCHES) % 4
        batches.setdefault(key, []).append((r, slot))
    step = _SLAB if groups > 1 else n_rows
    return [functools.partial(job, batch, slice(first, first + step))
            for batch in batches.values() for first in range(0, n_rows, step)]


def _operand_jobs(ref, rows_ref, groups, tile):
    return _combination_jobs(
        ref, groups, _MODEL, lambda f, i, rows: rows_ref[f, _TILES if i == tile else i, rows],
        {r: slot for (r, replaced), slot in _operand_slots(groups).items() if replaced == tile},
        ref.shape[1])


def _operand_loader(ref, groups, part):
    slots = _operand_slots(groups)
    rows = ref.shape[-2] * ref.dtype.itemsize // 4
    lanes = jax.lax.broadcasted_iota(jnp.int32, (rows, _LANES), 1)
    replaced = (lanes & _CHUNK) == (part & 1) * _CHUNK
    if isinstance(part, int):
        others = {r: slot for (r, tile), slot in slots.items() if tile == part // 2}
    else:
        others = {}
        for (r, tile), slot in slots.items():
            others[r] = slot if tile is None else jnp.where(part >> 1 == tile, slot, others[r])

    def load(r, *index):
        words = _load_words(ref, *index, slots[r, None])
        if r in others:
            words = jax.lax.select(replaced, _load_words(ref, *index, others[r]), words)
        return pltpu.bitcast(words, ref.dtype) if words.dtype != ref.dtype else words

    return load


def _store_packed(ref, index, value):
    ref.bitcast(jnp.uint32)[index] = pltpu.bitcast(value, jnp.uint32)


def _merge(ref, f):
    rest = ref[f, _TILES]
    return jnp.concatenate(
        [ref[f, i] for i in range(_TILES)] + [rest[:, :_CHUNK] + rest[:, _CHUNK:]], axis=1)


def _attention_masks(n_mem, seg):
    size = n_mem + seg
    shape = (2 * size, 2 * size)

    def position(axis):
        r = jax.lax.broadcasted_iota(jnp.int32, shape, axis)
        return r < size, jnp.where(r < seg, r + n_mem, jnp.where(r < size, r - seg, r - size))

    (first_i, i), (first_j, j) = position(0), position(1)
    same = first_i == first_j
    fill = jnp.where(same, _MASKED * _LOG2E, -jnp.inf).astype(jnp.float32)
    return same & ((i < n_mem) | (i >= j)), fill


def _when(condition, function):
    if not isinstance(condition, bool):
        pl.when(condition)(function)
    elif condition:
        function()


def _start(copies):
    for copy in copies:
        copy.start()


def _wait(copies):
    for copy in copies:
        copy.wait()


def _kernel(xt_hbm, mem0_hbm, wq_hbm, wk_hbm, wv_hbm, wot_hbm, w1_hbm, w3_hbm, w2t_hbm,
            outt_hbm, mem0_ref, tile_ref, x_ref, early_ref, wq_ref, wk_ref, wv_ref,
            wplain_ref, stage_ref, stage_sem, mem_sem, tile_sem, *wide_refs, seg):
    wide_refs = list(wide_refs)
    d_model, n_tok = xt_hbm.shape
    n_mem = mem0_ref.shape[0]
    _, n_heads, d_head = wq_hbm.shape
    n_seg = n_tok // seg
    n_io = n_tok // _LANES
    size = n_mem + seg
    ahead = seg // 2
    width = _TILES * _LANES
    score_scale = d_head ** -0.5 * _LOG2E
    f32, bf16, words = jnp.float32, jnp.bfloat16, jnp.uint32
    attn_tiles, ffn_tiles = len(_HOPCROFT_KERR), len(_STRASSEN) ** 2
    weight_refs = wq_ref, wk_ref, wv_ref
    behind = (_PARTS + 1) * attn_tiles
    stitched = 6

    side = _SideJobs(jax.lax.fori_loop(0, 3, lambda i, total: total - i, 3))

    def combine_weights(out_ref, groups, source_ref, block, n_rows, n_tiles):
        wide_refs.reverse()
        wide_ref = wide_refs[0]

        def widen(first, tiles):
            rows = range(first, first + n_rows)
            for j, tile in [(j, block(rows, j)) for j in tiles]:
                wide_ref[first // _LANES, j, pl.ds(first % _LANES, n_rows)] = tile

        jobs = [functools.partial(widen, first, range(j, j + n_tiles))
                for j in range(0, _TILES, n_tiles) for first in range(0, width, n_rows)]
        before = []
        while _WEAVE and side.jobs and side.jobs[-1][1] is wide_refs[1]:
            before.insert(0, side.jobs.pop())
        for n, job in enumerate(jobs):
            side.add(source_ref, job)
            for _ in range(_TURN_PAUSE if n_rows == _LANES else 0):
                side.add(None, None)
            side.jobs += before[n * len(before) // len(jobs):(n + 1) * len(before) // len(jobs)]
        for job in _combination_jobs(out_ref, groups, _WEIGHT,
                                     lambda i, j, rows: wide_ref[i, j, rows],
                                     {r: r for r in range(out_ref.shape[0])}, _LANES):
            side.add(wide_ref, job)

    def staged_rows(part, rows, packing):
        count = min(len(rows), _CHUNK)
        for first in rows[::count]:
            c, offset = divmod(first, _CHUNK)
            if isinstance(part, int):
                first = ((_PARTS if c == part else c) * _CHUNK + offset) // packing
            else:
                first = pl.multiple_of(
                    jnp.where(part == c, _PARTS, c) * (_CHUNK // packing) + offset // packing,
                    count // packing)
            yield pl.ds(first, count // packing)

    def block_copies(m, part, slot, rows=pl.ds(0, d_model // 2)):
        dst, sem = stage_ref.at[slot], stage_sem.at[slot]
        if m == 0:
            return [pltpu.make_async_copy(wot_hbm.bitcast(words).at[_TILES * part + j, rows],
                                          dst.at[rows, pl.ds(j * _LANES, _LANES)], sem)
                    for j in range(_TILES)]
        first = part * width if isinstance(part, int) else pl.multiple_of(part * width, width)
        src = (w1_hbm, w2t_hbm, w3_hbm)[m - 1].bitcast(words)
        return [pltpu.make_async_copy(src.at[rows, pl.ds(first, width)], dst.at[rows], sem)]

    def stitch_copies(m):
        return [copy for c in range(_PARTS) for copy in block_copies(
            m, c, stitched + m, pl.ds(c * _CHUNK // 2, _CHUNK // 2))]

    def staged(slot, part, rows, j):
        tile = pltpu.bitcast(jnp.concatenate(
            [stage_ref[slot, piece, j * _LANES:(j + 1) * _LANES]
             for piece in staged_rows(part, rows, 2)], axis=0), bf16)
        return (tile.T if len(rows) == _LANES else tile).astype(f32)

    def store_block(m, out_ref, unit, block):
        tiles = ffn_tiles if m else attn_tiles
        out_ref = out_ref.at[pl.ds(unit * tiles + (behind if m < 3 else 0), tiles)]
        combine_weights(out_ref, 4 if m else 2, stage_ref, block,
                        _CHUNK if m % 2 else _LANES, 1)

    def store_part(m, out_ref, part, slot):
        store_block(m, out_ref, part, lambda rows, j: (
            staged(slot, part, rows, j) - staged(stitched + m, part, rows, j)))

    def store_shared(m, out_ref):
        store_block(m, out_ref, _PARTS + 1 if m else _PARTS,
                    functools.partial(staged, stitched + m, _PARTS))

    def store_last(m, out_ref):
        slot, other, part = {1: (2, 5, 0), 2: (stitched + 4, None, _PARTS), 3: (5, 2, 1)}[m]

        def block(rows, j):
            own = staged(slot, part, rows, j)
            if m != 2 and rows[0] == (1 - part) * _CHUNK:
                return own - staged(other, part, rows, j)
            return own

        store_block(m, out_ref, _PARTS, block)
        for j in range(_TILES):
            rows = range(part * _CHUNK, (part + 1) * _CHUNK)
            wplain_ref[j + _TILES * (m == 2), pl.ds(part % 2 * _CHUNK, _CHUNK)] = staged(
                slot, _PARTS, rows, j).astype(bf16)

    def load_weights(early_in_ref, early_shared_ref, head_ref, head_sem, *rows_refs):
        n_chunks, _, rows_per_group, _ = early_in_ref.shape
        per_group = rows_per_group // ahead

        def head_copies(w, part, slot, rows=pl.ds(0, d_model)):
            src = (wq_hbm, wk_hbm, wv_hbm)[w].bitcast(words)
            return [pltpu.make_async_copy(src.at[rows, 2 * part + n, :],
                                          head_ref.at[slot, n, rows], head_sem.at[slot])
                    for n in range(2)]

        def head_stitch_copies(w):
            return [copy for c in range(_PARTS)
                    for copy in head_copies(w, c, stitched + w, pl.ds(c * _CHUNK, _CHUNK))]

        def head(slot, rows, j):
            pair = head_ref[slot, j // 2, rows, :]
            return pltpu.bitcast(pair & words(0xFFFF0000) if j % 2 else pair << 16, f32)

        def store_heads(w, part):
            def block(rows, j):
                rows = next(staged_rows(part, rows, 1))
                return head(3 * (part & 1) + w, rows, j) - head(stitched + w, rows, j)

            combine_weights(weight_refs[w].at[pl.ds(part * attn_tiles, attn_tiles)], 2,
                            head_ref, block, _CHUNK // 2, 2)

        def store_shared_heads(w):
            @pl.loop(0, _LANES // _SLAB)
            def _(n):
                def rows(i):
                    return pl.ds(pl.multiple_of(i * _LANES + n * _SLAB, _SLAB), _SLAB)

                operands = _operands(_levels(2), _WEIGHT,
                                     lambda i, j: head(stitched + w, rows(i), j))
                for r, operand in operands.items():
                    weight_refs[w][_PARTS * attn_tiles + r, rows(0)] = operand().astype(bf16)

        def x_copy(i):
            cols = pl.ds(i * _LANES, _LANES)
            return pltpu.make_async_copy(xt_hbm.at[:, cols], tile_ref.at[i, :d_model],
                                         tile_sem.at[i])

        def transpose_in(i):
            x_ref[i // 2, i % 2 * _LANES:(i % 2 + 1) * _LANES, :] = _load_packed(
                tile_ref, i, slice(0, d_model // 2)).T

        def normalize(c):
            for s in range(2 * per_group):
                block, first = divmod((_LAG + 2 * per_group * c + s) * seg, 2 * _LANES)
                _store_rows(rows_refs[c % 3], s // per_group, s % per_group * ahead,
                            _layernorm(x_ref[block, first:first + ahead, :].astype(f32)))

        def prepare(c, tiles=(None, *range(_TILES))):
            for tile in tiles:
                for n, job in enumerate(_operand_jobs(early_in_ref.at[c], rows_refs[c % 3], 2, tile)):
                    if tile is None and c + 2 >= n_chunks:
                        side.jobs.insert(2 * n, (c, rows_refs[c % 3], job))
                    else:
                        side.add(rows_refs[c % 3], job, c if tile is None else None)

        def project(w, part, c, operand):
            def keep(f, j, tile):
                early_shared_ref[w, c, f, j] = tile

            def store(f, j, tile):
                for s in range(per_group):
                    early_ref[part, (2 * c + f) * per_group + s, _TILES * w + j] = (
                        tile[s * ahead:(s + 1) * ahead].astype(bf16))

            shared = isinstance(part, int) and part == _PARTS
            unit_ref = weight_refs[w].at[pl.ds(part * attn_tiles, attn_tiles)]
            _collect(_levels(2), _WIDE,
                     lambda r: side.dot(operand(r, c), _load_packed(unit_ref, r)),
                     lambda f, j: None if shared else early_shared_ref[w, c, f, j],
                     keep if shared else store)

        def heads_of(part):
            return [copy for w in range(3) for copy in head_copies(w, part, 3 * (part & 1) + w)]

        def copies_for(part):
            return [copy for m in range(3) for copy in block_copies(m, part, 3 * (part & 1) + m)
                    ] + (heads_of(part + 1) if part + 1 < _PARTS
                         else block_copies(2, _PARTS, stitched + 4))

        def x_copies(first, last):
            return [x_copy((c + 1) % n_io) for c in range(first, last)]

        def fetch(c):
            transpose_in((c + 1) % n_io)
            if c < n_chunks:
                normalize(c)

        _start(x_copies(0, 3) + head_stitch_copies(0))
        for w in range(3):
            head_ref[stitched + w, :, width:d_model, :] = jnp.zeros((2, _CHUNK, d_head), words)
        for m in range(4):
            stage_ref[stitched + m, width // 2:d_model // 2, :] = jnp.zeros(
                (_CHUNK // 2, width), words)
        for ref in (early_in_ref, early_shared_ref):
            ref[(side.zero,) * (ref.ndim - 2)] = jnp.zeros(ref.shape[-2:], ref.dtype)
        _wait(x_copies(0, 3))
        _start(head_stitch_copies(1))
        for c in range(3):
            transpose_in(c + 1)
        operand = _operand_loader(early_in_ref, 2, _PARTS)
        following = (head_stitch_copies(2), x_copies(3, _MIDDLE),
                     x_copies(_MIDDLE, n_io) + head_copies(0, 0, 0))
        later = head_copies(1, 0, 1) + head_copies(2, 0, 2) + [
            copy for m in range(3) for copy in stitch_copies(m)]

        def project_chunks(pending, first, last):
            ready = pending + [(w, c) for c in range(first, last) for w in range(3)]
            held = [(w, c) for w, c in ready if w and c + 2 >= last and last < n_chunks]
            fetch(first)
            side.add(tile_ref, functools.partial(fetch, first + 1))
            prepare(first, [None])
            side.spread(len(pending) * attn_tiles)
            for w, c in ready:
                if w == 0:
                    side.finish(c)
                    if c + 2 < last + (last == n_chunks):
                        side.add(tile_ref, functools.partial(fetch, c + 2))
                    if c + 1 < last:
                        prepare(c + 1, [None])
                    prepare(c, range(_TILES))
                    if c + 3 == n_chunks:
                        store_heads(0, 0)
                    side.spread((3 * (n_chunks - c) - .5 if c + 3 >= n_chunks else 1
                                 if (1, c) in held else 3) * attn_tiles)
                if (w, c) not in held:
                    project(w, _PARTS, c, operand)
            side.finish()
            return held

        for w in range(3):
            _wait(head_stitch_copies(w) + (following[1] if w == 2 else []))
            _start(following[w])
            store_shared_heads(w)
            if w == 2:
                break
            for c in range(3):
                if w == 0:
                    normalize(c)
                prepare(c, range(_TILES) if w else [None])
            side.spread(2.5 * attn_tiles)
            for c in range(3):
                side.finish(c)
                project(w, _PARTS, c, operand)
            side.finish()
        held = project_chunks([(2, c) for c in range(3)], 3, _MIDDLE)
        _wait(following[2])
        _start(later + copies_for(0))
        project_chunks(held, _MIDDLE, n_chunks)
        _wait(later)

        for part in range(_PARTS - _UNROLL, _PARTS):
            if part + 1 == _PARTS:
                _start(stitch_copies(3) + block_copies(3, 0, 0) + block_copies(3, 1, 1))
            elif part:
                _start(copies_for(part + 1))
            _wait(copies_for(part))
            operand = _operand_loader(early_in_ref, 2, part)
            if part == 0:
                store_heads(1, 0)
                store_heads(2, 0)
                side.spread((n_chunks - _SLACK) * attn_tiles)
                for c in range(n_chunks):
                    project(0, 0, c, operand)
                side.finish()
                _start(copies_for(1))
            for m in range(3):
                store_part(m, weight_refs[m], part, 3 * (part & 1) + m)
                if part + 1 < _PARTS:
                    store_heads(m, part + 1)
                elif m == 1:
                    store_last(2, wv_ref)
                else:
                    store_shared(m, weight_refs[m])
            side.spread(((3 if part else 2) * n_chunks - _SLACK) * attn_tiles)
            for w in range(0 if part else 1, 3):
                for c in range(n_chunks):
                    project(w, part, c, operand)
            side.finish()

    def run_layers(wup_ref, pair_rows_ref, pair_in_ref, solo_rows_ref, solo_in_ref,
                   ffn_rows_ref, ffn_in_ref, attn_shared_ref, ffn_shared_ref, partial_ref, qkv_ref,
                   heads_ref, hidden_ref, attn_sum_ref, ffn_sum_ref, mem_ref, block_ref,
                   second_ref):
        def segment(s):
            first = (s & 7) * seg
            return s >> 3, pl.ds(first if isinstance(s, int) else pl.multiple_of(first, seg), seg)

        def transpose_out(i):
            first = (i & 1) * _LANES
            rows = pl.ds(first if isinstance(i, int) else pl.multiple_of(first, _LANES), _LANES)
            _store_packed(tile_ref, (i, slice(0, d_model // 2)), x_ref[i >> 1, rows].T)

        def contract(groups, part, tile_of, weight_ref, first, sum_ref, begun):
            operands = _operands(_levels(groups), _WIDE, tile_of)

            def targets(i):
                return [_TILES if 2 * i + half == part else i for half in range(2)]

            def start(f, i):
                low, high = (
                    sum_ref[f, n] if (n, half) in begun else None if groups < 4
                    else block_ref[f, :seg, n * _LANES:(n + 1) * _LANES]
                    for half, n in enumerate(targets(i)))
                if targets(i) == [i, i] and ((i, 0) in begun) == ((i, 1) in begun):
                    return low
                if low is None and high is None:
                    return None
                return jnp.where(_low_lanes(sum_ref.shape[-2:]), 0.0 if low is None else low,
                                 0.0 if high is None else high)

            def finish(f, i, tile):
                if targets(i) == [i, i]:
                    sum_ref[f, i] = tile
                else:
                    for half, n in enumerate(targets(i)):
                        lanes = slice(half * _CHUNK, (half + 1) * _CHUNK)
                        sum_ref[f, n, :, lanes] = tile[:, lanes]

            _collect(_levels(groups), _MODEL,
                     lambda r: side.dot(operands[r](), _load_packed(weight_ref, first + r)),
                     start, finish, partial_ref.at[part % 2])
            begun.update((n, half) for i in range(_TILES) for half, n in enumerate(targets(i)))

        def keep_and_add(ref, part, total, f, j, tile):
            ref[part, f, j] = tile
            if part < _PARTS:
                ref[total, f, j] = ref[total if part > 1 else 0, f, j] + tile if part else tile

        def attention_stage(stage, g, step):
            t, groups = step["t"], step["groups"]
            in_ref, rows_ref = (pair_in_ref, pair_rows_ref) if groups == 2 else (
                solo_in_ref, solo_rows_ref)
            rows = slice(0, in_ref.shape[1])
            if stage == "P":
                part, w = divmod(g, 3)
                side.finish(("P", None), ("P", part // 2))
                operand = _operand_loader(in_ref, groups, part)
                done = {}

                def finish(f, j, tile):
                    done[f, j] = tile
                    n = (_TILES * part + j) % qkv_ref.shape[0]
                    if part == _PARTS:
                        attn_shared_ref[w, f, j, rows] = tile
                    elif groups == 2 and (1 - f, j) in done:
                        upper, lower = done[0, j], done[1, j]
                        qkv_ref[n, w, :2 * size - ahead] = jnp.concatenate(
                            [upper[n_mem:n_mem + ahead], upper[:n_mem], lower[:n_mem],
                             upper[n_mem + ahead:], lower[n_mem:]], axis=0).astype(bf16)
                    elif groups == 1 and (0, j ^ 1) in done:
                        a, b = done[0, j & ~1], done[0, j | 1]
                        qkv_ref[n | 1, w] = jnp.concatenate(
                            [a[n_mem:], a[:n_mem], b], axis=0).astype(bf16)

                _collect(_levels(groups), _WIDE,
                         lambda r: side.dot(operand(r),
                                        _load_packed(weight_refs[w], part * attn_tiles + r)),
                         lambda f, j: attn_shared_ref[w, f, j, rows] if part < _PARTS else None,
                         finish)
            elif stage == "O":
                contract(groups, g, lambda f, j: heads_ref[g, f, j], wq_ref,
                         behind + g * attn_tiles, attn_sum_ref,
                         step["begun"])
            elif groups == 2 or g % 2:
                part, j = divmod(g, _TILES)

                def projected(w):
                    if groups == 1:
                        return _load_packed(qkv_ref, g % qkv_ref.shape[0], w)
                    return pltpu.bitcast(jnp.concatenate(
                        [_load_words(early_ref, part, t - _LAG, _TILES * w + j),
                         _load_words(qkv_ref, g % qkv_ref.shape[0], w, slice(0, size - ahead // 2))], axis=0), bf16)

                if stage == "S":
                    visible, fill = step["masks"]
                    s = jnp.where(visible, _dot_nt(projected(0), projected(1)) * score_scale, fill)
                    p = jnp.exp2(s - jnp.max(s, axis=-1, keepdims=True))
                    inv = pltpu.reciprocal(jnp.sum(p, axis=-1, keepdims=True), approx=True)
                    step[g] = p.astype(bf16), inv
                else:
                    p, inv = step[g]
                    o = _dot(p, projected(2)) * inv
                    halves = jnp.concatenate([o[seg:size], o[:seg]], axis=0), o[size:]
                    for f, half in enumerate(halves):
                        index = (f, j) if groups == 2 else (0, j - 1 + f)
                        keep_and_add(heads_ref, part, _PARTS, *index, half)

        def swiglu_stage(stage, g, state):
            plain = 2 * _PARTS + 2
            if stage == "G" and g == plain:
                x = jnp.concatenate([ffn_rows_ref[f, 0, :seg] for f in range(4)], axis=0).astype(bf16)
                for j in range(_TILES):
                    tile = _dot(x, _load_packed(wplain_ref, j))
                    for f in range(4):
                        ffn_shared_ref[2, f, j] = tile[f * seg:(f + 1) * seg]
            elif stage == "G":
                part, up = divmod(g, 2) if g < plain else (None, g - plain - 1)
                chunk = _PARTS if part is None else part if part < _PARTS else up
                side.finish(("G", None), ("G", chunk // 2))
                operand = _operand_loader(ffn_in_ref, 4, chunk)
                first = (_PARTS + 1 if part is None else part) * ffn_tiles + (0 if up else behind)

                def finish(f, j, tile):
                    if part is None:
                        ffn_shared_ref[up, f, j] = tile
                    elif up:
                        keep_and_add(hidden_ref, part, _PARTS + 1, f, j,
                                     hidden_ref[part, f, j] * tile)
                    else:
                        hidden_ref[part, f, j] = _silu(tile)

                _collect(_levels(4), _WIDE,
                         lambda r: side.dot(operand(r), _load_packed(wup_ref if up else wk_ref, first + r)),
                         lambda f, j: None if part is None else ffn_shared_ref[
                             up if part < _PARTS else 2, f, j],
                         finish, partial_ref.at[g % 2])
            elif g == _PARTS + 2:
                tile = _value(functools.reduce(
                    lambda total, j: _accumulate(total, 1, _dot_nt(
                        _load_packed(wplain_ref, _TILES + j, slice(0, _CHUNK // 2)),
                        jnp.concatenate([hidden_ref[_PARTS, f, j] for f in range(4)],
                                        axis=0).astype(bf16))), range(_TILES), None)).T
                for f in range(4):
                    ffn_sum_ref[f, _TILES, :, :_CHUNK] += tile[f * seg:(f + 1) * seg]
            else:
                for f in range(0 if state["begun"] else 4):
                    rest = block_ref[f, :seg, width:]
                    ffn_sum_ref[f, _TILES] = jnp.concatenate([rest, jnp.zeros_like(rest)], axis=1)
                state["begun"].update([(_TILES, 0), (_TILES, 1)])
                contract(4, g, lambda f, j: hidden_ref[g, f, j], wv_ref, behind + g * ffn_tiles, ffn_sum_ref,
                         state["begun"])

        def run(order, t, layers, *, resumed=False, queue=lambda: None):
            state = dict(stored=set(), begun={(n, half) for n in range(_TILES + 1) for half in range(2) if resumed})
            step = None
            masks = _attention_masks(n_mem, seg)
            place = 0 if layers == (0, 1) else t
            for name in order.split():
                stage, g = name[0], int(name[1:] or 0)
                if stage == "N":
                    begin_step(t, place, layers)
                    step = dict(t=t, groups=len(layers), begun=set(), masks=masks)
                    t, place = t + 1, place + 1
                elif stage == "A":
                    close_step(t - 1, place - 1, layers)
                elif stage == "M":
                    if len(layers) == 2:
                        normalize(g)
                elif stage == "F":
                    tile = g if g < _TILES else None
                    for job in _operand_jobs(ffn_in_ref, ffn_rows_ref, 4, tile):
                        side.add(ffn_rows_ref, job, ("G", tile))
                elif stage == "J":
                    queue()
                elif stage == "W":
                    side.spread(g)
                elif stage == "Z":
                    for _ in range(g):
                        side.add(None, None)
                elif stage == "X":
                    side.finish()
                elif stage == "E":
                    done = [_merge(ffn_sum_ref, f) for f in range(4)]
                    first = jnp.maximum(t - 2 * _LAG, 0)
                    for s in range(2):
                        second_ref[s, :seg] = done[s]
                        x_ref[segment(first + s)] = done[2 + s].astype(bf16)
                elif stage == "T":
                    side.add(x_ref, functools.partial(
                        transpose_out, jnp.maximum(t - 11, 0) >> 2))
                elif stage in "GD":
                    swiglu_stage(stage, g, state)
                else:
                    attention_stage(stage, g, step)
            side.finish()

        def layer_input(t, place, layer):
            return x_ref[segment(t)].astype(f32) if layer == 0 else second_ref[place & 1, :seg]

        def begin_step(t, place, layers):
            h = _layernorm(layer_input(t, place, layers[-1]))
            if len(layers) == 1:
                rows_ref, in_ref = solo_rows_ref, solo_in_ref
                _store_rows(rows_ref, 0, n_mem, h)
            else:
                rows_ref, in_ref, cut = pair_rows_ref, pair_in_ref, ahead // 2
                _store_rows(rows_ref, 0, n_mem, _layernorm(layer_input(t, place, 0)[ahead:]))
                _store_rows(rows_ref, 0, seg - cut, h[:cut])
                _store_rows(rows_ref, 1, n_mem, h[cut:])
            for f, layer in enumerate(layers):
                _store_rows(rows_ref, f, 0, mem_ref[layer])
            for tile in [None, *range(_TILES)]:
                for job in _operand_jobs(in_ref, rows_ref, len(layers), tile):
                    side.add(rows_ref, job, ("P", tile))

        def close_step(t, place, layers):
            for f, layer in enumerate(layers):
                out = _merge(attn_sum_ref, f)
                mem_ref[layer] = out[:n_mem]
                index = 2 * layer + (place & 1) if len(layers) == 2 else place & 3
                block_ref[index, :seg] = layer_input(t, place, layer) + out[n_mem:]

        def normalize(f):
            _store_rows(ffn_rows_ref, f, 0, _layernorm(block_ref[f, :seg]))

        def solo_swiglu(queue=lambda: None):
            for f in range(4):
                normalize(f)
            run(_SWIGLU, None, None, queue=queue)

        for ref in (pair_in_ref, solo_rows_ref, solo_in_ref, ffn_in_ref, attn_shared_ref,
                    ffn_shared_ref, partial_ref, qkv_ref, heads_ref, hidden_ref, attn_sum_ref,
                    ffn_sum_ref):
            ref[(side.zero,) * (ref.ndim - 2)] = jnp.zeros(ref.shape[-2:], ref.dtype)

        mem_copy.wait()
        mem_ref[0] = mem0_ref[...].astype(f32)
        last_copies = (stitch_copies(3), block_copies(3, _PARTS, 5), block_copies(1, _PARTS, 2), [])
        last_units = (functools.partial(store_shared, 1, wk_ref),
                      functools.partial(store_shared, 3, wup_ref),
                      functools.partial(store_last, 1, wk_ref),
                      functools.partial(store_last, 3, wup_ref))

        def copies_for(t):
            return last_copies[t] + [copy for n in range(2)
                                     for copy in block_copies(3, 2 * t + n, 3 * (t & 1) + n)]

        def queue(t):
            _start(copies_for(t + 1) if t + 1 < _LAG else [mem_copy])
            _wait(copies_for(t))
            last_units[t]()
            for n in range(2):
                store_part(3, wup_ref, 2 * t + n, 3 * (t & 1) + n)

        for t in range(_LAG):
            run("N J W540 " + _ATTENTION + " A", t, (0,), queue=functools.partial(queue, t))
        mem_copy.wait()
        mem_ref[1] = mem0_ref[...].astype(f32)
        solo_swiglu()
        for s in range(2):
            second_ref[s, :seg] = _merge(ffn_sum_ref, s)
            ffn_sum_ref[s] = ffn_sum_ref[2 + s]
        run("N W200 " + _ATTENTION + " A N W200 " + _ATTENTION, _LAG, (0, 1))
        for name in _CLOSE.split():
            if name[0] == "D":
                hidden_ref[int(name[1:]) if name != "D10" else _PARTS] = jnp.zeros(hidden_ref.shape[1:], f32)

        @pl.loop(_LAG // 2 + 1, n_seg // 2)
        def _steps(b):
            run(_CLOSE, 2 * b, (0, 1), resumed=True)
            run(_OPEN, 2 * b, (0, 1))

        out_copies = [
            pltpu.make_async_copy(tile_ref.at[i, :d_model], outt_hbm.at[:, pl.ds(i * _LANES, _LANES)],
                                  tile_sem.at[i]) for i in range(n_io)]
        _start(out_copies[:n_io - 3])
        run(_CLOSE, n_seg, (0, 1), resumed=True)
        run(_OPEN, n_seg, (1,))
        run(_CLOSE, n_seg + 2, (1,), resumed=True)
        transpose_out(n_io - 2)
        _start(out_copies[n_io - 3:n_io - 1])
        pl.loop(n_seg + 2, n_seg + _LAG)(lambda t: run("N W200 " + _ATTENTION + " A", t, (1,)))
        solo_swiglu()
        for s in range(_LAG):
            x_ref[segment(n_seg - _LAG + s)] = _merge(ffn_sum_ref, s).astype(bf16)
        transpose_out(n_io - 1)
        out_copies[n_io - 1].start()
        _wait(out_copies)

    mem_copy = pltpu.make_async_copy(mem0_hbm, mem0_ref, mem_sem)
    mem_copy.start()
    n_chunks = (n_seg - _LAG) * ahead // (2 * _EARLY_ROWS)
    pl.run_scoped(
        load_weights,
        pltpu.VMEM((n_chunks, len(_operand_slots(2)), _EARLY_ROWS, _LANES), bf16),
        pltpu.VMEM((3, n_chunks, 2, _TILES, _EARLY_ROWS, _LANES), f32),
        pltpu.VMEM((stitched + 3, 2, d_model + 8, d_head), words),
        pltpu.SemaphoreType.DMA((stitched + 3,)),
        *[pltpu.VMEM((2, _TILES + 1, _EARLY_ROWS + 8, _LANES), f32)] * 3)
    pl.run_scoped(
        run_layers,
        pltpu.VMEM(((_PARTS + 2) * ffn_tiles, _LANES, _LANES), bf16),
        pltpu.VMEM((2, _TILES + 1, seg + 8, _LANES), f32),
        pltpu.VMEM((len(_operand_slots(2)), seg, _LANES), bf16),
        pltpu.VMEM((1, _TILES + 1, size + 8, _LANES), f32),
        pltpu.VMEM((len(_operand_slots(1)), size, _LANES), f32),
        pltpu.VMEM((4, _TILES + 1, seg + 8, _LANES), f32),
        pltpu.VMEM((len(_operand_slots(4)), seg, _LANES), bf16),
        pltpu.VMEM((3, 2, _TILES, size, _LANES), f32),
        pltpu.VMEM((3, 4, _TILES, seg, _LANES), f32),
        pltpu.VMEM((2, 4, _TILES, seg, _LANES), f32),
        pltpu.VMEM((12, 3, 2 * size, _LANES), bf16),
        pltpu.VMEM((_PARTS + 1, 2, _TILES, size, _LANES), f32),
        pltpu.VMEM((_PARTS + 2, 4, _TILES, seg, _LANES), f32),
        pltpu.VMEM((2, _TILES + 1, size, _LANES), f32),
        pltpu.VMEM((4, _TILES + 1, seg, _LANES), f32),
        pltpu.VMEM((2, n_mem, d_model), f32),
        pltpu.VMEM((4, seg + 8, d_model), f32),
        pltpu.VMEM((2, seg + 8, d_model), f32))


@functools.partial(jax.jit, static_argnames=("A_seg_len",))
def pallas_interleave_layers__memory_aug_recurrent_mem_tr__glu_gated_swiglu__prompt_kernel(
    A_x: jax.Array,
    A_mem0: jax.Array,
    A_Wq: jax.Array,
    A_Wk: jax.Array,
    A_Wv: jax.Array,
    A_Wo: jax.Array,
    A_seg_len: int,
    B_x: jax.Array,
    B_w1: jax.Array,
    B_w3: jax.Array,
    B_w2: jax.Array,
):
    del B_x
    _, n_tok, d_model = A_x.shape
    n_mem = A_mem0.shape[1]
    _, n_heads, d_head = A_Wq.shape
    seg = A_seg_len
    assert A_x.shape[0] == 1 and _LAG * seg == d_head == _LANES and 4 * n_mem == seg
    assert n_heads == _PARTS * _TILES and d_model == (_PARTS + 1) * _CHUNK
    assert B_w1.shape[1] == (_PARTS + 1) * _TILES * _LANES
    bf16 = jnp.bfloat16
    attn_tiles = (_PARTS + 1) * len(_HOPCROFT_KERR)
    ffn_tiles = (_PARTS + 2) * len(_STRASSEN) ** 2
    hbm = pl.BlockSpec(memory_space=pltpu.HBM)
    out_t = pl.pallas_call(
        functools.partial(_kernel, seg=seg),
        out_shape=jax.ShapeDtypeStruct((d_model, n_tok), A_x.dtype),
        in_specs=[hbm] * 9,
        out_specs=hbm,
        scratch_shapes=[
            pltpu.VMEM((n_mem, d_model), bf16),
            pltpu.VMEM((n_tok // _LANES, d_model + 16, _LANES), bf16),
            pltpu.VMEM((n_tok // (2 * _LANES), 2 * _LANES + 16, d_model), bf16),
            pltpu.VMEM((_PARTS, n_tok // seg - _LAG, 3 * _TILES, seg // 2, _LANES), bf16),
            pltpu.VMEM((2 * attn_tiles, _LANES, _LANES), bf16),
            pltpu.VMEM((attn_tiles + ffn_tiles, _LANES, _LANES), bf16),
            pltpu.VMEM((attn_tiles + ffn_tiles, _LANES, _LANES), bf16),
            pltpu.VMEM((2 * _TILES, _LANES, _LANES), bf16),
            pltpu.VMEM((11, d_model // 2 + 8, _TILES * _LANES), jnp.uint32),
            pltpu.SemaphoreType.DMA((11,)),
            pltpu.SemaphoreType.DMA(()),
            pltpu.SemaphoreType.DMA((n_tok // _LANES,)),
            *[pltpu.VMEM((_TILES, _TILES, _LANES + 8, _LANES), jnp.float32)] * 2,
        ],
        compiler_params=pltpu.CompilerParams(
            vmem_limit_bytes=127 * 1024 * 1024, disable_bounds_checks=True,
            flags={"XLA_TPU_FORCE_LP_LLO_SCHEDULER": True}),
    )(A_x.reshape(n_tok, d_model).T, A_mem0.reshape(n_mem, d_model), A_Wq, A_Wk, A_Wv,
      A_Wo.transpose(0, 2, 1), B_w1, B_w3, B_w2.T)
    return out_t.T.reshape(A_x.shape)
```

```python
import functools
import math

import jax
import jax.numpy as jnp
import jax.experimental.pallas as pl
import jax.experimental.pallas.tpu as pltpu

_EPS = 1e-05
_MASKED = -1000000000.0
_LOG2E = math.log2(math.e)
_LANES = 128
_CHUNK = _LANES // 2
_SLAB = 16
_TILES = 4
_PARTS = 2 * _TILES
_LAG = 4
_WO, _W1, _W2, _W3 = range(4)
_MODEL, _WEIGHT, _WIDE = range(3)
_HOPCROFT_KERR = (
    (((1, 1, 2),), ((1, 2, 0), (1, 2, 2), (1, 2, 3), (-1, 1, 2)), ((1, 2, 2),)),
    (((1, 2, 2),), ((1, 2, 1), (1, 2, 2), (-1, 0, 2), (-1, 3, 2)), ((1, 0, 2),)),
    (((1, 0, 2), (1, 0, 3)), ((1, 2, 3),), ((-1, 2, 2), (1, 2, 3))),
    (((1, 2, 2), (1, 0, 3)), ((1, 2, 3), (1, 3, 2)), ((1, 2, 2), (-1, 1, 3))),
    (((1, 2, 2), (1, 2, 3)), ((1, 3, 2),), ((-1, 1, 2), (1, 1, 3))),
    (((1, 0, 0), (1, 0, 2)), ((1, 2, 0),), ((1, 2, 0), (-1, 2, 2))),
    (((1, 0, 0), (1, 2, 2)), ((1, 0, 2), (1, 2, 0)), ((-1, 1, 0), (1, 2, 2))),
    (((1, 2, 0), (1, 2, 2)), ((1, 0, 2),), ((1, 1, 0), (-1, 1, 2))),
    (((1, 0, 1), (1, 0, 2)), ((1, 2, 1),), ((1, 0, 1), (-1, 0, 2))),
    (((1, 0, 1), (1, 1, 2)), ((1, 1, 2), (1, 2, 1)), ((1, 1, 1), (1, 0, 2))),
    (((1, 1, 1), (1, 1, 2)), ((1, 1, 2),), ((-1, 1, 1), (1, 1, 2))),
    (((1, 1, 1), (1, 1, 3)), ((1, 0, 3), (-1, 1, 3)), ((1, 2, 1), (-1, 2, 3))),
    (((1, 0, 0), (1, 0, 1), (1, 0, 3)), ((1, 0, 3),), ((1, 2, 1), (-1, 2, 0), (1, 2, 3))),
    (((1, 2, 0), (1, 2, 1), (1, 0, 3)), ((1, 0, 3), (1, 3, 0)),
     ((1, 2, 0), (-1, 2, 1), (-1, 1, 3))),
    (((1, 2, 0), (1, 2, 1), (1, 2, 3)), ((1, 3, 0),), ((1, 1, 1), (-1, 1, 0), (1, 1, 3))),
    (((1, 1, 3),), ((1, 0, 3), (-1, 1, 3), (1, 3, 0), (1, 3, 2), (1, 3, 3)), ((1, 1, 3),)),
    (((1, 2, 1), (1, 2, 3)), ((1, 3, 0), (1, 3, 1)), ((1, 0, 1), (-1, 0, 3))),
    (((1, 1, 3), (-1, 2, 1)), ((1, 3, 0), (1, 3, 1), (-1, 0, 3), (1, 1, 3)),
     ((1, 2, 1), (-1, 0, 3))),
    (((1, 0, 3),), ((1, 3, 0), (1, 3, 1), (-1, 0, 3), (-1, 2, 3), (1, 3, 3)), ((1, 0, 3),)),
    (((1, 1, 0), (1, 1, 1)), ((1, 0, 3), (1, 1, 0)), ((1, 2, 0), (-1, 2, 1))),
    (((1, 2, 1), (-1, 1, 0)), ((1, 0, 1), (1, 1, 0)), ((1, 0, 0), (-1, 2, 1))),
    (((1, 0, 1),), ((1, 1, 0), (1, 1, 1), (1, 1, 3), (-1, 0, 3), (-1, 2, 1)), ((1, 2, 1),)),
    (((1, 2, 0), (1, 2, 1)), ((1, 0, 1), (1, 3, 0)), ((-1, 0, 0), (1, 0, 1))),
    (((1, 2, 1),), ((1, 3, 0), (1, 3, 1), (1, 0, 1), (-1, 1, 1), (-1, 1, 2)), ((1, 1, 1),)),
    (((1, 0, 0),), ((1, 0, 0), (1, 0, 1), (-1, 2, 0)), ((1, 0, 0),)),
    (((1, 1, 0),), ((1, 0, 0), (1, 0, 2), (-1, 1, 0)), ((1, 1, 0),)),
)
_RUNS = (5, 11, 19, 24, 24)
_STRASSEN = (
    (((-1, 2, 0),), ((1, 0, 0), (1, 0, 1)), ((1, 1, 1),)),
    (((1, 1, 0), (1, 1, 1)), ((1, 0, 0),), ((1, 1, 0), (-1, 1, 1))),
    (((1, 1, 1),), ((1, 1, 0), (-1, 0, 0)), ((1, 2, 0),)),
    (((1, 0, 0), (1, 1, 1)), ((1, 0, 0), (1, 1, 1)), ((1, 0, 0), (1, 1, 1))),
    (((1, 0, 0),), ((1, 0, 1), (-1, 1, 1)), ((1, 2, 1),)),
    (((1, 0, 0), (1, 0, 1)), ((1, 1, 1),), ((-1, 0, 0), (1, 0, 1))),
    (((1, 2, 1),), ((1, 1, 0), (1, 1, 1)), ((1, 0, 0),)),
)
_ATTENTION = (
    "P24 P25 P26 P0 P1 P2 S0 S1 S2 S3 P3 P4 V0 V1 V2 V3 P5 S4 S5 S6 S7 O0 P6 P7 V4 V5 V6 V7 "
    "P8 S8 S9 S10 S11 O1 P9 P10 V8 V9 V10 V11 P11 S12 S13 S14 S15 O2 P12 P13 V12 V13 V14 V15 "
    "P14 S16 S17 S18 S19 O3 P15 P16 V16 V17 V18 V19 P17 S20 S21 S22 S23 O4 P18 P19 V20 V21 "
    "V22 V23 P20 S24 S25 S26 S27 P21 P22 V24 V25 V26 V27 P23 S28 S29 S30 S31 O5 V28 V29 V30 "
    "V31 O6 O7 O8 A")
_SWIGLU = (
    "M0 M1 M2 M3 F4 X F0 F1 F2 F3 W500 G18 G19 G20 G16 G17 G0 D8 D10 G1 G2 D0 G3 G4 D1 G5 G6 "
    "D2 G7 G8 D3 G9 G10 D4 G11 G12 G13 G14 D5 G15 D6 D7 D9")
_TWO_STEPS = (
    "F0 W98 G18 G19 Z3 N W200 G20 G16 G17 P24 P25 P26 G0 P0 P1 P2 S0 S1 S2 S3 P3 P4 V0 V1 V2 "
    "V3 P5 D8 S4 S5 S6 S7 O0 G1 P6 P7 V4 V5 V6 V7 P8 S8 S9 S10 S11 O1 F1 W98 G2 P9 P10 V8 V9 "
    "V10 V11 P11 S12 S13 S14 S15 O2 D0 P12 P13 V12 V13 V14 V15 P14 S16 S17 S18 S19 O3 G3 P15 "
    "P16 V16 V17 V18 V19 P17 S20 S21 S22 S23 O4 G4 P18 P19 V20 V21 V22 V23 P20 S24 S25 S26 "
    "S27 O5 D1 P21 P22 V24 V25 V26 V27 P23 S28 S29 S30 S31 O6 G5 V28 V29 V30 V31 G6 O7 O8 A N "
    "W200 D2 F2 G7 G8 P24 P25 P26 D3 P0 P1 P2 S0 S1 S2 S3 P3 P4 V0 V1 V2 V3 P5 G9 S4 S5 S6 S7 "
    "O0 F3 W98 G10 P6 P7 V4 V5 V6 V7 P8 S8 S9 S10 S11 O1 D4 P9 P10 V8 V9 V10 V11 P11 S12 S13 "
    "S14 S15 O2 G11 P12 P13 V12 V13 V14 V15 P14 S16 S17 S18 S19 O3 G12 P15 P16 V16 V17 V18 "
    "V19 P17 S20 S21 S22 S23 O4 T W98 G13 P18 P19 V20 V21 V22 V23 P20 S24 S25 S26 S27 O5 G14 "
    "P21 P22 V24 V25 V26 V27 P23 S28 S29 S30 S31 O6 D5 V28 V29 V30 V31 G15 O7 O8 M0 M2 A M1 "
    "M3 D10 D6 Z0 F4 W80 D7 D9 E")


def _layernorm(x):
    m = jnp.mean(x, axis=-1, keepdims=True)
    d = x - m
    v = jnp.mean(d * d, axis=-1, keepdims=True)
    return d * jax.lax.rsqrt(v + _EPS)


def _silu(x):
    return x * pltpu.reciprocal(1.0 + jnp.exp2(x * -_LOG2E), approx=True)


def _dot(a, b, axis=0):
    return jax.lax.dot_general(a, b, (((1,), (axis,)), ((), ())),
                               preferred_element_type=jnp.float32)


def _load_words(ref, *index):
    return ref[index] if ref.dtype == jnp.float32 else ref.bitcast(jnp.uint32)[index]


def _load_packed(ref, *index):
    return pltpu.bitcast(_load_words(ref, *index), ref.dtype)


def _aligned(first, size):
    return pl.ds(first if isinstance(first, int) else pl.multiple_of(first, size), size)


def _accumulate(total, sign, value):
    if total is None:
        return sign, value
    if total[0] == sign:
        return sign, jax.lax.add(total[1], value)
    return 1, jax.lax.sub(*((total[1], value) if sign < 0 else (value, total[1])))


def _value(total):
    return total[1] if total[0] > 0 else -total[1]


def _levels(groups):
    if groups == 4:
        return [dict(enumerate(_STRASSEN))] * 2
    if groups == 2:
        return [dict(enumerate(_HOPCROFT_KERR))]

    def upper(terms):
        return tuple((sign, 0, i) for sign, f, i in terms if f != 1)

    return [{r: (upper(model), weight, upper(wide))
             for r, (model, weight, wide) in enumerate(_HOPCROFT_KERR)
             if upper(model) and upper(wide)}]


def _combination(terms, side, block):
    total = None
    for sign, a, b in terms:
        if side == _WEIGHT or a < 2:
            total = _accumulate(total, sign, block(a, b))
        else:
            total = _accumulate(total, *_accumulate(
                (sign, block(0, b)), -sign if side == _MODEL else sign, block(1, b)))
    return _value(total)


def _operands(levels, side, block):
    level, *inner = levels
    if not inner:
        block = functools.cache(block)
        return {r: functools.partial(_combination, product[side], side, block)
                for r, product in level.items()}
    operands = {}
    for r, product in level.items():
        def sub_block(a, b, terms=product[side]):
            return _combination(terms, side, lambda f, i: block(2 * f + a, 2 * i + b))

        for n, operand in _operands(inner, side, sub_block).items():
            operands[r * len(inner[0]) + n] = operand
    return operands


def _collect(levels, side, multiply, start, finish, partial_ref=None):
    level, *inner = levels
    terms = [term for product in level.values() for term in product[side]]
    left = {}
    for _, f, i in terms:
        left[f, i] = left.get((f, i), 0) + 1
    for i in sorted({i for _, f, i in terms if f == 2}):
        for f in range(2):
            left[f, i] = left.get((f, i), 0) + 1
    total = {}

    def add(r, f, i, sign, result):
        left[f, i] -= 1
        if f == 2:
            total[f, i] = _accumulate(total.get((f, i)), sign, result)
            if not left[f, i]:
                sign, result = total[f, i]
                add(r, 0, i, sign, result)
                add(r, 1, i, -sign if side == _MODEL else sign, result)
            return
        for (a, b), tile in result.items() if inner else [((0, 0), result)]:
            index = (2 * f + a, 2 * i + b) if inner else (f, i)
            key = f, i, a, b
            if key not in total:
                first = start(*index)
                before = None if first is None else (1, first)
            elif total[key][1] is None:
                before = total[key][0], partial_ref[index]
            else:
                before = total[key]
            total[key] = _accumulate(before, sign, tile)
            if not left[f, i]:
                finish(*index, _value(total[key]))
            elif inner and not any(g in (f, 2) and j == i for _, g, j in level[r + 1][side]):
                partial_ref[index] = total[key][1]
                total[key] = total[key][0], None

    for r, product in level.items():
        if inner:
            result = {}
            _collect(inner, side, lambda n: multiply(r * len(inner[0]) + n), lambda f, i: None,
                     lambda f, i, tile: result.update({(f, i): tile}))
        else:
            result = multiply(r)
        for sign, f, i in product[side]:
            add(r, f, i, sign, result)


@functools.cache
def _operand_slots(groups):
    used = {0: [0]}
    for level in _levels(groups):
        used = {r * len(level) + n: sorted({2 * i + j for i in tiles for _, _, j in terms})
                for r, tiles in used.items() for n, (terms, _, _) in level.items()}
    keys = [(r, tile) for r, tiles in used.items() for tile in [None] + tiles]
    return {key: slot for slot, key in enumerate(keys)}


class _SideJobs:
    def __init__(self, zero):
        self.zero, self.jobs, self.pace, self.due, self.count = zero, [], 0.0, 0.0, -1

    def add(self, source_ref=None, job=None, key=None):
        self.jobs.append((key, source_ref, job))

    def spread(self, products):
        self.pace = len(self.jobs) / products

    def finish(self, *keys):
        while self.jobs and (not keys or any(key in keys for key, _, _ in self.jobs)):
            _, ref, job = self.jobs.pop(0)
            if ref is not None:
                job()

    def dot(self, a, b):
        result = _dot(a, b)
        self.count += 1
        self.due = self.due + self.pace if self.jobs else 0.0
        while self.jobs and self.due >= 1.0:
            self.due -= 1.0
            _, ref, job = self.jobs.pop(0)
            if ref is None:
                continue
            rows = 32 // ref.dtype.itemsize
            first = self.count % 4 * (result.shape[0] // rows) // 4 * rows
            value = jax.lax.slice_in_dim(result, first, first + rows)
            index = (self.zero,) * (ref.ndim - 2) + (
                slice(ref.shape[-2] - rows, None), slice(0, _LANES))
            ref[index] = (pltpu.bitcast(value, ref.dtype) if ref.dtype == jnp.uint32
                          else value.astype(ref.dtype))
            job()
        return result

    def keep_in_memory(self, *refs):
        for ref in refs:
            ref[(self.zero,) * (ref.ndim - 2)] = jnp.zeros(ref.shape[-2:], ref.dtype)


def _store_rows(ref, f, first, x):
    rows = slice(first, first + x.shape[0])
    for i in range(_TILES):
        ref[f, i, rows] = x[:, i * _LANES:(i + 1) * _LANES]
    ref[f, _TILES, rows] = jnp.concatenate([x[:, _TILES * _LANES:]] * 2, axis=1)


def _load_rows(ref, f):
    rest = ref[f, _TILES]
    return jnp.concatenate(
        [ref[f, i] for i in range(_TILES)] + [rest[:, :_CHUNK] + rest[:, _CHUNK:]], axis=1)


def _combination_jobs(ref, groups, side, block, slots):
    def job(batch, rows):
        operands = _operands(_levels(groups), side, lambda a, b: block(a, b, rows))
        for r, slot in batch:
            ref[slot, rows] = jax.lax.convert_element_type(operands[r](), ref.dtype)

    batches = {}
    for r, slot in slots.items():
        key = r // len(_STRASSEN) if groups == 4 else sum(r >= cut for cut in _RUNS) % 4
        batches.setdefault(key, []).append((r, slot))
    step = _SLAB if groups > 1 else ref.shape[1]
    return [functools.partial(job, batch, slice(first, first + step))
            for batch in batches.values() for first in range(0, ref.shape[1], step)]


def _operand_jobs(ref, rows_ref, tile):
    groups = rows_ref.shape[0]
    return _combination_jobs(
        ref, groups, _MODEL, lambda f, i, rows: rows_ref[f, _TILES if i == tile else i, rows],
        {r: slot for (r, replaced), slot in _operand_slots(groups).items() if replaced == tile})


def _operand_loader(ref, groups, part):
    slots = _operand_slots(groups)
    rows = ref.shape[-2] * ref.dtype.itemsize // 4
    lanes = jax.lax.broadcasted_iota(jnp.int32, (rows, _LANES), 1)
    replaced = (lanes & _CHUNK) == (part & 1) * _CHUNK
    if isinstance(part, int):
        others = {r: slot for (r, tile), slot in slots.items() if tile == part // 2}
    else:
        others = {}
        for (r, tile), slot in slots.items():
            others[r] = slot if tile is None else jnp.where(part >> 1 == tile, slot, others[r])

    def load(r, *index):
        words = _load_words(ref, *index, slots[r, None])
        if r in others:
            words = jax.lax.select(replaced, _load_words(ref, *index, others[r]), words)
        return pltpu.bitcast(words, ref.dtype) if words.dtype != ref.dtype else words

    return load


def _attention_masks(n_mem, seg):
    size = n_mem + seg
    shape = (2 * size, 2 * size)

    def position(axis):
        r = jax.lax.broadcasted_iota(jnp.int32, shape, axis)
        return r < size, jnp.where(r < seg, r + n_mem, jnp.where(r < size, r - seg, r - size))

    (first_i, i), (first_j, j) = position(0), position(1)
    same = first_i == first_j
    fill = jnp.where(same, _MASKED * _LOG2E, -jnp.inf).astype(jnp.float32)
    return same & ((i < n_mem) | (i >= j)), fill


def _start(copies):
    for copy in copies:
        copy.start()


def _wait(copies):
    for copy in copies:
        copy.wait()


def _kernel(xt_hbm, mem0_hbm, wq_hbm, wk_hbm, wv_hbm, wot_hbm, w1_hbm, w2t_hbm, w3_hbm,
            outt_hbm, mem0_ref, tile_ref, x_ref, early_ref, wqkv_ref, wo_ref, w1_ref, w2_ref,
            wplain_ref, stage_ref, stage_sem, mem_sem, tile_sem, *wide_refs, seg):
    d_model, n_tok = xt_hbm.shape
    n_mem = mem0_ref.shape[0]
    d_head = wq_hbm.shape[2]
    n_seg = n_tok // seg
    n_io = n_tok // _LANES
    size = n_mem + seg
    ahead = seg // 2
    width = _TILES * _LANES
    score_scale = d_head ** -0.5 * _LOG2E
    f32, bf16, words = jnp.float32, jnp.bfloat16, jnp.uint32
    shared_slot = 6
    last_slots = {_W1: 2, _W2: shared_slot + 4, _W3: 5}
    wide_refs = list(wide_refs)
    side = _SideJobs(jax.lax.fori_loop(0, 3, lambda i, total: total - i, 3))

    def combine_weights(out_ref, source_ref, block, n_rows, n_tiles):
        wide_refs.reverse()
        wide_ref = wide_refs[0]

        def widen(first, tiles):
            rows = range(first, first + n_rows)
            for j, tile in [(j, block(rows, j)) for j in tiles]:
                wide_ref[first // _LANES, j, pl.ds(first % _LANES, n_rows)] = tile

        jobs = [functools.partial(widen, first, range(j, j + n_tiles))
                for j in range(0, _TILES, n_tiles) for first in range(0, width, n_rows)]
        before = []
        while side.jobs and side.jobs[-1][1] is wide_refs[1]:
            before.insert(0, side.jobs.pop())
        for n, job in enumerate(jobs):
            side.add(source_ref, job)
            if n_rows == _LANES:
                side.add()
            side.jobs += before[n * len(before) // len(jobs):(n + 1) * len(before) // len(jobs)]
        n_products = out_ref.shape[0]
        for job in _combination_jobs(out_ref, 2 if n_products == len(_HOPCROFT_KERR) else 4,
                                     _WEIGHT, lambda i, j, rows: wide_ref[i, j, rows],
                                     {r: r for r in range(n_products)}):
            side.add(wide_ref, job)

    def staged_rows(part, rows, packing):
        count = min(len(rows), _CHUNK)
        for first in rows[::count]:
            c, offset = divmod(first, _CHUNK)
            if isinstance(part, int):
                source = _PARTS if c == part else c
            else:
                source = jnp.where(part == c, _PARTS, c)
            yield _aligned(source * (_CHUNK // packing) + offset // packing, count // packing)

    def block_copies(m, part, slot, rows=pl.ds(0, d_model // 2)):
        src = (wot_hbm, w1_hbm, w2t_hbm, w3_hbm)[m].bitcast(words)
        dst, sem = stage_ref.at[slot], stage_sem.at[slot]
        if m == _WO:
            return [pltpu.make_async_copy(src.at[_TILES * part + j, rows],
                                          dst.at[rows, pl.ds(j * _LANES, _LANES)], sem)
                    for j in range(_TILES)]
        return [pltpu.make_async_copy(src.at[rows, _aligned(part * width, width)],
                                      dst.at[rows], sem)]

    def shared_copies(m):
        return [copy for c in range(_PARTS) for copy in block_copies(
            m, c, shared_slot + m, pl.ds(c * _CHUNK // 2, _CHUNK // 2))]

    def last_copies(m):
        return block_copies(m, _PARTS, last_slots[m])

    def staged(slot, part, rows, j):
        tile = pltpu.bitcast(jnp.concatenate(
            [stage_ref[slot, piece, j * _LANES:(j + 1) * _LANES]
             for piece in staged_rows(part, rows, 2)], axis=0), bf16)
        return (tile.T if len(rows) == _LANES else tile).astype(f32)

    def store_block(m, out_ref, block):
        combine_weights(out_ref, stage_ref, block, _LANES if m in (_WO, _W2) else _CHUNK, 1)

    def store_part(m, out_ref, part, slot):
        store_block(m, out_ref.at[part], lambda rows, j: (
            staged(slot, part, rows, j) - staged(shared_slot + m, part, rows, j)))

    def store_shared(m, out_ref):
        store_block(m, out_ref.at[out_ref.shape[0] - 1],
                    functools.partial(staged, shared_slot + m, _PARTS))

    def store_last(m, out_ref):
        part = {_W1: 0, _W3: 1, _W2: _PARTS}[m]

        def block(rows, j):
            own = staged(last_slots[m], part, rows, j)
            if m != _W2 and rows[0] == (1 - part) * _CHUNK:
                return own - staged(last_slots[_W1 + _W3 - m], part, rows, j)
            return own

        store_block(m, out_ref.at[_PARTS], block)
        for j in range(_TILES):
            rows = range(part * _CHUNK, (part + 1) * _CHUNK)
            wplain_ref[int(m == _W2), j, pl.ds(part % 2 * _CHUNK, _CHUNK)] = staged(
                last_slots[m], _PARTS, rows, j).astype(bf16)

    def first_step_copies(t):
        return [copy for n in range(2) for copy in block_copies(_W3, 2 * t + n, 3 * (t & 1) + n)
                ] + (shared_copies(_W3) if t == 0 else last_copies(_W3) if t == 1
                     else last_copies(_W1) if t == 2 else [])

    def load_weights(early_in_ref, early_shared_ref, head_ref, head_sem, *rows_refs):
        n_early = n_io - 1
        products = len(_HOPCROFT_KERR)

        def pair_copies(w, part, slot, rows):
            src = (wq_hbm, wk_hbm, wv_hbm)[w].bitcast(words)
            return [pltpu.make_async_copy(src.at[rows, 2 * part + n, :],
                                          head_ref.at[slot, n, rows], head_sem.at[slot])
                    for n in range(2)]

        def head_copies(part, which=range(3)):
            return [copy for w in which
                    for copy in pair_copies(w, part, 3 * (part & 1) + w, pl.ds(0, d_model))]

        def shared_head_copies(w):
            return [copy for c in range(_PARTS)
                    for copy in pair_copies(w, c, shared_slot + w, pl.ds(c * _CHUNK, _CHUNK))]

        def part_copies(part):
            return [copy for m in range(3) for copy in block_copies(m, part, 3 * (part & 1) + m)]

        def head(slot, rows, j):
            pair = head_ref[slot, j // 2, rows, :]
            return pltpu.bitcast(pair & words(0xFFFF0000) if j % 2 else pair << 16, f32)

        def store_heads(w, part):
            def block(rows, j):
                rows = next(staged_rows(part, rows, 1))
                return head(3 * (part & 1) + w, rows, j) - head(shared_slot + w, rows, j)

            combine_weights(wqkv_ref.at[w, part], head_ref, block, _CHUNK // 2, 2)

        def store_shared_heads(w):
            @pl.loop(0, _LANES // _SLAB)
            def _(n):
                operands = _operands(_levels(2), _WEIGHT, lambda i, j: head(
                    shared_slot + w, _aligned(i * _LANES + n * _SLAB, _SLAB), j))
                for r, operand in operands.items():
                    wqkv_ref[w, _PARTS, r, _aligned(n * _SLAB, _SLAB)] = operand().astype(bf16)

        def x_copies(first, last):
            tiles = [(c + 1) % n_io for c in range(first, last)]
            return [pltpu.make_async_copy(xt_hbm.at[:, pl.ds(i * _LANES, _LANES)],
                                          tile_ref.at[i, :d_model], tile_sem.at[i])
                    for i in tiles]

        def transpose_in(c):
            i = (c + 1) % n_io
            x_ref[i, :_LANES] = _load_packed(tile_ref, i, slice(0, d_model // 2)).T

        def normalize(c):
            for s in range(4):
                _store_rows(rows_refs[c % 3], s // 2, s % 2 * ahead,
                            _layernorm(x_ref[c + 1, s * seg:s * seg + ahead].astype(f32)))

        def fetch(c):
            transpose_in(c)
            if c < n_early:
                normalize(c)

        def prepare(c):
            rows_ref = rows_refs[c % 3]
            for n, job in enumerate(_operand_jobs(early_in_ref.at[c], rows_ref, None)):
                place = 2 * n if c + 2 >= n_early else len(side.jobs)
                side.jobs.insert(place, (c, rows_ref, job))

        def prepare_parts(c):
            for tile in range(_TILES):
                for job in _operand_jobs(early_in_ref.at[c], rows_refs[c % 3], tile):
                    side.add(rows_refs[c % 3], job)

        def project(w, part, c, operand):
            shared = isinstance(part, int) and part == _PARTS

            def keep(f, j, tile):
                early_shared_ref[w, c, f, j] = tile

            def store(f, j, tile):
                early_ref[2 * c + f, w, part, j] = tile.astype(bf16)

            _collect(_levels(2), _WIDE,
                     lambda r: side.dot(operand(r, c), _load_packed(wqkv_ref, w, part, r)),
                     lambda f, j: None if shared else early_shared_ref[w, c, f, j],
                     keep if shared else store)

        def project_shared(pending, first, last):
            operand = _operand_loader(early_in_ref, 2, _PARTS)
            ready = pending + [(w, c) for c in range(first, last) for w in range(3)]
            held = [(w, c) for w, c in ready if w and c + 2 >= last and last < n_early]
            fetch(first)
            side.add(tile_ref, functools.partial(fetch, first + 1))
            prepare(first)
            side.spread(len(pending) * products)
            for w, c in ready:
                if w == 0:
                    side.finish(c)
                    if c + 2 < last + (last == n_early):
                        side.add(tile_ref, functools.partial(fetch, c + 2))
                    if c + 1 < last:
                        prepare(c + 1)
                    prepare_parts(c)
                    if c + 3 == n_early:
                        store_heads(0, 0)
                    side.spread((3 * (n_early - c) - .5 if c + 3 >= n_early
                                 else 1 if (1, c) in held else 3) * products)
                if (w, c) not in held:
                    project(w, _PARTS, c, operand)
            side.finish()
            return held

        def project_part(part, which):
            operand = _operand_loader(early_in_ref, 2, part)
            side.spread((len(which) * n_early - .7) * products)
            for w in which:
                for c in range(n_early):
                    project(w, part, c, operand)
            side.finish()

        def store_parts(part, other):
            for m, out_ref in enumerate((wo_ref, w1_ref, w2_ref)):
                store_part(m, out_ref, part, 3 * (part & 1) + m)
                other(m)

        middle = n_io // 2
        _start(x_copies(0, 3) + shared_head_copies(0))
        for w in range(3):
            head_ref[shared_slot + w, :, width:d_model] = jnp.zeros((2, _CHUNK, d_head), words)
        for m in range(4):
            stage_ref[shared_slot + m, width // 2:d_model // 2] = jnp.zeros(
                (_CHUNK // 2, width), words)
        side.keep_in_memory(early_in_ref, early_shared_ref)
        _wait(x_copies(0, 3))
        _start(shared_head_copies(1))
        for c in range(3):
            transpose_in(c)
        copies = (shared_head_copies(2) + x_copies(3, middle), x_copies(middle, middle + 3),
                  x_copies(middle + 3, n_io) + head_copies(0, [0]))
        for w in range(2):
            _wait(shared_head_copies(w))
            _start(copies[w])
            store_shared_heads(w)
            for c in range(3):
                if w:
                    prepare_parts(c)
                else:
                    normalize(c)
                    prepare(c)
            side.spread(2.5 * products)
            for c in range(3):
                side.finish(c)
                project(w, _PARTS, c, _operand_loader(early_in_ref, 2, _PARTS))
            side.finish()
        _wait(copies[0])
        _start(copies[2])
        store_shared_heads(2)
        held = project_shared([(2, c) for c in range(3)], 3, middle)
        _wait(copies[1] + copies[2])
        copies = part_copies(0) + [copy for m in range(3) for copy in shared_copies(m)]
        _start(head_copies(0, [1, 2]) + copies)
        project_shared(held, middle, n_early)
        _start(head_copies(1))
        _wait(head_copies(0, [1, 2]))
        store_heads(1, 0)
        store_heads(2, 0)
        project_part(0, [0])
        _start(part_copies(1) + head_copies(2))
        _wait(copies + head_copies(1))
        store_parts(0, lambda w: store_heads(w, 1))
        project_part(0, [1, 2])

        @pl.loop(1, _PARTS - 1, unroll=True)
        def _(part):
            _start(part_copies(part + 1))
            pl.when(part + 2 < _PARTS)(lambda: _start(head_copies(part + 2)))
            pl.when(part + 2 == _PARTS)(lambda: _start(last_copies(_W2)))
            _wait(part_copies(part) + head_copies(part + 1))
            store_parts(part, lambda w: store_heads(w, part + 1))
            project_part(part, range(3))

        _start(first_step_copies(0))
        _wait(part_copies(_PARTS - 1) + last_copies(_W2))
        store_parts(_PARTS - 1, lambda m: store_last(_W2, w2_ref) if m == _W1
                    else store_shared(m, w2_ref if m == _W2 else wo_ref))
        project_part(_PARTS - 1, range(3))

    def run_layers(w3_ref, pair_rows_ref, pair_in_ref, solo_rows_ref, solo_in_ref, ffn_rows_ref,
                   ffn_in_ref, attn_shared_ref, ffn_shared_ref, partial_ref, qkv_ref, heads_ref,
                   hidden_ref, attn_sum_ref, ffn_sum_ref, mem_ref, block_ref, second_ref):
        def segment(s):
            return s >> 2, _aligned((s & 3) * seg, seg)

        def transpose_out(i):
            tile_ref.bitcast(words)[i, :d_model // 2] = pltpu.bitcast(x_ref[i, :_LANES].T, words)

        def contract(groups, part, rows_ref, weight_ref, sum_ref, begun):
            operands = _operands(_levels(groups), _WIDE, lambda f, j: rows_ref[part, f, j])

            def targets(i):
                return [_TILES if 2 * i + half == part else i for half in range(2)]

            def start(f, i):
                low, high = (
                    sum_ref[f, n] if (n, half) in begun else None if groups < 4
                    else block_ref[f, :, n * _LANES:(n + 1) * _LANES]
                    for half, n in enumerate(targets(i)))
                if targets(i) == [i, i] and ((i, 0) in begun) == ((i, 1) in begun):
                    return low
                if low is None and high is None:
                    return None
                lanes = jax.lax.broadcasted_iota(jnp.int32, sum_ref.shape[-2:], 1)
                return jnp.where(lanes < _CHUNK, 0.0 if low is None else low,
                                 0.0 if high is None else high)

            def finish(f, i, tile):
                if targets(i) == [i, i]:
                    sum_ref[f, i] = tile
                else:
                    for half, n in enumerate(targets(i)):
                        lanes = slice(half * _CHUNK, (half + 1) * _CHUNK)
                        sum_ref[f, n, :, lanes] = tile[:, lanes]

            _collect(_levels(groups), _MODEL,
                     lambda r: side.dot(operands[r](), _load_packed(weight_ref, part, r)),
                     start, finish, partial_ref.at[part % 2])
            begun.update((n, half) for i in range(_TILES) for half, n in enumerate(targets(i)))

        def keep_and_add(ref, part, f, j, tile):
            total = ref.shape[0] - 1
            ref[part, f, j] = tile
            if 0 < part < _PARTS:
                ref[total, f, j] = ref[total if part > 1 else 0, f, j] + tile

        def project(groups, w, part):
            in_ref = pair_in_ref if groups == 2 else solo_in_ref
            rows = slice(0, in_ref.shape[1])
            side.finish(("P", None), ("P", part // 2))
            operand = _operand_loader(in_ref, groups, part)
            out_ref = qkv_ref.at[w, part % qkv_ref.shape[1]]
            done = {}

            def finish(f, j, tile):
                done[f, j] = tile
                if part == _PARTS:
                    attn_shared_ref[w, f, j, rows] = tile
                elif groups == 2 and (1 - f, j) in done:
                    upper, lower = done[0, j], done[1, j]
                    out_ref[j, :2 * size - ahead] = jnp.concatenate(
                        [upper[n_mem:n_mem + ahead], upper[:n_mem], lower[:n_mem],
                         upper[n_mem + ahead:], lower[n_mem:]], axis=0).astype(bf16)
                elif groups == 1 and (0, j ^ 1) in done:
                    a, b = done[0, j & ~1], done[0, j | 1]
                    out_ref[j | 1] = jnp.concatenate(
                        [a[n_mem:], a[:n_mem], b], axis=0).astype(bf16)

            _collect(_levels(groups), _WIDE,
                     lambda r: side.dot(operand(r), _load_packed(wqkv_ref, w, part, r)),
                     lambda f, j: attn_shared_ref[w, f, j, rows] if part < _PARTS else None,
                     finish)

        def projected(groups, t, place, w, head):
            part, j = divmod(head, _TILES)
            index = w, part % qkv_ref.shape[1], j
            if groups == 1:
                return _load_packed(qkv_ref, *index)
            early = _load_words(early_ref, (t - _LAG) >> 1, w, part, j,
                                _aligned((place & 1) * (ahead // 2), ahead // 2))
            return pltpu.bitcast(jnp.concatenate(
                [early, _load_words(qkv_ref, *index, slice(0, size - ahead // 2))], axis=0), bf16)

        def by_group(tile):
            return enumerate(tile[f * seg:(f + 1) * seg] for f in range(4))

        def expand(g):
            plain = 2 * _PARTS + 2
            if g == plain:
                x = jnp.concatenate([ffn_rows_ref[f, 0, :seg] for f in range(4)], axis=0)
                for j in range(_TILES):
                    for f, tile in by_group(_dot(x.astype(bf16), _load_packed(wplain_ref, 0, j))):
                        ffn_shared_ref[2, f, j] = tile
                return
            part, up = divmod(g if g < plain else g - 1, 2)
            chunk = up if part == _PARTS else min(part, _PARTS)
            side.finish(("G", None), ("G", chunk // 2))
            operand = _operand_loader(ffn_in_ref, 4, chunk)
            weight_ref = w3_ref if up else w1_ref

            def finish(f, j, tile):
                if part > _PARTS:
                    ffn_shared_ref[up, f, j] = tile
                elif up:
                    keep_and_add(hidden_ref, part, f, j, hidden_ref[part, f, j] * tile)
                else:
                    hidden_ref[part, f, j] = _silu(tile)

            _collect(_levels(4), _WIDE,
                     lambda r: side.dot(operand(r), _load_packed(weight_ref, part, r)),
                     lambda f, j: None if part > _PARTS else ffn_shared_ref[
                         2 if part == _PARTS else up, f, j],
                     finish, partial_ref.at[g % 2])

        def reduce(g, begun):
            if not begun:
                for f in range(4):
                    rest = block_ref[f, :, width:]
                    ffn_sum_ref[f, _TILES] = jnp.concatenate([rest, jnp.zeros_like(rest)], axis=1)
                begun.update([(_TILES, 0), (_TILES, 1)])
            if g < w2_ref.shape[0]:
                contract(4, g, hidden_ref, w2_ref, ffn_sum_ref, begun)
                return
            total = None
            for j in range(_TILES):
                rows = jnp.concatenate([hidden_ref[_PARTS, f, j] for f in range(4)], axis=0)
                total = _accumulate(total, 1, _dot(
                    _load_packed(wplain_ref, 1, j, slice(0, _CHUNK // 2)), rows.astype(bf16), 1))
            for f, tile in by_group(_value(total).T):
                ffn_sum_ref[f, _TILES, :, :_CHUNK] += tile

        def layer_input(t, place, layer):
            return x_ref[segment(t)].astype(f32) if layer == 0 else second_ref[place & 1]

        def begin_step(t, place, layers):
            h = _layernorm(layer_input(t, place, layers[-1]))
            if len(layers) == 1:
                rows_ref, in_ref = solo_rows_ref, solo_in_ref
                _store_rows(rows_ref, 0, n_mem, h)
            else:
                rows_ref, in_ref, cut = pair_rows_ref, pair_in_ref, ahead // 2
                _store_rows(rows_ref, 0, n_mem, _layernorm(layer_input(t, place, 0)[ahead:]))
                _store_rows(rows_ref, 0, seg - cut, h[:cut])
                _store_rows(rows_ref, 1, n_mem, h[cut:])
            for f, layer in enumerate(layers):
                _store_rows(rows_ref, f, 0, mem_ref[layer])
            for tile in [None, *range(_TILES)]:
                for job in _operand_jobs(in_ref, rows_ref, tile):
                    side.add(rows_ref, job, ("P", tile))

        def close_step(t, place, layers):
            for f, layer in enumerate(layers):
                out = _load_rows(attn_sum_ref, f)
                mem_ref[layer] = out[:n_mem]
                index = 2 * layer + (place & 1) if len(layers) == 2 else place & 3
                block_ref[index] = layer_input(t, place, layer) + out[n_mem:]

        def run(order, layers=(), t=0, place=0):
            groups, first = len(layers), t
            visible, fill = _attention_masks(n_mem, seg)
            attn_begun, ffn_begun, probs = set(), set(), {}
            for name in order.split():
                stage, g = name[0], int(name[1:] or 0)
                if stage == "N":
                    begin_step(t, place, layers)
                elif stage == "P":
                    project(groups, g % 3, g // 3)
                elif stage == "S" and (groups == 2 or g % 2):
                    q, k = (projected(groups, t, place, w, g) for w in range(2))
                    s = jnp.where(visible, _dot(q, k, 1) * score_scale, fill)
                    p = jnp.exp2(s - jnp.max(s, axis=-1, keepdims=True))
                    inv = pltpu.reciprocal(jnp.sum(p, axis=-1, keepdims=True), approx=True)
                    probs[g] = p.astype(bf16), inv
                elif stage == "V" and (groups == 2 or g % 2):
                    o = _dot(probs[g][0], projected(groups, t, place, 2, g)) * probs[g][1]
                    halves = jnp.concatenate([o[seg:size], o[:seg]], axis=0), o[size:]
                    for f, half in enumerate(halves):
                        index = (f, g % _TILES) if groups == 2 else (0, g % _TILES - 1 + f)
                        keep_and_add(heads_ref, g // _TILES, *index, half)
                elif stage == "O":
                    contract(groups, g, heads_ref, wo_ref, attn_sum_ref, attn_begun)
                elif stage == "A":
                    close_step(t, place, layers)
                    t, place, attn_begun = t + 1, place + 1, set()
                elif stage == "M":
                    _store_rows(ffn_rows_ref, g, 0, _layernorm(block_ref[g]))
                elif stage == "F":
                    tile = g if g < _TILES else None
                    for job in _operand_jobs(ffn_in_ref, ffn_rows_ref, tile):
                        side.add(ffn_rows_ref, job, ("G", tile))
                elif stage == "G":
                    expand(g)
                elif stage == "D":
                    reduce(g, ffn_begun)
                elif stage == "E":
                    for s in range(2):
                        second_ref[s] = _load_rows(ffn_sum_ref, s)
                        x_ref[segment(first - _LAG - 2 + s)] = _load_rows(
                            ffn_sum_ref, 2 + s).astype(bf16)
                elif stage == "T":
                    side.add(x_ref, functools.partial(
                        transpose_out, jnp.maximum(first - 10, 0) >> 2))
                elif stage == "Z":
                    for _ in range(g):
                        side.add()
                elif stage == "W":
                    side.spread(g)
                elif stage == "X":
                    side.finish()

        side.keep_in_memory(pair_in_ref, solo_rows_ref, solo_in_ref, ffn_in_ref, attn_shared_ref,
                            ffn_shared_ref, partial_ref, qkv_ref, heads_ref, hidden_ref,
                            attn_sum_ref, ffn_sum_ref)
        attn_sum_ref[...] = jnp.zeros_like(attn_sum_ref)
        mem_copy.wait()
        mem_ref[0] = mem0_ref[...].astype(f32)
        for t in range(_LAG):
            run("N", (0,), t, t)
            _start(first_step_copies(t + 1) if t + 1 < _LAG else [mem_copy])
            _wait(first_step_copies(t))
            (store_shared, store_last)[t // 2](*((_W1, w1_ref), (_W3, w3_ref))[t % 2])
            for n in range(2):
                store_part(_W3, w3_ref, 2 * t + n, 3 * (t & 1) + n)
            run("W540 " + _ATTENTION + " X", (0,), t, t)
        mem_copy.wait()
        mem_ref[1] = mem0_ref[...].astype(f32)
        run(_SWIGLU)
        for s in range(2):
            second_ref[s] = _load_rows(ffn_sum_ref, s)
        run(2 * ("N W200 " + _ATTENTION + " ") + "M0 M2 M1 M3 F4 X", (0, 1), _LAG)
        for s in range(2):
            second_ref[s] = _load_rows(ffn_sum_ref, 2 + s)

        @pl.loop(_LAG // 2 + 1, n_seg // 2)
        def _(b):
            run(_TWO_STEPS + " X", (0, 1), 2 * b)

        out_copies = [
            pltpu.make_async_copy(tile_ref.at[i, :d_model],
                                  outt_hbm.at[:, pl.ds(i * _LANES, _LANES)], tile_sem.at[i])
            for i in range(n_io)]
        _start(out_copies[:n_io - 2])
        run(" ".join(name for name in _TWO_STEPS.split()
                     if name[0] not in "MT" and name != "F4") + " X", (1,), n_seg)
        pl.loop(n_seg + 2, n_seg + _LAG)(
            lambda t: run("N W200 " + _ATTENTION + " X", (1,), t, t))
        transpose_out(n_io - 2)
        run(_SWIGLU)
        for s in range(_LAG):
            x_ref[segment(n_seg - _LAG + s)] = _load_rows(ffn_sum_ref, s).astype(bf16)
        transpose_out(n_io - 1)
        _start(out_copies[n_io - 2:])
        _wait(out_copies)

    spare = 8
    mem_copy = pltpu.make_async_copy(mem0_hbm, mem0_ref, mem_sem)
    mem_copy.start()
    pl.run_scoped(
        load_weights,
        pltpu.VMEM((n_io - 1, len(_operand_slots(2)), seg, _LANES), bf16),
        pltpu.VMEM((3, n_io - 1, 2, _TILES, seg, _LANES), f32),
        pltpu.VMEM((shared_slot + 3, 2, d_model + spare, d_head), words),
        pltpu.SemaphoreType.DMA((shared_slot + 3,)),
        *[pltpu.VMEM((2, _TILES + 1, seg + spare, _LANES), f32)] * 3)
    pl.run_scoped(
        run_layers,
        pltpu.VMEM(w1_ref.shape, bf16),
        pltpu.VMEM((2, _TILES + 1, seg + spare, _LANES), f32),
        pltpu.VMEM((len(_operand_slots(2)), seg, _LANES), bf16),
        pltpu.VMEM((1, _TILES + 1, size + spare, _LANES), f32),
        pltpu.VMEM((len(_operand_slots(1)), size, _LANES), f32),
        pltpu.VMEM((4, _TILES + 1, seg + spare, _LANES), f32),
        pltpu.VMEM((len(_operand_slots(4)), seg, _LANES), bf16),
        pltpu.VMEM((3, 2, _TILES, size, _LANES), f32),
        pltpu.VMEM((3, 4, _TILES, seg, _LANES), f32),
        pltpu.VMEM((2, 4, _TILES, seg, _LANES), f32),
        pltpu.VMEM((3, 3, _TILES, 2 * size, _LANES), bf16),
        pltpu.VMEM((_PARTS + 1, 2, _TILES, size, _LANES), f32),
        pltpu.VMEM((_PARTS + 2, 4, _TILES, seg, _LANES), f32),
        pltpu.VMEM((2, _TILES + 1, size, _LANES), f32),
        pltpu.VMEM((4, _TILES + 1, seg, _LANES), f32),
        pltpu.VMEM((2, n_mem, d_model), f32),
        pltpu.VMEM((4, seg, d_model), f32),
        pltpu.VMEM((2, seg, d_model), f32))


@functools.partial(jax.jit, static_argnames=("A_seg_len",))
def pallas_interleave_layers__memory_aug_recurrent_mem_tr__glu_gated_swiglu__prompt_kernel(
    A_x: jax.Array,
    A_mem0: jax.Array,
    A_Wq: jax.Array,
    A_Wk: jax.Array,
    A_Wv: jax.Array,
    A_Wo: jax.Array,
    A_seg_len: int,
    B_x: jax.Array,
    B_w1: jax.Array,
    B_w3: jax.Array,
    B_w2: jax.Array,
):
    del B_x
    _, n_tok, d_model = A_x.shape
    n_mem = A_mem0.shape[1]
    _, n_heads, d_head = A_Wq.shape
    seg = A_seg_len
    assert A_x.shape[0] == 1 and _LAG * seg == d_head == _LANES and 4 * n_mem == seg
    assert n_heads == _PARTS * _TILES and d_model == (_PARTS + 1) * _CHUNK
    assert B_w1.shape[1] == (_PARTS + 1) * _TILES * _LANES and n_tok == 16 * _LANES
    bf16 = jnp.bfloat16
    attn_blocks = (_PARTS + 1, len(_HOPCROFT_KERR), _LANES, _LANES)
    ffn_blocks = (_PARTS + 2, len(_STRASSEN) ** 2, _LANES, _LANES)
    hbm = pl.BlockSpec(memory_space=pltpu.HBM)
    out_t = pl.pallas_call(
        functools.partial(_kernel, seg=seg),
        out_shape=jax.ShapeDtypeStruct((d_model, n_tok), A_x.dtype),
        in_specs=[hbm] * 9,
        out_specs=hbm,
        scratch_shapes=[
            pltpu.VMEM((n_mem, d_model), bf16),
            pltpu.VMEM((n_tok // _LANES, d_model + _SLAB, _LANES), bf16),
            pltpu.VMEM((n_tok // _LANES, _LANES + _SLAB, d_model), bf16),
            pltpu.VMEM(((n_tok // seg - _LAG) // 2, 3, _PARTS, _TILES, seg, _LANES), bf16),
            pltpu.VMEM((3, *attn_blocks), bf16),
            pltpu.VMEM(attn_blocks, bf16),
            pltpu.VMEM(ffn_blocks, bf16),
            pltpu.VMEM(ffn_blocks, bf16),
            pltpu.VMEM((2, _TILES, _LANES, _LANES), bf16),
            pltpu.VMEM((11, (d_model + _SLAB) // 2, _TILES * _LANES), jnp.uint32),
            pltpu.SemaphoreType.DMA((11,)),
            pltpu.SemaphoreType.DMA(()),
            pltpu.SemaphoreType.DMA((n_tok // _LANES,)),
            *[pltpu.VMEM((_TILES, _TILES, _LANES + _SLAB // 2, _LANES), jnp.float32)] * 2,
        ],
        compiler_params=pltpu.CompilerParams(
            vmem_limit_bytes=127 * 1024 * 1024,
            flags={"XLA_TPU_FORCE_LP_LLO_SCHEDULER": True}),
    )(A_x.reshape(n_tok, d_model).T, A_mem0.reshape(n_mem, d_model), A_Wq, A_Wk, A_Wv,
      A_Wo.transpose(0, 2, 1), B_w1, B_w2.T, B_w3)
    return out_t.T.reshape(A_x.shape)
```

```python
import functools
import math

import jax
import jax.numpy as jnp
import jax.experimental.pallas as pl
import jax.experimental.pallas.tpu as pltpu

_EPS = 1e-05
_MASKED = -1000000000.0
_LOG2E = math.log2(math.e)
_LANES = 128
_CHUNK = _LANES // 2
_SLAB = 16
_TILES = 4
_PARTS = 2 * _TILES
_LAG = 4
_WO, _W1, _W2, _W3 = range(4)
_MODEL, _WEIGHT, _WIDE = range(3)
_HOPCROFT_KERR = (
    (((1, 1, 2),), ((1, 2, 0), (1, 2, 2), (1, 2, 3), (-1, 1, 2)), ((1, 2, 2),)),
    (((1, 2, 2),), ((1, 2, 1), (1, 2, 2), (-1, 0, 2), (-1, 3, 2)), ((1, 0, 2),)),
    (((1, 0, 2), (1, 0, 3)), ((1, 2, 3),), ((-1, 2, 2), (1, 2, 3))),
    (((1, 2, 2), (1, 0, 3)), ((1, 2, 3), (1, 3, 2)), ((1, 2, 2), (-1, 1, 3))),
    (((1, 2, 2), (1, 2, 3)), ((1, 3, 2),), ((-1, 1, 2), (1, 1, 3))),
    (((1, 0, 0), (1, 0, 2)), ((1, 2, 0),), ((1, 2, 0), (-1, 2, 2))),
    (((1, 0, 0), (1, 2, 2)), ((1, 0, 2), (1, 2, 0)), ((-1, 1, 0), (1, 2, 2))),
    (((1, 2, 0), (1, 2, 2)), ((1, 0, 2),), ((1, 1, 0), (-1, 1, 2))),
    (((1, 0, 1), (1, 0, 2)), ((1, 2, 1),), ((1, 0, 1), (-1, 0, 2))),
    (((1, 0, 1), (1, 1, 2)), ((1, 1, 2), (1, 2, 1)), ((1, 1, 1), (1, 0, 2))),
    (((1, 1, 1), (1, 1, 2)), ((1, 1, 2),), ((-1, 1, 1), (1, 1, 2))),
    (((1, 1, 1), (1, 1, 3)), ((1, 0, 3), (-1, 1, 3)), ((1, 2, 1), (-1, 2, 3))),
    (((1, 0, 0), (1, 0, 1), (1, 0, 3)), ((1, 0, 3),), ((1, 2, 1), (-1, 2, 0), (1, 2, 3))),
    (((1, 2, 0), (1, 2, 1), (1, 0, 3)), ((1, 0, 3), (1, 3, 0)),
     ((1, 2, 0), (-1, 2, 1), (-1, 1, 3))),
    (((1, 2, 0), (1, 2, 1), (1, 2, 3)), ((1, 3, 0),), ((1, 1, 1), (-1, 1, 0), (1, 1, 3))),
    (((1, 1, 3),), ((1, 0, 3), (-1, 1, 3), (1, 3, 0), (1, 3, 2), (1, 3, 3)), ((1, 1, 3),)),
    (((1, 2, 1), (1, 2, 3)), ((1, 3, 0), (1, 3, 1)), ((1, 0, 1), (-1, 0, 3))),
    (((1, 1, 3), (-1, 2, 1)), ((1, 3, 0), (1, 3, 1), (-1, 0, 3), (1, 1, 3)),
     ((1, 2, 1), (-1, 0, 3))),
    (((1, 0, 3),), ((1, 3, 0), (1, 3, 1), (-1, 0, 3), (-1, 2, 3), (1, 3, 3)), ((1, 0, 3),)),
    (((1, 1, 0), (1, 1, 1)), ((1, 0, 3), (1, 1, 0)), ((1, 2, 0), (-1, 2, 1))),
    (((1, 2, 1), (-1, 1, 0)), ((1, 0, 1), (1, 1, 0)), ((1, 0, 0), (-1, 2, 1))),
    (((1, 0, 1),), ((1, 1, 0), (1, 1, 1), (1, 1, 3), (-1, 0, 3), (-1, 2, 1)), ((1, 2, 1),)),
    (((1, 2, 0), (1, 2, 1)), ((1, 0, 1), (1, 3, 0)), ((-1, 0, 0), (1, 0, 1))),
    (((1, 2, 1),), ((1, 3, 0), (1, 3, 1), (1, 0, 1), (-1, 1, 1), (-1, 1, 2)), ((1, 1, 1),)),
    (((1, 0, 0),), ((1, 0, 0), (1, 0, 1), (-1, 2, 0)), ((1, 0, 0),)),
    (((1, 1, 0),), ((1, 0, 0), (1, 0, 2), (-1, 1, 0)), ((1, 1, 0),)),
)
_RUNS = (5, 11, 19, 24, 24)
_STRASSEN = (
    (((-1, 2, 0),), ((1, 0, 0), (1, 0, 1)), ((1, 1, 1),)),
    (((1, 1, 0), (1, 1, 1)), ((1, 0, 0),), ((1, 1, 0), (-1, 1, 1))),
    (((1, 1, 1),), ((1, 1, 0), (-1, 0, 0)), ((1, 2, 0),)),
    (((1, 0, 0), (1, 1, 1)), ((1, 0, 0), (1, 1, 1)), ((1, 0, 0), (1, 1, 1))),
    (((1, 0, 0),), ((1, 0, 1), (-1, 1, 1)), ((1, 2, 1),)),
    (((1, 0, 0), (1, 0, 1)), ((1, 1, 1),), ((-1, 0, 0), (1, 0, 1))),
    (((1, 2, 1),), ((1, 1, 0), (1, 1, 1)), ((1, 0, 0),)),
)
_ATTENTION = (
    "P24 P25 P26 P0 P1 P2 S0 S1 S2 S3 P3 P4 V0 V1 V2 V3 P5 S4 S5 S6 S7 O0 P6 P7 V4 V5 V6 V7 "
    "P8 S8 S9 S10 S11 O1 P9 P10 V8 V9 V10 V11 P11 S12 S13 S14 S15 O2 P12 P13 V12 V13 V14 V15 "
    "P14 S16 S17 S18 S19 O3 P15 P16 V16 V17 V18 V19 P17 S20 S21 S22 S23 P18 P19 V20 V21 V22 "
    "V23 P20 S24 S25 S26 S27 P21 P22 V24 V25 V26 V27 P23 S28 S29 S30 S31 O4 V28 V29 V30 V31 "
    "O5 O6 O7 O8 A")
_SWIGLU = (
    "M0 M1 M2 M3 F4 X F0 F1 F2 F3 W500 G18 G19 G20 G16 G17 G0 D8 D10 G1 G2 D0 G3 G4 D1 G5 G6 "
    "D2 G7 G8 D3 G9 G10 D4 G11 G12 G13 G14 D5 G15 D6 D7 D9")
_TWO_STEPS = (
    "E F4 X N Z7 F0 W250 G19 G20 P24 P25 P26 G16 P0 P1 G17 P2 S0 S1 S2 S3 P3 P4 V0 V1 V2 V3 "
    "P5 G0 S4 S5 S6 S7 O0 G1 P6 P7 V4 V5 V6 V7 P8 D8 S8 S9 S10 S11 O1 F1 W200 G2 P9 P10 V8 V9 "
    "V10 V11 P11 S12 S13 S14 S15 O2 D0 P12 P13 V12 V13 V14 V15 P14 S16 S17 S18 S19 O3 G3 P15 "
    "P16 V16 V17 V18 V19 P17 S20 S21 S22 S23 O4 G4 P18 P19 V20 V21 V22 V23 P20 S24 S25 S26 "
    "S27 O5 F2 W200 D1 P21 P22 V24 V25 V26 V27 P23 S28 S29 S30 S31 O6 G5 V28 V29 V30 V31 G6 "
    "O7 O8 A Z0 N W200 D2 G7 D3 P24 P25 P26 G8 P0 P1 P2 S0 S1 S2 S3 P3 P4 V0 V1 V2 V3 P5 G9 "
    "S4 S5 S6 S7 O0 P6 F3 W200 G10 P7 V4 V5 V6 V7 P8 S8 S9 S10 S11 O1 D4 P10 P9 V8 V9 V10 V11 "
    "P11 S12 S13 S14 S15 O2 G11 P12 P13 V12 V13 V14 V15 P14 S16 S17 S18 S19 O3 G12 P15 P16 "
    "V16 V17 V18 V19 P17 S20 S21 S22 S23 O4 T W78 P18 P19 V20 V21 V22 V23 P20 S24 S25 S26 S27 "
    "O5 G14 G13 P21 P22 V24 V25 V26 V27 P23 S28 S29 S30 S31 O6 D5 V28 V29 V30 V31 G15 O7 O8 "
    "M0 M2 A M3 D10 D6 M1 D7 D9 G18")
_LAST_STEPS = (
    "E F4 X N F0 F1 W400 G19 G20 " + _ATTENTION.replace("O0", "O0 G16 G17 G0 D8 G1 G2 D0 G3")
    + " N F2 F3 W450 G4 D1 D10 G5 G6 D2 G7 G8 D3 G9 G10 D4 G11 G12 G13 G14 D5 G15 D6 D7 D9 E2 "
    + _ATTENTION + 2 * (" N W200 " + _ATTENTION))


def _layernorm(x):
    m = jnp.mean(x, axis=-1, keepdims=True)
    d = x - m
    v = jnp.mean(d * d, axis=-1, keepdims=True)
    return d * jax.lax.rsqrt(v + _EPS)


def _scaled_silu(x):
    return x * pltpu.reciprocal(1.0 + jnp.exp2(x), approx=True)


def _dot(a, b, axis=0):
    return jax.lax.dot_general(a, b, (((1,), (axis,)), ((), ())),
                               preferred_element_type=jnp.float32)


def _load_words(ref, *index):
    return ref[index] if ref.dtype == jnp.float32 else ref.bitcast(jnp.uint32)[index]


def _load_packed(ref, *index):
    return pltpu.bitcast(_load_words(ref, *index), ref.dtype)


def _aligned(first, size):
    return pl.ds(first if isinstance(first, int) else pl.multiple_of(first, size), size)


def _accumulate(total, sign, value):
    if total is None:
        return sign, value
    if total[0] == sign:
        return sign, jax.lax.add(total[1], value)
    return 1, jax.lax.sub(*((total[1], value) if sign < 0 else (value, total[1])))


def _value(total):
    return total[1] if total[0] > 0 else -total[1]


def _levels(groups):
    if groups == 4:
        return [dict(enumerate(_STRASSEN))] * 2
    if groups == 2:
        return [dict(enumerate(_HOPCROFT_KERR))]

    def upper(terms):
        return tuple((sign, 0, i) for sign, f, i in terms if f != 1)

    return [{r: (upper(model), weight, upper(wide))
             for r, (model, weight, wide) in enumerate(_HOPCROFT_KERR)
             if upper(model) and upper(wide)}]


def _combination(terms, side, block):
    total = None
    for sign, a, b in terms:
        if side == _WEIGHT or a < 2:
            total = _accumulate(total, sign, block(a, b))
        else:
            total = _accumulate(total, *_accumulate(
                (sign, block(0, b)), -sign if side == _MODEL else sign, block(1, b)))
    return _value(total)


def _operands(levels, side, block):
    level, *inner = levels
    if not inner:
        block = functools.cache(block)
        return {r: functools.partial(_combination, product[side], side, block)
                for r, product in level.items()}
    operands = {}
    for r, product in level.items():
        def sub_block(a, b, terms=product[side]):
            return _combination(terms, side, lambda f, i: block(2 * f + a, 2 * i + b))

        for n, operand in _operands(inner, side, sub_block).items():
            operands[r * len(inner[0]) + n] = operand
    return operands


def _collect(levels, side, multiply, start, finish, partial_ref=None):
    level, *inner = levels
    terms = [term for product in level.values() for term in product[side]]
    left = {}
    for _, f, i in terms:
        left[f, i] = left.get((f, i), 0) + 1
    for i in sorted({i for _, f, i in terms if f == 2}):
        for f in range(2):
            left[f, i] = left.get((f, i), 0) + 1
    total = {}

    def add(r, f, i, sign, result):
        left[f, i] -= 1
        if f == 2:
            total[f, i] = _accumulate(total.get((f, i)), sign, result)
            if not left[f, i]:
                sign, result = total[f, i]
                add(r, 0, i, sign, result)
                add(r, 1, i, -sign if side == _MODEL else sign, result)
            return
        for (a, b), tile in result.items() if inner else [((0, 0), result)]:
            index = (2 * f + a, 2 * i + b) if inner else (f, i)
            key = f, i, a, b
            if key not in total:
                first = start(*index)
                before = None if first is None else (1, first)
            elif total[key][1] is None:
                before = total[key][0], partial_ref[index]
            else:
                before = total[key]
            total[key] = _accumulate(before, sign, tile)
            if not left[f, i]:
                finish(*index, _value(total[key]))
            elif inner and not any(g in (f, 2) and j == i for _, g, j in level[r + 1][side]):
                partial_ref[index] = total[key][1]
                total[key] = total[key][0], None

    for r, product in level.items():
        if inner:
            result = {}
            _collect(inner, side, lambda n: multiply(r * len(inner[0]) + n), lambda f, i: None,
                     lambda f, i, tile: result.update({(f, i): tile}))
        else:
            result = multiply(r)
        for sign, f, i in product[side]:
            add(r, f, i, sign, result)


@functools.cache
def _operand_slots(groups):
    used = {0: [0]}
    for level in _levels(groups):
        used = {r * len(level) + n: sorted({2 * i + j for i in tiles for _, _, j in terms})
                for r, tiles in used.items() for n, (terms, _, _) in level.items()}
    keys = [(r, tile) for r, tiles in used.items() for tile in [None] + tiles]
    return {key: slot for slot, key in enumerate(keys)}


class _SideJobs:
    def __init__(self, zero):
        self.zero, self.jobs, self.pace, self.due, self.count = zero, [], 0.0, 0.0, -1

    def add(self, source_ref=None, job=None, key=None):
        self.jobs.append((key, source_ref, job))

    def spread(self, products):
        self.pace = len(self.jobs) / products

    def finish(self, *keys):
        while self.jobs and (not keys or any(key in keys for key, _, _ in self.jobs)):
            _, ref, job = self.jobs.pop(0)
            if ref is not None:
                job()

    def dot(self, a, b):
        result = _dot(a, b)
        self.count += 1
        self.due = self.due + self.pace if self.jobs else 0.0
        while self.jobs and self.due >= 1.0:
            self.due -= 1.0
            _, ref, job = self.jobs.pop(0)
            if ref is None:
                continue
            rows = 32 // ref.dtype.itemsize
            first = self.count % 4 * (result.shape[0] // rows) // 4 * rows
            value = jax.lax.slice_in_dim(result, first, first + rows)
            index = (self.zero,) * (ref.ndim - 2) + (
                slice(ref.shape[-2] - rows, None), slice(0, _LANES))
            ref[index] = (pltpu.bitcast(value, ref.dtype) if ref.dtype == jnp.uint32
                          else value.astype(ref.dtype))
            job()
        return result

    def keep_in_memory(self, *refs):
        for ref in refs:
            ref[(self.zero,) * (ref.ndim - 2)] = jnp.zeros(ref.shape[-2:], ref.dtype)


def _store_rows(ref, f, first, x):
    rows = slice(first, first + x.shape[0])
    for i in range(_TILES):
        ref[f, i, rows] = x[:, i * _LANES:(i + 1) * _LANES]
    ref[f, _TILES, rows] = jnp.concatenate([x[:, _TILES * _LANES:]] * 2, axis=1)


def _load_rows(ref, f):
    rest = ref[f, _TILES]
    return jnp.concatenate(
        [ref[f, i] for i in range(_TILES)] + [rest[:, :_CHUNK] + rest[:, _CHUNK:]], axis=1)


def _combination_jobs(ref, groups, side, block, slots):
    def job(batch, rows):
        operands = _operands(_levels(groups), side, lambda a, b: block(a, b, rows))
        for r, slot in batch:
            ref[slot, rows] = jax.lax.convert_element_type(operands[r](), ref.dtype)

    batches = {}
    for r, slot in slots.items():
        key = r // len(_STRASSEN) if groups == 4 else sum(r >= cut for cut in _RUNS) % 4
        batches.setdefault(key, []).append((r, slot))
    step = _SLAB if groups > 1 else ref.shape[1]
    return [functools.partial(job, batch, slice(first, first + step))
            for batch in batches.values() for first in range(0, ref.shape[1], step)]


def _operand_jobs(ref, rows_ref, tile):
    groups = rows_ref.shape[0]
    return _combination_jobs(
        ref, groups, _MODEL, lambda f, i, rows: rows_ref[f, _TILES if i == tile else i, rows],
        {r: slot for (r, replaced), slot in _operand_slots(groups).items() if replaced == tile})


def _operand_loader(ref, groups, part):
    slots = _operand_slots(groups)
    rows = ref.shape[-2] * ref.dtype.itemsize // 4
    lanes = jax.lax.broadcasted_iota(jnp.int32, (rows, _LANES), 1)
    replaced = (lanes & _CHUNK) == (part & 1) * _CHUNK
    if isinstance(part, int):
        others = {r: slot for (r, tile), slot in slots.items() if tile == part // 2}
    else:
        others = {}
        for (r, tile), slot in slots.items():
            others[r] = slot if tile is None else jnp.where(part >> 1 == tile, slot, others[r])

    def load(r, *index):
        words = _load_words(ref, *index, slots[r, None])
        if r in others:
            words = jax.lax.select(replaced, _load_words(ref, *index, others[r]), words)
        return pltpu.bitcast(words, ref.dtype) if words.dtype != ref.dtype else words

    return load


def _attention_masks(n_mem, seg):
    size = n_mem + seg
    shape = (2 * size, _LANES)

    def position(axis):
        r = jax.lax.broadcasted_iota(jnp.int32, shape, axis)
        return r < size, jnp.where(r < seg, r + n_mem, jnp.where(r < size, r - seg, r - size))

    (first_i, i), (first_j, j) = position(0), position(1)
    same = (first_i == first_j) & (j < size)
    fill = jnp.where(same, _MASKED * _LOG2E, -jnp.inf).astype(jnp.float32)
    return same & ((i < n_mem) | (i >= j)), fill


def _start(copies):
    for copy in copies:
        copy.start()


def _wait(copies):
    for copy in copies:
        copy.wait()


def _kernel(xt_hbm, mem0_hbm, wq_hbm, wk_hbm, wv_hbm, wot_hbm, w1_hbm, w2t_hbm, w3_hbm,
            outt_hbm, mem0_ref, tile_ref, x_ref, early_ref, wqkv_ref, wo_ref, w1_ref, w2_ref,
            wplain_ref, stage_ref, stage_sem, mem_sem, tile_sem, *wide_refs, seg):
    d_model, n_tok = xt_hbm.shape
    n_mem = mem0_ref.shape[0]
    d_head = wq_hbm.shape[2]
    n_seg = n_tok // seg
    n_io = n_tok // _LANES
    size = n_mem + seg
    ahead = seg // 2
    width = _TILES * _LANES
    score_scale = d_head ** -0.5 * _LOG2E
    scales = {_W1: -_LOG2E, _W3: -1 / _LOG2E}
    f32, bf16, words = jnp.float32, jnp.bfloat16, jnp.uint32
    shared_slot = 6
    last_slots = {_W1: 2, _W2: shared_slot + 4, _W3: 5}
    wide_refs = list(wide_refs)
    side = _SideJobs(jax.lax.fori_loop(0, 3, lambda i, total: total - i, 3))

    def combine_weights(out_ref, source_ref, block, n_rows, n_tiles):
        wide_refs.reverse()
        wide_ref = wide_refs[0]

        def widen(first, tiles):
            rows = range(first, first + n_rows)
            for j, tile in [(j, block(rows, j)) for j in tiles]:
                wide_ref[first // _LANES, j, pl.ds(first % _LANES, n_rows)] = tile

        jobs = [functools.partial(widen, first, range(j, j + n_tiles))
                for j in range(0, _TILES, n_tiles) for first in range(0, width, n_rows)]
        before = []
        while side.jobs and side.jobs[-1][1] is wide_refs[1]:
            before.insert(0, side.jobs.pop())
        for n, job in enumerate(jobs):
            side.add(source_ref, job)
            if n_rows == _LANES:
                side.add()
            side.jobs += before[n * len(before) // len(jobs):(n + 1) * len(before) // len(jobs)]
        n_products = out_ref.shape[0]
        for job in _combination_jobs(out_ref, 2 if n_products == len(_HOPCROFT_KERR) else 4,
                                     _WEIGHT, lambda i, j, rows: wide_ref[i, j, rows],
                                     {r: r for r in range(n_products)}):
            side.add(wide_ref, job)

    def staged_rows(part, rows, packing):
        count = min(len(rows), _CHUNK)
        for first in rows[::count]:
            c, offset = divmod(first, _CHUNK)
            if isinstance(part, int):
                source = _PARTS if c == part else c
            else:
                source = jnp.where(part == c, _PARTS, c)
            yield _aligned(source * (_CHUNK // packing) + offset // packing, count // packing)

    def block_copies(m, part, slot, rows=pl.ds(0, d_model // 2)):
        src = (wot_hbm, w1_hbm, w2t_hbm, w3_hbm)[m].bitcast(words)
        dst, sem = stage_ref.at[slot], stage_sem.at[slot]
        if m == _WO:
            return [pltpu.make_async_copy(src.at[_TILES * part + j, rows],
                                          dst.at[rows, pl.ds(j * _LANES, _LANES)], sem)
                    for j in range(_TILES)]
        return [pltpu.make_async_copy(src.at[rows, _aligned(part * width, width)],
                                      dst.at[rows], sem)]

    def shared_copies(m):
        return [copy for c in range(_PARTS) for copy in block_copies(
            m, c, shared_slot + m, pl.ds(c * _CHUNK // 2, _CHUNK // 2))]

    def last_copies(m):
        return block_copies(m, _PARTS, last_slots[m])

    def staged(slot, part, rows, j):
        tile = pltpu.bitcast(jnp.concatenate(
            [stage_ref[slot, piece, j * _LANES:(j + 1) * _LANES]
             for piece in staged_rows(part, rows, 2)], axis=0), bf16)
        return (tile.T if len(rows) == _LANES else tile).astype(f32)

    def store_block(m, out_ref, block):
        if m in scales:
            combine_weights(out_ref, stage_ref, lambda *at: block(*at) * scales[m], _SLAB, _TILES)
        else:
            combine_weights(out_ref, stage_ref, block, _LANES, 1)

    def store_part(m, out_ref, part, slot):
        store_block(m, out_ref.at[part], lambda rows, j: (
            staged(slot, part, rows, j) - staged(shared_slot + m, part, rows, j)))

    def store_shared(m, out_ref):
        store_block(m, out_ref.at[out_ref.shape[0] - 1],
                    functools.partial(staged, shared_slot + m, _PARTS))

    def store_last(m, out_ref):
        part = {_W1: 0, _W3: 1, _W2: _PARTS}[m]

        def block(rows, j):
            own = staged(last_slots[m], part, rows, j)
            if m != _W2 and rows[0] // _CHUNK == 1 - part:
                other = _W1 + _W3 - m
                return own - staged(last_slots[other], part, rows, j) * (
                    scales[other] / scales[m])
            return own

        store_block(m, out_ref.at[_PARTS], block)
        for j in range(_TILES):
            rows = range(part * _CHUNK, (part + 1) * _CHUNK)
            wplain_ref[int(m == _W2), j, pl.ds(part % 2 * _CHUNK, _CHUNK)] = (staged(
                last_slots[m], _PARTS, rows, j) * scales.get(m, 1.0)).astype(bf16)

    def first_step_copies(t):
        return [copy for n in range(2) for copy in block_copies(_W3, 2 * t + n, 3 * (t & 1) + n)
                ] + (shared_copies(_W3) if t == 0 else last_copies(_W3) if t == 1
                     else last_copies(_W1) if t == 2 else [])

    def load_weights(early_in_ref, early_shared_ref, head_ref, head_sem, *rows_refs):
        n_early = n_io - 1
        products = len(_HOPCROFT_KERR)

        def pair_copies(w, part, slot, rows):
            src = (wq_hbm, wk_hbm, wv_hbm)[w].bitcast(words)
            return [pltpu.make_async_copy(src.at[rows, 2 * part + n, :],
                                          head_ref.at[slot, n, rows], head_sem.at[slot])
                    for n in range(2)]

        def head_copies(part, which=range(3)):
            return [copy for w in which
                    for copy in pair_copies(w, part, 3 * w + 2 * (part & 1), pl.ds(0, d_model))]

        def shared_head_copies(w):
            return [copy for c in range(_PARTS)
                    for copy in pair_copies(w, c, 3 * w + 1, pl.ds(c * _CHUNK, _CHUNK))]

        def part_copies(part):
            return [copy for m in range(3) for copy in block_copies(m, part, 3 * (part & 1) + m)]

        def head(slot, rows, j):
            pair = head_ref[slot, j // 2, rows, :]
            return pltpu.bitcast(pair & words(0xFFFF0000) if j % 2 else pair << 16, f32)

        def store_heads(w, part):
            def block(rows, j):
                rows = next(staged_rows(part, rows, 1))
                tile = head(3 * w + 2 * (part & 1), rows, j) - head(3 * w + 1, rows, j)
                return tile if w else tile * score_scale

            combine_weights(wqkv_ref.at[w, part], head_ref, block, _CHUNK // 2, 2)

        def store_shared_heads(w):
            @pl.loop(0, _LANES // _SLAB)
            def _(n):
                operands = _operands(_levels(2), _WEIGHT, lambda i, j: head(
                    3 * w + 1, _aligned(i * _LANES + n * _SLAB, _SLAB), j) * (
                        1.0 if w else score_scale))
                for r, operand in operands.items():
                    wqkv_ref[w, _PARTS, r, _aligned(n * _SLAB, _SLAB)] = operand().astype(bf16)

        def x_copies(first, last, sem):
            tiles = [(c + 1) % n_io for c in range(first, last)]
            return [pltpu.make_async_copy(xt_hbm.at[:, pl.ds(i * _LANES, _LANES)],
                                          tile_ref.at[i, :d_model], tile_sem.at[sem])
                    for i in tiles]

        def transpose_in(c):
            i = (c + 1) % n_io
            x_ref[i, :_LANES] = _load_packed(tile_ref, i, slice(0, d_model // 2)).T

        def normalize(c):
            for s in range(4):
                _store_rows(rows_refs[c % 3], s // 2, s % 2 * ahead,
                            _layernorm(x_ref[c + 1, s * seg:s * seg + ahead].astype(f32)))

        def fetch(c):
            transpose_in(c)
            if c < n_early:
                normalize(c)

        def prepare(c):
            rows_ref = rows_refs[c % 3]
            for n, job in enumerate(_operand_jobs(early_in_ref.at[c], rows_ref, None)):
                place = 2 * n if c + 2 >= n_early else len(side.jobs)
                side.jobs.insert(place, (c, rows_ref, job))

        def prepare_parts(c):
            for tile in range(_TILES):
                for job in _operand_jobs(early_in_ref.at[c], rows_refs[c % 3], tile):
                    side.add(rows_refs[c % 3], job)

        def project(w, part, c, operand):
            shared = isinstance(part, int) and part == _PARTS

            def keep(f, j, tile):
                early_shared_ref[w, c, f, j] = tile

            def store(f, j, tile):
                early_ref[2 * c + f, w, part, j] = tile.astype(bf16)

            _collect(_levels(2), _WIDE,
                     lambda r: side.dot(operand(r, c), _load_packed(wqkv_ref, w, part, r)),
                     lambda f, j: None if shared else early_shared_ref[w, c, f, j],
                     keep if shared else store)

        def project_shared(pending, first, last):
            operand = _operand_loader(early_in_ref, 2, _PARTS)
            ready = pending + [(w, c) for c in range(first, last) for w in range(3)]
            held = [(w, c) for w, c in ready if w and c + 2 >= last and last < n_early]
            fetch(first)
            side.add(tile_ref, functools.partial(fetch, first + 1))
            prepare(first)
            side.spread(len(pending) * products)
            for w, c in ready:
                if w == 0:
                    side.finish(c)
                    if c + 2 < last + (last == n_early):
                        side.add(tile_ref, functools.partial(fetch, c + 2))
                    if c + 1 < last:
                        prepare(c + 1)
                    prepare_parts(c)
                    if c + 3 == n_early:
                        store_heads(0, 0)
                    side.spread((3 * (n_early - c) - .5 if c + 3 >= n_early
                                 else 1 if (1, c) in held else 3) * products)
                if (w, c) not in held:
                    project(w, _PARTS, c, operand)
            side.finish()
            return held

        def project_part(part, which):
            operand = _operand_loader(early_in_ref, 2, part)
            side.count = 1
            side.spread((len(which) * n_early - .7) * products)
            for w in which:
                for c in range(n_early):
                    project(w, part, c, operand)
            side.finish()

        def store_parts(part, other):
            for m, out_ref in enumerate((wo_ref, w1_ref, w2_ref)):
                store_part(m, out_ref, part, 3 * (part & 1) + m)
                other(m)

        middle = n_io // 2
        _start(x_copies(0, 3, 0) + shared_head_copies(0))
        for w in range(3):
            head_ref[3 * w + 1, :, width:d_model] = jnp.zeros((2, _CHUNK, d_head), words)
        for m in range(4):
            stage_ref[shared_slot + m, width // 2:d_model // 2] = jnp.zeros(
                (_CHUNK // 2, width), words)
        side.keep_in_memory(early_in_ref, early_shared_ref)
        _wait(x_copies(0, 3, 0))
        _start(shared_head_copies(1))
        for c in range(3):
            transpose_in(c)
        copies = (shared_head_copies(2) + x_copies(3, middle, 0), x_copies(middle, middle + 3, 1),
                  x_copies(middle + 3, n_io, 1) + head_copies(0, [0]))
        for w in range(2):
            _wait(shared_head_copies(w))
            _start(copies[w])
            store_shared_heads(w)
            for c in range(3):
                if w:
                    prepare_parts(c)
                else:
                    normalize(c)
                    prepare(c)
            side.spread(2.5 * products)
            for c in range(3):
                side.finish(c)
                project(w, _PARTS, c, _operand_loader(early_in_ref, 2, _PARTS))
            side.finish()
        _wait(copies[0])
        _start(copies[2])
        store_shared_heads(2)
        held = project_shared([(2, c) for c in range(3)], 3, middle)
        _wait(copies[1] + copies[2])
        copies = part_copies(0) + [copy for m in range(3) for copy in shared_copies(m)]
        _start(head_copies(0, [1, 2]) + copies)
        project_shared(held, middle, n_early)
        _start(head_copies(1))
        _wait(head_copies(0, [1, 2]))
        store_heads(1, 0)
        store_heads(2, 0)
        project_part(0, [0])
        _start(part_copies(1) + head_copies(2))
        _wait(copies + head_copies(1))
        store_parts(0, lambda w: store_heads(w, 1))
        project_part(0, [1, 2])

        @pl.loop(1, _PARTS // 2, unroll=True)
        def _(n):
            for part in (2 * n - 1, 2 * n):
                _start(part_copies(part + 1))
                pl.when(part + 2 < _PARTS)(lambda: _start(head_copies(part + 2)))
                pl.when(part + 2 == _PARTS)(lambda: _start(last_copies(_W2)))
                _wait(part_copies(part) + head_copies(part + 1))
                store_parts(part, lambda w: store_heads(w, part + 1))
                project_part(part, range(3))

        _start(first_step_copies(0))
        _wait(part_copies(_PARTS - 1) + last_copies(_W2))
        store_parts(_PARTS - 1, lambda m: store_last(_W2, w2_ref) if m == _W1
                    else store_shared(m, w2_ref if m == _W2 else wo_ref))
        project_part(_PARTS - 1, range(3))

    def run_layers(w3_ref, pair_rows_ref, pair_in_ref, solo_rows_ref, solo_in_ref, ffn_rows_ref,
                   ffn_in_ref, attn_shared_ref, ffn_shared_ref, partial_ref, qkv_ref, heads_ref,
                   hidden_ref, attn_sum_ref, ffn_sum_ref, mem_ref, block_ref, second_ref):
        def segment(s):
            return s >> 2, _aligned((s & 3) * seg, seg)

        def transpose_out(i):
            tile_ref.bitcast(words)[i, :d_model // 2] = pltpu.bitcast(x_ref[i, :_LANES].T, words)

        def contract(groups, part, rows_ref, weight_ref, sum_ref, begun):
            operands = _operands(_levels(groups), _WIDE, lambda f, j: rows_ref[part, f, j])

            def targets(i):
                return [_TILES if 2 * i + half == part else i for half in range(2)]

            def start(f, i):
                low, high = (
                    sum_ref[f, n] if (n, half) in begun else None if groups < 4
                    else block_ref[f, :, n * _LANES:(n + 1) * _LANES]
                    for half, n in enumerate(targets(i)))
                if targets(i) == [i, i] and ((i, 0) in begun) == ((i, 1) in begun):
                    return low
                if low is None and high is None:
                    return None
                lanes = jax.lax.broadcasted_iota(jnp.int32, sum_ref.shape[-2:], 1)
                return jnp.where(lanes < _CHUNK, 0.0 if low is None else low,
                                 0.0 if high is None else high)

            def finish(f, i, tile):
                if targets(i) == [i, i]:
                    sum_ref[f, i] = tile
                else:
                    for half, n in enumerate(targets(i)):
                        lanes = slice(half * _CHUNK, (half + 1) * _CHUNK)
                        sum_ref[f, n, :, lanes] = tile[:, lanes]

            _collect(_levels(groups), _MODEL,
                     lambda r: side.dot(operands[r](), _load_packed(weight_ref, part, r)),
                     start, finish, partial_ref.at[part % 2])
            begun.update((n, half) for i in range(_TILES) for half, n in enumerate(targets(i)))

        def keep_and_add(ref, part, f, j, tile):
            total = ref.shape[0] - 1
            ref[part, f, j] = tile
            if 0 < part < _PARTS:
                ref[total, f, j] = ref[total if part > 1 else 0, f, j] + tile

        def project(groups, w, part):
            in_ref = pair_in_ref if groups == 2 else solo_in_ref
            rows = slice(0, in_ref.shape[1])
            side.finish(("P", None), ("P", part // 2))
            operand = _operand_loader(in_ref, groups, part)
            out_ref = qkv_ref.at[w, part % qkv_ref.shape[1]]
            done = {}

            def finish(f, j, tile):
                done[f, j] = tile
                if part == _PARTS:
                    attn_shared_ref[w, f, j, rows] = tile
                elif groups == 2 and (1 - f, j) in done:
                    upper, lower = done[0, j], done[1, j]
                    out_ref[j, :2 * size - ahead] = jnp.concatenate(
                        [upper[n_mem:n_mem + ahead], upper[:n_mem], lower[:n_mem],
                         upper[n_mem + ahead:], lower[n_mem:]], axis=0).astype(bf16)
                elif groups == 1 and (0, j ^ 1) in done:
                    a, b = done[0, j & ~1], done[0, j | 1]
                    out_ref[j | 1] = jnp.concatenate(
                        [a[n_mem:], a[:n_mem], b], axis=0).astype(bf16)

            _collect(_levels(groups), _WIDE,
                     lambda r: side.dot(operand(r), _load_packed(wqkv_ref, w, part, r)),
                     lambda f, j: attn_shared_ref[w, f, j, rows] if part < _PARTS else None,
                     finish)

        def projected(groups, t, place, w, head):
            part, j = divmod(head, _TILES)
            index = w, part % qkv_ref.shape[1], j
            if groups == 1:
                rows = [_load_words(qkv_ref, *index)]
            else:
                rows = [_load_words(early_ref, (t - _LAG) >> 1, w, part, j,
                                    pl.ds(place * ahead // 2, ahead // 2)),
                        _load_words(qkv_ref, *index, slice(0, size - ahead // 2))]
            if w == 1:
                rows.append(jnp.zeros((_CHUNK - size, d_head), words))
            return pltpu.bitcast(jnp.concatenate(rows, axis=0), bf16)

        def by_group(tile):
            return enumerate(tile[f * seg:(f + 1) * seg] for f in range(4))

        def expand(g):
            plain = 2 * _PARTS + 2
            if g == plain:
                x = jnp.concatenate([ffn_rows_ref[f, 0, :seg] for f in range(4)], axis=0)
                for j in range(_TILES):
                    for f, tile in by_group(_dot(x.astype(bf16), _load_packed(wplain_ref, 0, j))):
                        ffn_shared_ref[2, f, j] = tile
                return
            part, up = divmod(g if g < plain else g - 1, 2)
            chunk = up if part == _PARTS else min(part, _PARTS)
            side.finish(("G", None), ("G", chunk // 2))
            operand = _operand_loader(ffn_in_ref, 4, chunk)
            weight_ref = w3_ref if up else w1_ref

            def finish(f, j, tile):
                if part > _PARTS:
                    ffn_shared_ref[up, f, j] = tile
                elif up:
                    keep_and_add(hidden_ref, part, f, j, hidden_ref[part, f, j] * tile)
                else:
                    hidden_ref[part, f, j] = _scaled_silu(tile)

            _collect(_levels(4), _WIDE,
                     lambda r: side.dot(operand(r), _load_packed(weight_ref, part, r)),
                     lambda f, j: None if part > _PARTS else ffn_shared_ref[
                         2 if part == _PARTS else up, f, j],
                     finish, partial_ref.at[g % 2])

        def reduce(g, begun):
            if not begun:
                for f in range(4):
                    rest = block_ref[f, :, width:]
                    ffn_sum_ref[f, _TILES] = jnp.concatenate([rest, jnp.zeros_like(rest)], axis=1)
                begun.update([(_TILES, 0), (_TILES, 1)])
            if g < w2_ref.shape[0]:
                contract(4, g, hidden_ref, w2_ref, ffn_sum_ref, begun)
                return
            total = None
            for j in range(_TILES):
                rows = jnp.concatenate([hidden_ref[_PARTS, f, j] for f in range(4)], axis=0)
                total = _accumulate(total, 1, _dot(
                    _load_packed(wplain_ref, 1, j, slice(0, _CHUNK // 2)), rows.astype(bf16), 1))
            for f, tile in by_group(_value(total).T):
                ffn_sum_ref[f, _TILES, :, :_CHUNK] += tile

        def layer_input(t, place, layer):
            return x_ref[segment(t)].astype(f32) if layer == 0 else second_ref[place]

        def begin_step(t, place, layers):
            h = _layernorm(layer_input(t, place, layers[-1]))
            if len(layers) == 1:
                rows_ref, in_ref = solo_rows_ref, solo_in_ref
                _store_rows(rows_ref, 0, n_mem, h)
            else:
                rows_ref, in_ref, cut = pair_rows_ref, pair_in_ref, ahead // 2
                _store_rows(rows_ref, 0, n_mem, _layernorm(layer_input(t, place, 0)[ahead:]))
                _store_rows(rows_ref, 0, seg - cut, h[:cut])
                _store_rows(rows_ref, 1, n_mem, h[cut:])
            for f, layer in enumerate(layers):
                _store_rows(rows_ref, f, 0, mem_ref[layer])
            for tile in [None, *range(_TILES)]:
                for job in _operand_jobs(in_ref, rows_ref, tile):
                    side.add(rows_ref, job, ("P", tile))

        def close_step(t, place, layers):
            for f, layer in enumerate(layers):
                out = _load_rows(attn_sum_ref, f)
                mem_ref[layer] = out[:n_mem]
                index = 2 * layer + place if len(layers) == 2 else place
                block_ref[index] = layer_input(t, place, layer) + out[n_mem:]

        def run(order, layers=(), t=0, place=0):
            groups, first = len(layers), t
            visible, fill = _attention_masks(n_mem, seg)
            attn_begun, ffn_begun, probs = set(), set(), {}
            for name in order.split():
                stage, g = name[0], int(name[1:] or 0)
                if stage == "N":
                    begin_step(t, place, layers)
                elif stage == "P":
                    project(groups, g % 3, g // 3)
                elif stage == "S" and (groups == 2 or g % 2):
                    q, k = (projected(groups, t, place, w, g) for w in range(2))
                    s = jnp.where(visible, _dot(q, k, 1), fill)
                    p = jnp.exp2(s - jnp.max(s, axis=-1, keepdims=True))
                    inv = pltpu.reciprocal(jnp.sum(p, axis=-1, keepdims=True), approx=True)
                    probs[g] = p[:, :2 * size].astype(bf16), inv
                elif stage == "V" and (groups == 2 or g % 2):
                    o = _dot(probs[g][0], projected(groups, t, place, 2, g)) * probs[g][1]
                    halves = jnp.concatenate([o[seg:size], o[:seg]], axis=0), o[size:]
                    for f, half in enumerate(halves):
                        index = (f, g % _TILES) if groups == 2 else (0, g % _TILES - 1 + f)
                        keep_and_add(heads_ref, g // _TILES, *index, half)
                elif stage == "O":
                    contract(groups, g, heads_ref, wo_ref, attn_sum_ref, attn_begun)
                elif stage == "A":
                    close_step(t, place, layers)
                    t, place, attn_begun = t + 1, place + 1, set()
                elif stage == "M":
                    _store_rows(ffn_rows_ref, g, 0, _layernorm(block_ref[g]))
                elif stage == "F":
                    tile = g if g < _TILES else None
                    for job in _operand_jobs(ffn_in_ref, ffn_rows_ref, tile):
                        side.add(ffn_rows_ref, job, ("G", tile))
                elif stage == "G":
                    expand(g)
                elif stage == "D":
                    reduce(g, ffn_begun)
                elif stage == "E":
                    for s in range(2):
                        second_ref[g + s] = _load_rows(ffn_sum_ref, s)
                        x_ref[segment(jnp.maximum(first + g - 2 * _LAG, 0) + s)] = _load_rows(
                            ffn_sum_ref, 2 + s).astype(bf16)
                elif stage == "T":
                    side.add(x_ref, functools.partial(
                        transpose_out, jnp.maximum(first - 10, 0) >> 2))
                elif stage == "Z":
                    for _ in range(g):
                        side.add()
                elif stage == "W":
                    side.spread(g)
                elif stage == "X":
                    side.finish()

        side.keep_in_memory(pair_in_ref, solo_rows_ref, solo_in_ref, ffn_in_ref, attn_shared_ref,
                            ffn_shared_ref, partial_ref, qkv_ref, heads_ref, hidden_ref,
                            attn_sum_ref, ffn_sum_ref)
        attn_sum_ref[...] = jnp.zeros_like(attn_sum_ref)
        mem_copy.wait()
        mem_ref[0] = mem0_ref[...].astype(f32)
        for t in range(_LAG):
            run("N", (0,), t, t)
            _start(first_step_copies(t + 1) if t + 1 < _LAG else [mem_copy])
            _wait(first_step_copies(t))
            (store_shared, store_last)[t // 2](*((_W1, w1_ref), (_W3, w3_ref))[t % 2])
            for n in range(2):
                store_part(_W3, w3_ref, 2 * t + n, 3 * (t & 1) + n)
            run("W540 " + _ATTENTION + " X", (0,), t, t)
        mem_copy.wait()
        mem_ref[1] = mem0_ref[...].astype(f32)
        run(_SWIGLU)
        for s in range(2):
            second_ref[s] = _load_rows(ffn_sum_ref, s)
            ffn_sum_ref[s] = ffn_sum_ref[2 + s]
        run(2 * ("N W200 " + _ATTENTION + " ") + "M0 M2 M1 M3 G18 X", (0, 1), _LAG)

        @pl.loop(_LAG // 2 + 1, n_seg // 2)
        def _(b):
            run(_TWO_STEPS + " X", (0, 1), 2 * b)

        out_copies = [
            pltpu.make_async_copy(tile_ref.at[i, :d_model],
                                  outt_hbm.at[:, pl.ds(i * _LANES, _LANES)], tile_sem.at[0])
            for i in range(n_io)]
        _start(out_copies[:n_io - 2])
        run(_LAST_STEPS, (1,), n_seg)
        run("T W100 " + _SWIGLU, (), n_seg + 2)
        for s in range(_LAG):
            x_ref[segment(n_seg - _LAG + s)] = _load_rows(ffn_sum_ref, s).astype(bf16)
        transpose_out(n_io - 1)
        _start(out_copies[n_io - 2:])
        _wait(out_copies)

    spare = 8
    mem_copy = pltpu.make_async_copy(mem0_hbm, mem0_ref, mem_sem)
    mem_copy.start()
    pl.run_scoped(
        load_weights,
        pltpu.VMEM((n_io - 1, len(_operand_slots(2)), seg, _LANES), bf16),
        pltpu.VMEM((3, n_io - 1, 2, _TILES, seg, _LANES), f32),
        pltpu.VMEM((9, 2, d_model + spare, d_head), words),
        pltpu.SemaphoreType.DMA((9,)),
        *[pltpu.VMEM((2, _TILES + 1, seg + spare, _LANES), f32)] * 3)
    pl.run_scoped(
        run_layers,
        pltpu.VMEM(w1_ref.shape, bf16),
        pltpu.VMEM((2, _TILES + 1, seg + spare, _LANES), f32),
        pltpu.VMEM((len(_operand_slots(2)), seg, _LANES), bf16),
        pltpu.VMEM((1, _TILES + 1, size + spare, _LANES), f32),
        pltpu.VMEM((len(_operand_slots(1)), size, _LANES), f32),
        pltpu.VMEM((4, _TILES + 1, seg + spare, _LANES), f32),
        pltpu.VMEM((len(_operand_slots(4)), seg, _LANES), bf16),
        pltpu.VMEM((3, 2, _TILES, size, _LANES), f32),
        pltpu.VMEM((3, 4, _TILES, seg, _LANES), f32),
        pltpu.VMEM((2, 4, _TILES, seg, _LANES), f32),
        pltpu.VMEM((3, 3, _TILES, 2 * size, _LANES), bf16),
        pltpu.VMEM((_PARTS + 1, 2, _TILES, size, _LANES), f32),
        pltpu.VMEM((_PARTS + 2, 4, _TILES, seg, _LANES), f32),
        pltpu.VMEM((2, _TILES + 1, size, _LANES), f32),
        pltpu.VMEM((4, _TILES + 1, seg, _LANES), f32),
        pltpu.VMEM((2, n_mem, d_model), f32),
        pltpu.VMEM((4, seg, d_model), f32),
        pltpu.VMEM((4, seg, d_model), f32))


@functools.partial(jax.jit, static_argnames=("A_seg_len",))
def pallas_interleave_layers__memory_aug_recurrent_mem_tr__glu_gated_swiglu__prompt_kernel(
    A_x: jax.Array,
    A_mem0: jax.Array,
    A_Wq: jax.Array,
    A_Wk: jax.Array,
    A_Wv: jax.Array,
    A_Wo: jax.Array,
    A_seg_len: int,
    B_x: jax.Array,
    B_w1: jax.Array,
    B_w3: jax.Array,
    B_w2: jax.Array,
):
    del B_x
    _, n_tok, d_model = A_x.shape
    n_mem = A_mem0.shape[1]
    _, n_heads, d_head = A_Wq.shape
    seg = A_seg_len
    assert A_x.shape[0] == 1 and _LAG * seg == d_head == _LANES and 4 * n_mem == seg
    assert n_heads == _PARTS * _TILES and d_model == (_PARTS + 1) * _CHUNK
    assert B_w1.shape[1] == (_PARTS + 1) * _TILES * _LANES and n_tok == 16 * _LANES
    bf16 = jnp.bfloat16
    attn_blocks = (_PARTS + 1, len(_HOPCROFT_KERR), _LANES, _LANES)
    ffn_blocks = (_PARTS + 2, len(_STRASSEN) ** 2, _LANES, _LANES)
    hbm = pl.BlockSpec(memory_space=pltpu.HBM)
    out_t = pl.pallas_call(
        functools.partial(_kernel, seg=seg),
        out_shape=jax.ShapeDtypeStruct((d_model, n_tok), A_x.dtype),
        in_specs=[hbm] * 9,
        out_specs=hbm,
        scratch_shapes=[
            pltpu.VMEM((n_mem, d_model), bf16),
            pltpu.VMEM((n_tok // _LANES, d_model + _SLAB, _LANES), bf16),
            pltpu.VMEM((n_tok // _LANES, _LANES + _SLAB, d_model), bf16),
            pltpu.VMEM(((n_tok // seg - _LAG) // 2, 3, _PARTS, _TILES, seg, _LANES), bf16),
            pltpu.VMEM((3, *attn_blocks), bf16),
            pltpu.VMEM(attn_blocks, bf16),
            pltpu.VMEM(ffn_blocks, bf16),
            pltpu.VMEM(ffn_blocks, bf16),
            pltpu.VMEM((2, _TILES, _LANES, _LANES), bf16),
            pltpu.VMEM((11, (d_model + _SLAB) // 2, _TILES * _LANES), jnp.uint32),
            pltpu.SemaphoreType.DMA((11,)),
            pltpu.SemaphoreType.DMA(()),
            pltpu.SemaphoreType.DMA((2,)),
            *[pltpu.VMEM((_TILES, _TILES, _LANES + _SLAB // 2, _LANES), jnp.float32)] * 2,
        ],
        compiler_params=pltpu.CompilerParams(
            vmem_limit_bytes=127 * 1024 * 1024,
            flags={"XLA_TPU_FORCE_LP_LLO_SCHEDULER": True,
                   "XLA_TPU_EVENLY_DISTRIBUTE_CRITICAL_NODES": True}),
    )(A_x.reshape(n_tok, d_model).T, A_mem0.reshape(n_mem, d_model), A_Wq, A_Wk, A_Wv,
      A_Wo.transpose(0, 2, 1), B_w1, B_w2.T, B_w3)
    return out_t.T.reshape(A_x.shape)
```

```python
import functools
import math

import jax
import jax.numpy as jnp
import jax.experimental.pallas as pl
import jax.experimental.pallas.tpu as pltpu

_EPS = 1e-05
_MASKED = -1000000000.0
_LOG2E = math.log2(math.e)
_LANES = 128
_CHUNK = _LANES // 2
_SLAB = 16
_TILES = 4
_PARTS = 2 * _TILES
_LAG = 4
_WO, _W1, _W2, _W3 = range(4)
_MODEL, _WEIGHT, _WIDE = range(3)
_HOPCROFT_KERR = (
    (((1, 1, 2),), ((1, 2, 0), (1, 2, 2), (1, 2, 3), (-1, 1, 2)), ((1, 2, 2),)),
    (((1, 2, 2),), ((1, 2, 1), (1, 2, 2), (-1, 0, 2), (-1, 3, 2)), ((1, 0, 2),)),
    (((1, 0, 2), (1, 0, 3)), ((1, 2, 3),), ((-1, 2, 2), (1, 2, 3))),
    (((1, 2, 2), (1, 0, 3)), ((1, 2, 3), (1, 3, 2)), ((1, 2, 2), (-1, 1, 3))),
    (((1, 2, 2), (1, 2, 3)), ((1, 3, 2),), ((-1, 1, 2), (1, 1, 3))),
    (((1, 0, 0), (1, 0, 2)), ((1, 2, 0),), ((1, 2, 0), (-1, 2, 2))),
    (((1, 0, 0), (1, 2, 2)), ((1, 0, 2), (1, 2, 0)), ((-1, 1, 0), (1, 2, 2))),
    (((1, 2, 0), (1, 2, 2)), ((1, 0, 2),), ((1, 1, 0), (-1, 1, 2))),
    (((1, 0, 1), (1, 0, 2)), ((1, 2, 1),), ((1, 0, 1), (-1, 0, 2))),
    (((1, 0, 1), (1, 1, 2)), ((1, 1, 2), (1, 2, 1)), ((1, 1, 1), (1, 0, 2))),
    (((1, 1, 1), (1, 1, 2)), ((1, 1, 2),), ((-1, 1, 1), (1, 1, 2))),
    (((1, 1, 1), (1, 1, 3)), ((1, 0, 3), (-1, 1, 3)), ((1, 2, 1), (-1, 2, 3))),
    (((1, 0, 0), (1, 0, 1), (1, 0, 3)), ((1, 0, 3),), ((1, 2, 1), (-1, 2, 0), (1, 2, 3))),
    (((1, 2, 0), (1, 2, 1), (1, 0, 3)), ((1, 0, 3), (1, 3, 0)),
     ((1, 2, 0), (-1, 2, 1), (-1, 1, 3))),
    (((1, 2, 0), (1, 2, 1), (1, 2, 3)), ((1, 3, 0),), ((1, 1, 1), (-1, 1, 0), (1, 1, 3))),
    (((1, 1, 3),), ((1, 0, 3), (-1, 1, 3), (1, 3, 0), (1, 3, 2), (1, 3, 3)), ((1, 1, 3),)),
    (((1, 2, 1), (1, 2, 3)), ((1, 3, 0), (1, 3, 1)), ((1, 0, 1), (-1, 0, 3))),
    (((1, 1, 3), (-1, 2, 1)), ((1, 3, 0), (1, 3, 1), (-1, 0, 3), (1, 1, 3)),
     ((1, 2, 1), (-1, 0, 3))),
    (((1, 0, 3),), ((1, 3, 0), (1, 3, 1), (-1, 0, 3), (-1, 2, 3), (1, 3, 3)), ((1, 0, 3),)),
    (((1, 1, 0), (1, 1, 1)), ((1, 0, 3), (1, 1, 0)), ((1, 2, 0), (-1, 2, 1))),
    (((1, 2, 1), (-1, 1, 0)), ((1, 0, 1), (1, 1, 0)), ((1, 0, 0), (-1, 2, 1))),
    (((1, 0, 1),), ((1, 1, 0), (1, 1, 1), (1, 1, 3), (-1, 0, 3), (-1, 2, 1)), ((1, 2, 1),)),
    (((1, 2, 0), (1, 2, 1)), ((1, 0, 1), (1, 3, 0)), ((-1, 0, 0), (1, 0, 1))),
    (((1, 2, 1),), ((1, 3, 0), (1, 3, 1), (1, 0, 1), (-1, 1, 1), (-1, 1, 2)), ((1, 1, 1),)),
    (((1, 0, 0),), ((1, 0, 0), (1, 0, 1), (-1, 2, 0)), ((1, 0, 0),)),
    (((1, 1, 0),), ((1, 0, 0), (1, 0, 2), (-1, 1, 0)), ((1, 1, 0),)),
)
_RUNS = (5, 11, 19, 24, 24)
_STRASSEN = (
    (((-1, 2, 0),), ((1, 0, 0), (1, 0, 1)), ((1, 1, 1),)),
    (((1, 1, 0), (1, 1, 1)), ((1, 0, 0),), ((1, 1, 0), (-1, 1, 1))),
    (((1, 1, 1),), ((1, 1, 0), (-1, 0, 0)), ((1, 2, 0),)),
    (((1, 0, 0), (1, 1, 1)), ((1, 0, 0), (1, 1, 1)), ((1, 0, 0), (1, 1, 1))),
    (((1, 0, 0),), ((1, 0, 1), (-1, 1, 1)), ((1, 2, 1),)),
    (((1, 0, 0), (1, 0, 1)), ((1, 1, 1),), ((-1, 0, 0), (1, 0, 1))),
    (((1, 2, 1),), ((1, 1, 0), (1, 1, 1)), ((1, 0, 0),)),
)
_ATTENTION = (
    "P24 P25 P26 P0 P1 P2 S0 S1 S2 S3 P3 P4 V0 V1 V2 V3 P5 S4 S5 S6 S7 O0 P6 P7 V4 V5 V6 V7 "
    "P8 S8 S9 S10 S11 O1 P9 P10 V8 V9 V10 V11 P11 S12 S13 S14 S15 O2 P12 P13 V12 V13 V14 V15 "
    "P14 S16 S17 S18 S19 O3 P15 P16 V16 V17 V18 V19 P17 S20 S21 S22 S23 P18 P19 V20 V21 V22 "
    "V23 P20 S24 S25 S26 S27 P21 P22 V24 V25 V26 V27 P23 S28 S29 S30 S31 O4 V28 V29 V30 V31 "
    "O5 O6 O7 O8 A")
_SWIGLU = (
    "M0 M1 M2 M3 F4 X F0 F1 F2 F3 W500 G18 G19 G20 G16 G17 G0 D8 D10 G1 G2 D0 G3 G4 D1 G5 G6 "
    "D2 G7 G8 D3 G9 G10 D4 G11 G12 G13 G14 D5 G15 D6 D7 D9")
_TWO_STEPS = (
    "E F4 X N Z11 G19 F0 W250 G20 P24 P25 P26 P0 G16 P1 P2 G17 S0 S1 S2 S3 P3 P4 V0 V1 V2 V3 "
    "P5 G0 S4 S5 S6 S7 O0 G1 P6 P7 V4 V5 V6 V7 P8 D8 S8 S9 S10 S11 O1 F1 W200 G2 P9 P10 V8 V9 "
    "V10 V11 P11 S12 S13 S14 S15 O2 D0 P12 P13 V12 V13 V14 V15 P14 S16 S17 S18 S19 O3 G3 P15 "
    "P16 V16 V17 V18 V19 P17 S20 S21 S22 S23 O4 P18 G4 P19 V20 V21 V22 V23 P20 S24 S25 S26 "
    "S27 O5 F2 W160 D1 P21 P22 V24 V25 V26 V27 P23 S28 S29 S30 S31 O6 G5 V28 V29 V30 V31 G6 "
    "O7 O8 A Z4 N W200 D2 G7 D3 P24 P25 P26 G8 P0 P1 P2 S0 S1 S2 S3 P3 P4 V0 V1 V2 V3 P5 G9 "
    "S4 S5 S6 S7 O0 F3 W120 P6 G10 P7 V4 V5 V6 V7 P8 S8 S9 S10 S11 O1 D4 P10 P9 V8 V9 V10 V11 "
    "P11 S12 S13 S14 S15 O2 G11 P12 P13 V12 V13 V14 V15 P14 S16 S17 S18 S19 O3 G12 P15 P16 "
    "V16 V17 V18 V19 P17 S20 S21 S22 S23 O4 P18 P19 V20 V21 V22 V23 P20 S24 S25 S26 S27 O5 "
    "G14 G13 P21 P22 V24 V25 V26 V27 P23 S28 S29 S30 S31 O6 D5 M0 V28 V29 V30 V31 G15 O7 O8 "
    "M2 D9 A D10 M3 D6 M1 D7 G18")
_LAST_STEPS = (
    "E F4 X N F0 F1 W400 G19 G20 " + _ATTENTION.replace("O0", "O0 G16 G17 G0 D8 G1 G2 D0 G3")
    + " N F2 F3 W450 G4 D1 D10 G5 G6 D2 G7 G8 D3 G9 G10 D4 G11 G12 G13 G14 D5 G15 D6 D7 D9 E2 "
    + _ATTENTION + 2 * (" N W200 " + _ATTENTION))


def _layernorm(x):
    m = jnp.mean(x, axis=-1, keepdims=True)
    d = x - m
    v = jnp.mean(d * d, axis=-1, keepdims=True)
    return d * jax.lax.rsqrt(v + _EPS)


def _scaled_silu(x):
    return x * pltpu.reciprocal(1.0 + jnp.exp2(x), approx=True)


def _dot(a, b, axis=0):
    return jax.lax.dot_general(a, b, (((1,), (axis,)), ((), ())),
                               preferred_element_type=jnp.float32)


def _load_words(ref, *index):
    return ref[index] if ref.dtype == jnp.float32 else ref.bitcast(jnp.uint32)[index]


def _load_packed(ref, *index):
    return pltpu.bitcast(_load_words(ref, *index), ref.dtype)


def _aligned(first, size):
    return pl.ds(first if isinstance(first, int) else pl.multiple_of(first, size), size)


def _accumulate(total, sign, value):
    if total is None:
        return sign, value
    if total[0] == sign:
        return sign, jax.lax.add(total[1], value)
    return 1, jax.lax.sub(*((total[1], value) if sign < 0 else (value, total[1])))


def _value(total):
    return total[1] if total[0] > 0 else -total[1]


def _levels(groups):
    if groups == 4:
        return [dict(enumerate(_STRASSEN))] * 2
    if groups == 2:
        return [dict(enumerate(_HOPCROFT_KERR))]

    def upper(terms):
        return tuple((sign, 0, i) for sign, f, i in terms if f != 1)

    return [{r: (upper(model), weight, upper(wide))
             for r, (model, weight, wide) in enumerate(_HOPCROFT_KERR)
             if upper(model) and upper(wide)}]


def _combination(terms, side, block):
    total = None
    for sign, a, b in terms:
        if side == _WEIGHT or a < 2:
            total = _accumulate(total, sign, block(a, b))
        else:
            total = _accumulate(total, *_accumulate(
                (sign, block(0, b)), -sign if side == _MODEL else sign, block(1, b)))
    return _value(total)


def _operands(levels, side, block):
    level, *inner = levels
    if not inner:
        block = functools.cache(block)
        return {r: functools.partial(_combination, product[side], side, block)
                for r, product in level.items()}
    operands = {}
    for r, product in level.items():
        def sub_block(a, b, terms=product[side]):
            return _combination(terms, side, lambda f, i: block(2 * f + a, 2 * i + b))

        for n, operand in _operands(inner, side, sub_block).items():
            operands[r * len(inner[0]) + n] = operand
    return operands


def _collect(levels, side, multiply, start, finish, partial_ref=None):
    level, *inner = levels
    terms = [term for product in level.values() for term in product[side]]
    left = {}
    for _, f, i in terms:
        left[f, i] = left.get((f, i), 0) + 1
    for i in sorted({i for _, f, i in terms if f == 2}):
        for f in range(2):
            left[f, i] = left.get((f, i), 0) + 1
    total = {}

    def add(r, f, i, sign, result):
        left[f, i] -= 1
        if f == 2:
            total[f, i] = _accumulate(total.get((f, i)), sign, result)
            if not left[f, i]:
                sign, result = total[f, i]
                add(r, 0, i, sign, result)
                add(r, 1, i, -sign if side == _MODEL else sign, result)
            return
        for (a, b), tile in result.items() if inner else [((0, 0), result)]:
            index = (2 * f + a, 2 * i + b) if inner else (f, i)
            key = f, i, a, b
            if key not in total:
                first = start(*index)
                before = None if first is None else (1, first)
            elif total[key][1] is None:
                before = total[key][0], partial_ref[index]
            else:
                before = total[key]
            total[key] = _accumulate(before, sign, tile)
            if not left[f, i]:
                finish(*index, _value(total[key]))
            elif inner and not any(g in (f, 2) and j == i for _, g, j in level[r + 1][side]):
                partial_ref[index] = total[key][1]
                total[key] = total[key][0], None

    for r, product in level.items():
        if inner:
            result = {}
            _collect(inner, side, lambda n: multiply(r * len(inner[0]) + n), lambda f, i: None,
                     lambda f, i, tile: result.update({(f, i): tile}))
        else:
            result = multiply(r)
        for sign, f, i in product[side]:
            add(r, f, i, sign, result)


@functools.cache
def _operand_slots(groups):
    used = {0: [0]}
    for level in _levels(groups):
        used = {r * len(level) + n: sorted({2 * i + j for i in tiles for _, _, j in terms})
                for r, tiles in used.items() for n, (terms, _, _) in level.items()}
    keys = [(r, tile) for r, tiles in used.items() for tile in [None] + tiles]
    return {key: slot for slot, key in enumerate(keys)}


class _SideJobs:
    def __init__(self, zero):
        self.zero, self.jobs, self.pace, self.due, self.count = zero, [], 0.0, 0.0, -1

    def add(self, source_ref=None, job=None, key=None):
        self.jobs.append((key, source_ref, job))

    def spread(self, products):
        self.pace = len(self.jobs) / products

    def finish(self, *keys):
        while self.jobs and (not keys or any(key in keys for key, _, _ in self.jobs)):
            _, ref, job = self.jobs.pop(0)
            if ref is not None:
                job()

    def dot(self, a, b):
        result = _dot(a, b)
        self.count += 1
        self.due = self.due + self.pace if self.jobs else 0.0
        while self.jobs and self.due >= 1.0:
            self.due -= 1.0
            _, ref, job = self.jobs.pop(0)
            if ref is None:
                continue
            rows = 32 // ref.dtype.itemsize
            first = self.count % 4 * (result.shape[0] // rows) // 4 * rows
            value = jax.lax.slice_in_dim(result, first, first + rows)
            index = (self.zero,) * (ref.ndim - 2) + (
                slice(ref.shape[-2] - rows, None), slice(0, _LANES))
            ref[index] = (pltpu.bitcast(value, ref.dtype) if ref.dtype == jnp.uint32
                          else value.astype(ref.dtype))
            job()
        return result

    def keep_in_memory(self, *refs):
        for ref in refs:
            ref[(self.zero,) * (ref.ndim - 2)] = jnp.zeros(ref.shape[-2:], ref.dtype)


def _store_rows(ref, f, first, x):
    rows = slice(first, first + x.shape[0])
    for i in range(_TILES):
        ref[f, i, rows] = x[:, i * _LANES:(i + 1) * _LANES]
    ref[f, _TILES, rows] = jnp.concatenate([x[:, _TILES * _LANES:]] * 2, axis=1)


def _load_rows(ref, f):
    rest = ref[f, _TILES]
    return jnp.concatenate(
        [ref[f, i] for i in range(_TILES)] + [rest[:, :_CHUNK] + rest[:, _CHUNK:]], axis=1)


def _combination_jobs(ref, groups, side, block, slots):
    def job(batch, rows):
        operands = _operands(_levels(groups), side, lambda a, b: block(a, b, rows))
        for r, slot in batch:
            ref[slot, rows] = jax.lax.convert_element_type(operands[r](), ref.dtype)

    batches = {}
    for r, slot in slots.items():
        key = r // len(_STRASSEN) if groups == 4 else sum(r >= cut for cut in _RUNS) % 4
        batches.setdefault(key, []).append((r, slot))
    step = _SLAB if groups > 1 else ref.shape[1]
    return [functools.partial(job, batch, slice(first, first + step))
            for batch in batches.values() for first in range(0, ref.shape[1], step)]


def _operand_jobs(ref, rows_ref, tile):
    groups = rows_ref.shape[0]
    return _combination_jobs(
        ref, groups, _MODEL, lambda f, i, rows: rows_ref[f, _TILES if i == tile else i, rows],
        {r: slot for (r, replaced), slot in _operand_slots(groups).items() if replaced == tile})


def _operand_loader(ref, groups, part):
    slots = _operand_slots(groups)
    rows = ref.shape[-2] * ref.dtype.itemsize // 4
    lanes = jax.lax.broadcasted_iota(jnp.int32, (rows, _LANES), 1)
    replaced = (lanes & _CHUNK) == (part & 1) * _CHUNK
    if isinstance(part, int):
        others = {r: slot for (r, tile), slot in slots.items() if tile == part // 2}
    else:
        others = {}
        for (r, tile), slot in slots.items():
            others[r] = slot if tile is None else jnp.where(part >> 1 == tile, slot, others[r])

    def load(r, *index):
        words = _load_words(ref, *index, slots[r, None])
        if r in others:
            words = jax.lax.select(replaced, _load_words(ref, *index, others[r]), words)
        return pltpu.bitcast(words, ref.dtype) if words.dtype != ref.dtype else words

    return load


def _attention_masks(n_mem, seg):
    size = n_mem + seg
    shape = (2 * size, _LANES)

    def position(axis):
        r = jax.lax.broadcasted_iota(jnp.int32, shape, axis)
        return r < size, jnp.where(r < seg, r + n_mem, jnp.where(r < size, r - seg, r - size))

    (first_i, i), (first_j, j) = position(0), position(1)
    same = (first_i == first_j) & (j < size)
    fill = jnp.where(same, _MASKED * _LOG2E, -jnp.inf).astype(jnp.float32)
    return same & ((i < n_mem) | (i >= j)), fill


def _start(copies):
    for copy in copies:
        copy.start()


def _wait(copies):
    for copy in copies:
        copy.wait()


def _kernel(xt_hbm, mem0_hbm, wq_hbm, wk_hbm, wv_hbm, wot_hbm, w1_hbm, w2t_hbm, w3_hbm,
            outt_hbm, mem0_ref, tile_ref, x_ref, early_ref, wqkv_ref, wo_ref, w1_ref, w2_ref,
            wplain_ref, stage_ref, stage_sem, mem_sem, tile_sem, *wide_refs, seg):
    d_model, n_tok = xt_hbm.shape
    n_mem = mem0_ref.shape[0]
    d_head = wq_hbm.shape[2]
    n_seg = n_tok // seg
    n_io = n_tok // _LANES
    size = n_mem + seg
    ahead = seg // 2
    width = _TILES * _LANES
    score_scale = d_head ** -0.5 * _LOG2E
    scales = {_W1: -_LOG2E, _W3: -1 / _LOG2E}
    f32, bf16, words = jnp.float32, jnp.bfloat16, jnp.uint32
    shared_slot = 6
    last_slots = {_W1: 2, _W2: shared_slot + 4, _W3: 5}
    wide_refs = list(wide_refs)
    side = _SideJobs(jax.lax.fori_loop(0, 3, lambda i, total: total - i, 3))

    def combine_weights(out_ref, source_ref, block, n_rows, n_tiles):
        wide_refs.reverse()
        wide_ref = wide_refs[0]

        def widen(first, tiles):
            rows = range(first, first + n_rows)
            for j, tile in [(j, block(rows, j)) for j in tiles]:
                wide_ref[first // _LANES, j, pl.ds(first % _LANES, n_rows)] = tile

        jobs = [functools.partial(widen, first, range(j, j + n_tiles))
                for j in range(0, _TILES, n_tiles) for first in range(0, width, n_rows)]
        before = []
        while side.jobs and side.jobs[-1][1] is wide_refs[1]:
            before.insert(0, side.jobs.pop())
        for n, job in enumerate(jobs):
            side.add(source_ref, job)
            if n_rows == _LANES:
                side.add()
            side.jobs += before[n * len(before) // len(jobs):(n + 1) * len(before) // len(jobs)]
        n_products = out_ref.shape[0]
        for job in _combination_jobs(out_ref, 2 if n_products == len(_HOPCROFT_KERR) else 4,
                                     _WEIGHT, lambda i, j, rows: wide_ref[i, j, rows],
                                     {r: r for r in range(n_products)}):
            side.add(wide_ref, job)

    def staged_rows(part, rows, packing):
        count = min(len(rows), _CHUNK)
        for first in rows[::count]:
            c, offset = divmod(first, _CHUNK)
            if isinstance(part, int):
                source = _PARTS if c == part else c
            else:
                source = jnp.where(part == c, _PARTS, c)
            yield _aligned(source * (_CHUNK // packing) + offset // packing, count // packing)

    def block_copies(m, part, slot, rows=pl.ds(0, d_model // 2)):
        src = (wot_hbm, w1_hbm, w2t_hbm, w3_hbm)[m].bitcast(words)
        dst, sem = stage_ref.at[slot], stage_sem.at[slot]
        if m == _WO:
            return [pltpu.make_async_copy(src.at[_TILES * part + j, rows],
                                          dst.at[rows, pl.ds(j * _LANES, _LANES)], sem)
                    for j in range(_TILES)]
        return [pltpu.make_async_copy(src.at[rows, _aligned(part * width, width)],
                                      dst.at[rows], sem)]

    def shared_copies(m):
        return [copy for c in range(_PARTS) for copy in block_copies(
            m, c, shared_slot + m, pl.ds(c * _CHUNK // 2, _CHUNK // 2))]

    def last_copies(m):
        return block_copies(m, _PARTS, last_slots[m])

    def staged(slot, part, rows, j):
        tile = pltpu.bitcast(jnp.concatenate(
            [stage_ref[slot, piece, j * _LANES:(j + 1) * _LANES]
             for piece in staged_rows(part, rows, 2)], axis=0), bf16)
        return (tile.T if len(rows) == _LANES else tile).astype(f32)

    def store_block(m, out_ref, block):
        if m in scales:
            combine_weights(out_ref, stage_ref, lambda *at: block(*at) * scales[m], _SLAB, _TILES)
        else:
            combine_weights(out_ref, stage_ref, block, _LANES, 1)

    def store_part(m, out_ref, part, slot):
        store_block(m, out_ref.at[part], lambda rows, j: (
            staged(slot, part, rows, j) - staged(shared_slot + m, part, rows, j)))

    def store_shared(m, out_ref):
        store_block(m, out_ref.at[out_ref.shape[0] - 1],
                    functools.partial(staged, shared_slot + m, _PARTS))

    def store_last(m, out_ref):
        part = {_W1: 0, _W3: 1, _W2: _PARTS}[m]

        def block(rows, j):
            own = staged(last_slots[m], part, rows, j)
            if m != _W2 and rows[0] // _CHUNK == 1 - part:
                other = _W1 + _W3 - m
                return own - staged(last_slots[other], part, rows, j) * (
                    scales[other] / scales[m])
            return own

        store_block(m, out_ref.at[_PARTS], block)
        for j in range(_TILES):
            rows = range(part * _CHUNK, (part + 1) * _CHUNK)
            wplain_ref[int(m == _W2), j, pl.ds(part % 2 * _CHUNK, _CHUNK)] = (staged(
                last_slots[m], _PARTS, rows, j) * scales.get(m, 1.0)).astype(bf16)

    def first_step_copies(t):
        return [copy for n in range(2) for copy in block_copies(_W3, 2 * t + n, 3 * (t & 1) + n)
                ] + (shared_copies(_W3) + block_copies(_W1, 0, 2) if t == 0
                     else last_copies(_W3) if t == 1 else last_copies(_W1) if t == 2 else [])

    def load_weights(early_in_ref, early_shared_ref, head_ref, head_sem, *rows_refs):
        n_early = n_io - 1
        products = len(_HOPCROFT_KERR)

        def pair_copies(w, part, slot, rows):
            src = (wq_hbm, wk_hbm, wv_hbm)[w].bitcast(words)
            return [pltpu.make_async_copy(src.at[rows, 2 * part + n, :],
                                          head_ref.at[slot, n, rows], head_sem.at[slot])
                    for n in range(2)]

        def head_copies(part, which=range(3)):
            return [copy for w in which
                    for copy in pair_copies(w, part, 3 * w + 2 * (part & 1), pl.ds(0, d_model))]

        def shared_head_copies(w):
            return [copy for c in range(_PARTS)
                    for copy in pair_copies(w, c, 3 * w + 1, pl.ds(c * _CHUNK, _CHUNK))]

        def part_copies(part, which=range(3)):
            return [copy for m in which for copy in block_copies(m, part, 3 * (part & 1) + m)]

        def head(slot, rows, j):
            pair = head_ref[slot, j // 2, rows, :]
            return pltpu.bitcast(pair & words(0xFFFF0000) if j % 2 else pair << 16, f32)

        def store_heads(w, part):
            def block(rows, j):
                rows = next(staged_rows(part, rows, 1))
                tile = head(3 * w + 2 * (part & 1), rows, j) - head(3 * w + 1, rows, j)
                return tile if w else tile * score_scale

            combine_weights(wqkv_ref.at[w, part], head_ref, block, _CHUNK // 2, 2)

        def store_shared_heads(w):
            @pl.loop(0, _LANES // _SLAB)
            def _(n):
                operands = _operands(_levels(2), _WEIGHT, lambda i, j: head(
                    3 * w + 1, _aligned(i * _LANES + n * _SLAB, _SLAB), j) * (
                        1.0 if w else score_scale))
                for r, operand in operands.items():
                    wqkv_ref[w, _PARTS, r, _aligned(n * _SLAB, _SLAB)] = operand().astype(bf16)

        def x_copies(first, last, sem):
            tiles = [(c + 1) % n_io for c in range(first, last)]
            return [pltpu.make_async_copy(xt_hbm.at[:, pl.ds(i * _LANES, _LANES)],
                                          tile_ref.at[i, :d_model], tile_sem.at[sem])
                    for i in tiles]

        def transpose_in(c):
            i = (c + 1) % n_io
            x_ref[i, :_LANES] = _load_packed(tile_ref, i, slice(0, d_model // 2)).T

        def normalize(c):
            for s in range(4):
                _store_rows(rows_refs[c % 3], s // 2, s % 2 * ahead,
                            _layernorm(x_ref[c + 1, s * seg:s * seg + ahead].astype(f32)))

        def fetch(c):
            transpose_in(c)
            if c < n_early:
                normalize(c)

        def prepare(c):
            rows_ref = rows_refs[c % 3]
            for n, job in enumerate(_operand_jobs(early_in_ref.at[c], rows_ref, None)):
                place = 2 * n if c + 2 >= n_early else len(side.jobs)
                side.jobs.insert(place, (c, rows_ref, job))

        def prepare_parts(c):
            for tile in range(_TILES):
                for job in _operand_jobs(early_in_ref.at[c], rows_refs[c % 3], tile):
                    side.add(rows_refs[c % 3], job)

        def project(w, part, c, operand):
            shared = isinstance(part, int) and part == _PARTS

            def keep(f, j, tile):
                early_shared_ref[w, c, f, j] = tile

            def store(f, j, tile):
                early_ref[2 * c + f, w, part, j] = tile.astype(bf16)

            _collect(_levels(2), _WIDE,
                     lambda r: side.dot(operand(r, c), _load_packed(wqkv_ref, w, part, r)),
                     lambda f, j: None if shared else early_shared_ref[w, c, f, j],
                     keep if shared else store)

        def project_shared(pending, first, last):
            operand = _operand_loader(early_in_ref, 2, _PARTS)
            ready = pending + [(w, c) for c in range(first, last) for w in range(3)]
            held = [(w, c) for w, c in ready if w and c + 2 >= last and last < n_early]
            fetch(first)
            side.add(tile_ref, functools.partial(fetch, first + 1))
            prepare(first)
            side.spread(len(pending) * products)
            for w, c in ready:
                if w == 0:
                    side.finish(c)
                    if c + 2 < last + (last == n_early):
                        side.add(tile_ref, functools.partial(fetch, c + 2))
                    if c + 1 < last:
                        prepare(c + 1)
                    prepare_parts(c)
                    if c + 3 == n_early:
                        store_heads(0, 0)
                    side.spread((3 * (n_early - c) - .5 if c + 3 >= n_early
                                 else 1 if (1, c) in held else 3) * products)
                if (w, c) not in held:
                    project(w, _PARTS, c, operand)
            side.finish()
            return held

        def project_part(part, which):
            operand = _operand_loader(early_in_ref, 2, part)
            side.count = 1
            side.spread((len(which) * n_early - .7) * products)
            for w in which:
                for c in range(n_early):
                    project(w, part, c, operand)
            side.finish()

        def store_parts(part, other, which=range(3)):
            for m, out_ref in enumerate((wo_ref, w1_ref, w2_ref)):
                if m in which:
                    store_part(m, out_ref, part, 3 * (part & 1) + m)
                other(m)

        middle = n_io // 2
        _start(x_copies(0, 3, 0) + shared_head_copies(0))
        for w in range(3):
            head_ref[3 * w + 1, :, width:d_model] = jnp.zeros((2, _CHUNK, d_head), words)
        for m in range(4):
            stage_ref[shared_slot + m, width // 2:d_model // 2] = jnp.zeros(
                (_CHUNK // 2, width), words)
        side.keep_in_memory(early_in_ref, early_shared_ref)
        _wait(x_copies(0, 3, 0))
        _start(shared_head_copies(1) + shared_head_copies(2))
        for c in range(3):
            transpose_in(c)
        copies = (x_copies(3, middle, 0), x_copies(middle, middle + 1, 1),
                  x_copies(middle + 1, n_io, 1) + head_copies(0, [0]))
        for w in range(2):
            _wait(shared_head_copies(w))
            _start(copies[w])
            store_shared_heads(w)
            for c in range(3):
                if w:
                    prepare_parts(c)
                else:
                    normalize(c)
                    prepare(c)
            side.spread(2.5 * products)
            for c in range(3):
                side.finish(c)
                project(w, _PARTS, c, _operand_loader(early_in_ref, 2, _PARTS))
            side.finish()
        _wait(shared_head_copies(2) + copies[0])
        _start(copies[2])
        store_shared_heads(2)
        held = project_shared([(2, c) for c in range(3)], 3, middle)
        _wait(copies[1] + copies[2])
        copies = part_copies(0, (_WO, _W2)) + shared_copies(_WO) + shared_copies(_W2)
        _start(head_copies(0, [1, 2]) + copies + head_copies(1))
        project_shared(held, middle, n_early)
        _wait(head_copies(0, [1, 2]))
        _start(shared_copies(_W1))
        store_heads(1, 0)
        store_heads(2, 0)
        project_part(0, [0])
        _wait(copies + head_copies(1))
        _start(part_copies(1) + head_copies(2))
        store_parts(0, lambda w: store_heads(w, 1), (_WO, _W2))
        project_part(0, [1, 2])
        _wait(shared_copies(_W1))

        @pl.loop(1, _PARTS // 2, unroll=True)
        def _(n):
            for part in (2 * n - 1, 2 * n):
                _wait(part_copies(part) + head_copies(part + 1))
                _start(part_copies(part + 1))
                pl.when(part + 2 < _PARTS)(lambda: _start(head_copies(part + 2)))
                pl.when(part + 2 == _PARTS)(lambda: _start(last_copies(_W2)))
                store_parts(part, lambda w: store_heads(w, part + 1))
                project_part(part, range(3))

        _wait(part_copies(_PARTS - 1) + last_copies(_W2))
        _start(first_step_copies(0))
        store_parts(_PARTS - 1, lambda m: store_last(_W2, w2_ref) if m == _W1
                    else store_shared(m, w2_ref if m == _W2 else wo_ref))
        project_part(_PARTS - 1, range(3))

    def run_layers(w3_ref, pair_rows_ref, pair_in_ref, solo_rows_ref, solo_in_ref, ffn_rows_ref,
                   ffn_in_ref, attn_shared_ref, ffn_shared_ref, partial_ref, qkv_ref, heads_ref,
                   hidden_ref, attn_sum_ref, ffn_sum_ref, mem_ref, block_ref, second_ref):
        def segment(s):
            return s >> 2, _aligned((s & 3) * seg, seg)

        def transpose_out(i):
            tile_ref.bitcast(words)[i, :d_model // 2] = pltpu.bitcast(x_ref[i, :_LANES].T, words)

        def contract(groups, part, rows_ref, weight_ref, sum_ref, begun):
            operands = _operands(_levels(groups), _WIDE, lambda f, j: rows_ref[part, f, j])

            def targets(i):
                return [_TILES if 2 * i + half == part else i for half in range(2)]

            def start(f, i):
                low, high = (
                    sum_ref[f, n] if (n, half) in begun else None if groups < 4
                    else block_ref[f, :, n * _LANES:(n + 1) * _LANES]
                    for half, n in enumerate(targets(i)))
                if targets(i) == [i, i] and ((i, 0) in begun) == ((i, 1) in begun):
                    return low
                if low is None and high is None:
                    return None
                lanes = jax.lax.broadcasted_iota(jnp.int32, sum_ref.shape[-2:], 1)
                return jnp.where(lanes < _CHUNK, 0.0 if low is None else low,
                                 0.0 if high is None else high)

            def finish(f, i, tile):
                if targets(i) == [i, i]:
                    sum_ref[f, i] = tile
                else:
                    for half, n in enumerate(targets(i)):
                        lanes = slice(half * _CHUNK, (half + 1) * _CHUNK)
                        sum_ref[f, n, :, lanes] = tile[:, lanes]

            _collect(_levels(groups), _MODEL,
                     lambda r: side.dot(operands[r](), _load_packed(weight_ref, part, r)),
                     start, finish, partial_ref.at[part % 2])
            begun.update((n, half) for i in range(_TILES) for half, n in enumerate(targets(i)))

        def keep_and_add(ref, part, f, j, tile):
            total = ref.shape[0] - 1
            ref[part, f, j] = tile
            if 0 < part < _PARTS:
                ref[total, f, j] = ref[total if part > 1 else 0, f, j] + tile

        def project(groups, w, part):
            in_ref = pair_in_ref if groups == 2 else solo_in_ref
            rows = slice(0, in_ref.shape[1])
            side.finish(("P", None), ("P", part // 2))
            operand = _operand_loader(in_ref, groups, part)
            out_ref = qkv_ref.at[w, part % qkv_ref.shape[1]]
            done = {}

            def finish(f, j, tile):
                done[f, j] = tile
                if part == _PARTS:
                    attn_shared_ref[w, f, j, rows] = tile
                elif groups == 2 and (1 - f, j) in done:
                    upper, lower = done[0, j], done[1, j]
                    out_ref[j, :2 * size - ahead] = jnp.concatenate(
                        [upper[n_mem:n_mem + ahead], upper[:n_mem], lower[:n_mem],
                         upper[n_mem + ahead:], lower[n_mem:]], axis=0).astype(bf16)
                elif groups == 1 and (0, j ^ 1) in done:
                    a, b = done[0, j & ~1], done[0, j | 1]
                    out_ref[j | 1] = jnp.concatenate(
                        [a[n_mem:], a[:n_mem], b], axis=0).astype(bf16)

            _collect(_levels(groups), _WIDE,
                     lambda r: side.dot(operand(r), _load_packed(wqkv_ref, w, part, r)),
                     lambda f, j: attn_shared_ref[w, f, j, rows] if part < _PARTS else None,
                     finish)

        def projected(groups, t, place, w, head):
            part, j = divmod(head, _TILES)
            index = w, part % qkv_ref.shape[1], j
            if groups == 1:
                rows = [_load_words(qkv_ref, *index)]
            else:
                rows = [_load_words(early_ref, (t - _LAG) >> 1, w, part, j,
                                    pl.ds(place * ahead // 2, ahead // 2)),
                        _load_words(qkv_ref, *index, slice(0, size - ahead // 2))]
            if w == 1:
                rows.append(jnp.zeros((_CHUNK - size, d_head), words))
            return pltpu.bitcast(jnp.concatenate(rows, axis=0), bf16)

        def by_group(tile):
            return enumerate(tile[f * seg:(f + 1) * seg] for f in range(4))

        def expand(g):
            plain = 2 * _PARTS + 2
            if g == plain:
                x = jnp.concatenate([ffn_rows_ref[f, 0, :seg] for f in range(4)], axis=0)
                for j in range(_TILES):
                    for f, tile in by_group(_dot(x.astype(bf16), _load_packed(wplain_ref, 0, j))):
                        ffn_shared_ref[2, f, j] = tile
                return
            part, up = divmod(g if g < plain else g - 1, 2)
            chunk = up if part == _PARTS else min(part, _PARTS)
            side.finish(("G", None), ("G", chunk // 2))
            operand = _operand_loader(ffn_in_ref, 4, chunk)
            weight_ref = w3_ref if up else w1_ref

            def finish(f, j, tile):
                if part > _PARTS:
                    ffn_shared_ref[up, f, j] = tile
                elif up:
                    keep_and_add(hidden_ref, part, f, j, hidden_ref[part, f, j] * tile)
                else:
                    hidden_ref[part, f, j] = _scaled_silu(tile)

            _collect(_levels(4), _WIDE,
                     lambda r: side.dot(operand(r), _load_packed(weight_ref, part, r)),
                     lambda f, j: None if part > _PARTS else ffn_shared_ref[
                         2 if part == _PARTS else up, f, j],
                     finish, partial_ref.at[g % 2])

        def reduce(g, begun):
            if not begun:
                for f in range(4):
                    rest = block_ref[f, :, width:]
                    ffn_sum_ref[f, _TILES] = jnp.concatenate([rest, jnp.zeros_like(rest)], axis=1)
                begun.update([(_TILES, 0), (_TILES, 1)])
            if g < w2_ref.shape[0]:
                contract(4, g, hidden_ref, w2_ref, ffn_sum_ref, begun)
                return
            total = None
            for j in range(_TILES):
                rows = jnp.concatenate([hidden_ref[_PARTS, f, j] for f in range(4)], axis=0)
                total = _accumulate(total, 1, _dot(
                    _load_packed(wplain_ref, 1, j, slice(0, _CHUNK // 2)), rows.astype(bf16), 1))
            for f, tile in by_group(_value(total).T):
                ffn_sum_ref[f, _TILES, :, :_CHUNK] += tile

        def layer_input(t, place, layer):
            return x_ref[segment(t)].astype(f32) if layer == 0 else second_ref[place]

        def begin_step(t, place, layers):
            h = _layernorm(layer_input(t, place, layers[-1]))
            if len(layers) == 1:
                rows_ref, in_ref = solo_rows_ref, solo_in_ref
                _store_rows(rows_ref, 0, n_mem, h)
            else:
                rows_ref, in_ref, cut = pair_rows_ref, pair_in_ref, ahead // 2
                _store_rows(rows_ref, 0, n_mem, _layernorm(layer_input(t, place, 0)[ahead:]))
                _store_rows(rows_ref, 0, seg - cut, h[:cut])
                _store_rows(rows_ref, 1, n_mem, h[cut:])
            for f, layer in enumerate(layers):
                _store_rows(rows_ref, f, 0, mem_ref[layer])
            for tile in [None, *range(_TILES)]:
                for job in _operand_jobs(in_ref, rows_ref, tile):
                    side.add(rows_ref, job, ("P", tile))

        def close_step(t, place, layers):
            for f, layer in enumerate(layers):
                out = _load_rows(attn_sum_ref, f)
                mem_ref[layer] = out[:n_mem]
                index = 2 * layer + place if len(layers) == 2 else place
                block_ref[index] = layer_input(t, place, layer) + out[n_mem:]

        def run(order, layers=(), t=0, place=0):
            groups, first = len(layers), t
            visible, fill = _attention_masks(n_mem, seg)
            attn_begun, ffn_begun, probs = set(), set(), {}
            for name in order.split():
                stage, g = name[0], int(name[1:] or 0)
                if stage == "N":
                    begin_step(t, place, layers)
                elif stage == "P":
                    project(groups, g % 3, g // 3)
                elif stage == "S" and (groups == 2 or g % 2):
                    q, k = (projected(groups, first, place, w, g) for w in range(2))
                    s = jnp.where(visible, _dot(q, k, 1), fill)
                    p = jnp.exp2(s - jnp.max(s, axis=-1, keepdims=True))
                    inv = pltpu.reciprocal(jnp.sum(p, axis=-1, keepdims=True), approx=True)
                    probs[g] = p[:, :2 * size].astype(bf16), inv
                elif stage == "V" and (groups == 2 or g % 2):
                    o = _dot(probs[g][0], projected(groups, first, place, 2, g)) * probs[g][1]
                    halves = jnp.concatenate([o[seg:size], o[:seg]], axis=0), o[size:]
                    for f, half in enumerate(halves):
                        index = (f, g % _TILES) if groups == 2 else (0, g % _TILES - 1 + f)
                        keep_and_add(heads_ref, g // _TILES, *index, half)
                elif stage == "O":
                    contract(groups, g, heads_ref, wo_ref, attn_sum_ref, attn_begun)
                elif stage == "A":
                    close_step(t, place, layers)
                    t, place, attn_begun = t + 1, place + 1, set()
                elif stage == "M":
                    _store_rows(ffn_rows_ref, g, 0, _layernorm(block_ref[g]))
                elif stage == "F":
                    tile = g if g < _TILES else None
                    for job in _operand_jobs(ffn_in_ref, ffn_rows_ref, tile):
                        side.add(ffn_rows_ref, job, ("G", tile))
                elif stage == "G":
                    expand(g)
                elif stage == "D":
                    reduce(g, ffn_begun)
                elif stage == "E":
                    for s in range(2):
                        second_ref[g + s] = _load_rows(ffn_sum_ref, s)
                        x_ref[segment(jnp.maximum(first + g - 2 * _LAG, 0) + s)] = _load_rows(
                            ffn_sum_ref, 2 + s).astype(bf16)
                elif stage == "T":
                    side.add(x_ref, functools.partial(transpose_out, g))
                elif stage == "C":
                    _start(out_copies[:n_io - 1])
                elif stage == "Z":
                    for _ in range(g):
                        side.add()
                elif stage == "W":
                    side.spread(g)
                elif stage == "X":
                    side.finish()

        side.keep_in_memory(pair_in_ref, solo_rows_ref, solo_in_ref, ffn_in_ref, attn_shared_ref,
                            ffn_shared_ref, partial_ref, qkv_ref, heads_ref, hidden_ref,
                            attn_sum_ref, ffn_sum_ref)
        attn_sum_ref[...] = jnp.zeros_like(attn_sum_ref)
        mem_copy.wait()
        mem_ref[0] = mem0_ref[...].astype(f32)
        for t in range(_LAG):
            run("N", (0,), t, t)
            _wait(first_step_copies(t))
            _start(first_step_copies(t + 1) if t + 1 < _LAG else [mem_copy])
            (store_shared, store_last)[t // 2](*((_W1, w1_ref), (_W3, w3_ref))[t % 2])
            for n in range(2):
                store_part(_W3, w3_ref, 2 * t + n, 3 * (t & 1) + n)
            if t == 0:
                store_part(_W1, w1_ref, 0, 2)
            run("W540 " + _ATTENTION + " X", (0,), t, t)
        mem_copy.wait()
        mem_ref[1] = mem0_ref[...].astype(f32)
        run(_SWIGLU)
        for s in range(2):
            second_ref[s] = _load_rows(ffn_sum_ref, s)
            ffn_sum_ref[s] = ffn_sum_ref[2 + s]
        run(2 * ("N W200 " + _ATTENTION + " ") + "M0 M2 M1 M3 G18 X", (0, 1), _LAG)

        @pl.loop(_LAG // 2 + 1, n_seg // 2)
        def _(b):
            run(_TWO_STEPS + " X", (0, 1), 2 * b)

        out_copies = [
            pltpu.make_async_copy(tile_ref.at[i, :d_model],
                                  outt_hbm.at[:, pl.ds(i * _LANES, _LANES)], tile_sem.at[0])
            for i in range(n_io)]
        run(_LAST_STEPS, (1,), n_seg)
        run(_SWIGLU.replace("W500", " ".join(f"T{i} Z3" for i in range(n_io - 1)) + " W900")
            .replace("D5", "X C D5"))
        for s in range(_LAG):
            x_ref[segment(n_seg - _LAG + s)] = _load_rows(ffn_sum_ref, s).astype(bf16)
        transpose_out(n_io - 1)
        _start(out_copies[n_io - 1:])
        _wait(out_copies)

    spare = 8
    mem_copy = pltpu.make_async_copy(mem0_hbm, mem0_ref, mem_sem)
    mem_copy.start()
    pl.run_scoped(
        load_weights,
        pltpu.VMEM((n_io - 1, len(_operand_slots(2)), seg, _LANES), bf16),
        pltpu.VMEM((3, n_io - 1, 2, _TILES, seg, _LANES), f32),
        pltpu.VMEM((9, 2, d_model + spare, d_head), words),
        pltpu.SemaphoreType.DMA((9,)),
        *[pltpu.VMEM((2, _TILES + 1, seg + spare, _LANES), f32)] * 3)
    pl.run_scoped(
        run_layers,
        pltpu.VMEM(w1_ref.shape, bf16),
        pltpu.VMEM((2, _TILES + 1, seg + spare, _LANES), f32),
        pltpu.VMEM((len(_operand_slots(2)), seg, _LANES), bf16),
        pltpu.VMEM((1, _TILES + 1, size + spare, _LANES), f32),
        pltpu.VMEM((len(_operand_slots(1)), size, _LANES), f32),
        pltpu.VMEM((4, _TILES + 1, seg + spare, _LANES), f32),
        pltpu.VMEM((len(_operand_slots(4)), seg, _LANES), bf16),
        pltpu.VMEM((3, 2, _TILES, size, _LANES), f32),
        pltpu.VMEM((3, 4, _TILES, seg, _LANES), f32),
        pltpu.VMEM((2, 4, _TILES, seg, _LANES), f32),
        pltpu.VMEM((3, 3, _TILES, 2 * size, _LANES), bf16),
        pltpu.VMEM((_PARTS + 1, 2, _TILES, size, _LANES), f32),
        pltpu.VMEM((_PARTS + 2, 4, _TILES, seg, _LANES), f32),
        pltpu.VMEM((2, _TILES + 1, size, _LANES), f32),
        pltpu.VMEM((4, _TILES + 1, seg, _LANES), f32),
        pltpu.VMEM((2, n_mem, d_model), f32),
        pltpu.VMEM((4, seg, d_model), f32),
        pltpu.VMEM((4, seg, d_model), f32))


@functools.partial(jax.jit, static_argnames=("A_seg_len",))
def pallas_interleave_layers__memory_aug_recurrent_mem_tr__glu_gated_swiglu__prompt_kernel(
    A_x: jax.Array,
    A_mem0: jax.Array,
    A_Wq: jax.Array,
    A_Wk: jax.Array,
    A_Wv: jax.Array,
    A_Wo: jax.Array,
    A_seg_len: int,
    B_x: jax.Array,
    B_w1: jax.Array,
    B_w3: jax.Array,
    B_w2: jax.Array,
):
    del B_x
    _, n_tok, d_model = A_x.shape
    n_mem = A_mem0.shape[1]
    _, n_heads, d_head = A_Wq.shape
    seg = A_seg_len
    assert A_x.shape[0] == 1 and _LAG * seg == d_head == _LANES and 4 * n_mem == seg
    assert n_heads == _PARTS * _TILES and d_model == (_PARTS + 1) * _CHUNK
    assert B_w1.shape[1] == (_PARTS + 1) * _TILES * _LANES and n_tok == 16 * _LANES
    bf16 = jnp.bfloat16
    attn_blocks = (_PARTS + 1, len(_HOPCROFT_KERR), _LANES, _LANES)
    ffn_blocks = (_PARTS + 2, len(_STRASSEN) ** 2, _LANES, _LANES)
    hbm = pl.BlockSpec(memory_space=pltpu.HBM)
    out_t = pl.pallas_call(
        functools.partial(_kernel, seg=seg),
        out_shape=jax.ShapeDtypeStruct((d_model, n_tok), A_x.dtype),
        in_specs=[hbm] * 9,
        out_specs=hbm,
        scratch_shapes=[
            pltpu.VMEM((n_mem, d_model), bf16),
            pltpu.VMEM((n_tok // _LANES, d_model + _SLAB, _LANES), bf16),
            pltpu.VMEM((n_tok // _LANES, _LANES + _SLAB, d_model), bf16),
            pltpu.VMEM(((n_tok // seg - _LAG) // 2, 3, _PARTS, _TILES, seg, _LANES), bf16),
            pltpu.VMEM((3, *attn_blocks), bf16),
            pltpu.VMEM(attn_blocks, bf16),
            pltpu.VMEM(ffn_blocks, bf16),
            pltpu.VMEM(ffn_blocks, bf16),
            pltpu.VMEM((2, _TILES, _LANES, _LANES), bf16),
            pltpu.VMEM((11, (d_model + _SLAB) // 2, _TILES * _LANES), jnp.uint32),
            pltpu.SemaphoreType.DMA((11,)),
            pltpu.SemaphoreType.DMA(()),
            pltpu.SemaphoreType.DMA((2,)),
            *[pltpu.VMEM((_TILES, _TILES, _LANES + _SLAB // 2, _LANES), jnp.float32)] * 2,
        ],
        compiler_params=pltpu.CompilerParams(
            vmem_limit_bytes=127 * 1024 * 1024,
            flags={"XLA_TPU_FORCE_LP_LLO_SCHEDULER": True,
                   "XLA_TPU_EVENLY_DISTRIBUTE_CRITICAL_NODES": True}),
    )(A_x.reshape(n_tok, d_model).T, A_mem0.reshape(n_mem, d_model), A_Wq, A_Wk, A_Wv,
      A_Wo.transpose(0, 2, 1), B_w1, B_w2.T, B_w3)
    return out_t.T.reshape(A_x.shape)
```

```python
import functools
import math

import jax
import jax.numpy as jnp
import jax.experimental.pallas as pl
import jax.experimental.pallas.tpu as pltpu

_EPS = 1e-05
_MASKED = -1000000000.0
_LOG2E = math.log2(math.e)
_LANES = 128
_CHUNK = _LANES // 2
_SLAB = 16
_TILES = 4
_PARTS = 2 * _TILES
_LAG = 4
_WO, _W1, _W2, _W3 = range(4)
_MODEL, _WEIGHT, _WIDE = range(3)
_HOPCROFT_KERR = (
    (((1, 1, 2),), ((1, 2, 0), (1, 2, 2), (1, 2, 3), (-1, 1, 2)), ((1, 2, 2),)),
    (((1, 2, 2),), ((1, 2, 1), (1, 2, 2), (-1, 0, 2), (-1, 3, 2)), ((1, 0, 2),)),
    (((1, 0, 2), (1, 0, 3)), ((1, 2, 3),), ((-1, 2, 2), (1, 2, 3))),
    (((1, 2, 2), (1, 0, 3)), ((1, 2, 3), (1, 3, 2)), ((1, 2, 2), (-1, 1, 3))),
    (((1, 2, 2), (1, 2, 3)), ((1, 3, 2),), ((-1, 1, 2), (1, 1, 3))),
    (((1, 0, 0), (1, 0, 2)), ((1, 2, 0),), ((1, 2, 0), (-1, 2, 2))),
    (((1, 0, 0), (1, 2, 2)), ((1, 0, 2), (1, 2, 0)), ((-1, 1, 0), (1, 2, 2))),
    (((1, 2, 0), (1, 2, 2)), ((1, 0, 2),), ((1, 1, 0), (-1, 1, 2))),
    (((1, 0, 1), (1, 0, 2)), ((1, 2, 1),), ((1, 0, 1), (-1, 0, 2))),
    (((1, 0, 1), (1, 1, 2)), ((1, 1, 2), (1, 2, 1)), ((1, 1, 1), (1, 0, 2))),
    (((1, 1, 1), (1, 1, 2)), ((1, 1, 2),), ((-1, 1, 1), (1, 1, 2))),
    (((1, 1, 1), (1, 1, 3)), ((1, 0, 3), (-1, 1, 3)), ((1, 2, 1), (-1, 2, 3))),
    (((1, 0, 0), (1, 0, 1), (1, 0, 3)), ((1, 0, 3),), ((1, 2, 1), (-1, 2, 0), (1, 2, 3))),
    (((1, 2, 0), (1, 2, 1), (1, 0, 3)), ((1, 0, 3), (1, 3, 0)),
     ((1, 2, 0), (-1, 2, 1), (-1, 1, 3))),
    (((1, 2, 0), (1, 2, 1), (1, 2, 3)), ((1, 3, 0),), ((1, 1, 1), (-1, 1, 0), (1, 1, 3))),
    (((1, 1, 3),), ((1, 0, 3), (-1, 1, 3), (1, 3, 0), (1, 3, 2), (1, 3, 3)), ((1, 1, 3),)),
    (((1, 2, 1), (1, 2, 3)), ((1, 3, 0), (1, 3, 1)), ((1, 0, 1), (-1, 0, 3))),
    (((1, 1, 3), (-1, 2, 1)), ((1, 3, 0), (1, 3, 1), (-1, 0, 3), (1, 1, 3)),
     ((1, 2, 1), (-1, 0, 3))),
    (((1, 0, 3),), ((1, 3, 0), (1, 3, 1), (-1, 0, 3), (-1, 2, 3), (1, 3, 3)), ((1, 0, 3),)),
    (((1, 1, 0), (1, 1, 1)), ((1, 0, 3), (1, 1, 0)), ((1, 2, 0), (-1, 2, 1))),
    (((1, 2, 1), (-1, 1, 0)), ((1, 0, 1), (1, 1, 0)), ((1, 0, 0), (-1, 2, 1))),
    (((1, 0, 1),), ((1, 1, 0), (1, 1, 1), (1, 1, 3), (-1, 0, 3), (-1, 2, 1)), ((1, 2, 1),)),
    (((1, 2, 0), (1, 2, 1)), ((1, 0, 1), (1, 3, 0)), ((-1, 0, 0), (1, 0, 1))),
    (((1, 2, 1),), ((1, 3, 0), (1, 3, 1), (1, 0, 1), (-1, 1, 1), (-1, 1, 2)), ((1, 1, 1),)),
    (((1, 0, 0),), ((1, 0, 0), (1, 0, 1), (-1, 2, 0)), ((1, 0, 0),)),
    (((1, 1, 0),), ((1, 0, 0), (1, 0, 2), (-1, 1, 0)), ((1, 1, 0),)),
)
_RUNS = (5, 11, 19, 24, 24)
_STRASSEN = (
    (((-1, 2, 0),), ((1, 0, 0), (1, 0, 1)), ((1, 1, 1),)),
    (((1, 1, 0), (1, 1, 1)), ((1, 0, 0),), ((1, 1, 0), (-1, 1, 1))),
    (((1, 1, 1),), ((1, 1, 0), (-1, 0, 0)), ((1, 2, 0),)),
    (((1, 0, 0), (1, 1, 1)), ((1, 0, 0), (1, 1, 1)), ((1, 0, 0), (1, 1, 1))),
    (((1, 0, 0),), ((1, 0, 1), (-1, 1, 1)), ((1, 2, 1),)),
    (((1, 0, 0), (1, 0, 1)), ((1, 1, 1),), ((-1, 0, 0), (1, 0, 1))),
    (((1, 2, 1),), ((1, 1, 0), (1, 1, 1)), ((1, 0, 0),)),
)
_ATTENTION = (
    "P24 P25 P26 P0 P1 P2 S0 S1 S2 S3 P3 P4 V0 V1 V2 V3 P5 S4 S5 S6 S7 O0 P6 P7 V4 V5 V6 V7 "
    "P8 S8 S9 S10 S11 O1 P9 P10 V8 V9 V10 V11 P11 S12 S13 S14 S15 O2 P12 P13 V12 V13 V14 V15 "
    "P14 S16 S17 S18 S19 O3 P15 P16 V16 V17 V18 V19 P17 S20 S21 S22 S23 P18 P19 V20 V21 V22 "
    "V23 P20 S24 S25 S26 S27 P21 P22 V24 V25 V26 V27 P23 S28 S29 S30 S31 O4 V28 V29 V30 V31 "
    "O5 O6 O7 O8 A")
_STEP = "N W200 " + _ATTENTION
_SWIGLU = (
    "M0 M1 M2 M3 F4 X F0 F1 F2 F3 W500 G18 G19 G20 G16 G17 G0 D8 D10 G1 G2 D0 G3 G4 D1 G5 G6 "
    "D2 G7 G8 D3 G9 G10 D4 G11 G12 G13 G14 D5 G15 D6 D7 D9")
_TWO_STEPS = (
    "E F4 X N Z11 G19 F0 W250 G20 P24 P25 P26 P0 G16 P1 P2 G17 S0 S1 S2 S3 P3 P4 V0 V1 V2 V3 "
    "P5 G0 S4 S5 S6 S7 O0 G1 P6 P7 V4 V5 V6 V7 P8 D8 S8 S9 S10 S11 O1 F1 W200 G2 P9 P10 V8 V9 "
    "V10 V11 P11 S12 S13 S14 S15 O2 D0 P12 P13 V12 V13 V14 V15 P14 S16 S17 S18 S19 O3 G3 P15 "
    "P16 V16 V17 V18 V19 P17 S20 S21 S22 S23 O4 P18 G4 P19 V20 V21 V22 V23 P20 S24 S25 S26 "
    "S27 O5 F2 W160 D1 P21 P22 V24 V25 V26 V27 P23 S28 S29 S30 S31 O6 G5 V28 V29 V30 V31 G6 "
    "O7 O8 A Z4 N W200 D2 G7 D3 P24 P25 P26 G8 P0 P1 P2 S0 S1 S2 S3 P3 P4 V0 V1 V2 V3 P5 G9 "
    "S4 S5 S6 S7 O0 F3 W120 P6 G10 P7 V4 V5 V6 V7 P8 S8 S9 S10 S11 O1 D4 P10 P9 V8 V9 V10 V11 "
    "P11 S12 S13 S14 S15 O2 G11 P12 P13 V12 V13 V14 V15 P14 S16 S17 S18 S19 O3 G12 P15 P16 "
    "V16 V17 V18 V19 P17 S20 S21 S22 S23 O4 P18 P19 V20 V21 V22 V23 P20 S24 S25 S26 S27 O5 "
    "G14 G13 P21 P22 V24 V25 V26 V27 P23 S28 S29 S30 S31 O6 D5 M0 V28 V29 V30 V31 G15 O7 O8 "
    "M2 D9 A D10 M3 D6 M1 D7 G18")
_LAST_STEPS = (
    "E F4 X N F0 F1 W400 G19 G20 " + _ATTENTION.replace("O0", "O0 G16 G17 G0 D8 G1 G2 D0 G3")
    + " N F2 F3 W450 G4 D1 D10 G5 G6 D2 G7 G8 D3 G9 G10 D4 G11 G12 G13 G14 D5 G15 D6 D7 D9 E2 "
    + _ATTENTION)


def _layernorm(x):
    m = jnp.mean(x, axis=-1, keepdims=True)
    d = x - m
    v = jnp.mean(d * d, axis=-1, keepdims=True)
    return d * jax.lax.rsqrt(v + _EPS)


def _scaled_silu(x):
    return x * pltpu.reciprocal(1.0 + jnp.exp2(x), approx=True)


def _dot(a, b, axis=0):
    return jax.lax.dot_general(a, b, (((1,), (axis,)), ((), ())),
                               preferred_element_type=jnp.float32)


def _load_words(ref, *index):
    return ref[index] if ref.dtype == jnp.float32 else ref.bitcast(jnp.uint32)[index]


def _load_packed(ref, *index):
    return pltpu.bitcast(_load_words(ref, *index), ref.dtype)


def _aligned(first, size):
    return pl.ds(first if isinstance(first, int) else pl.multiple_of(first, size), size)


def _accumulate(total, sign, value):
    if total is None:
        return sign, value
    if total[0] == sign:
        return sign, jax.lax.add(total[1], value)
    return 1, jax.lax.sub(*((total[1], value) if sign < 0 else (value, total[1])))


def _value(total):
    return total[1] if total[0] > 0 else -total[1]


def _levels(groups):
    if groups == 4:
        return [dict(enumerate(_STRASSEN))] * 2
    if groups == 2:
        return [dict(enumerate(_HOPCROFT_KERR))]

    def upper(terms):
        return tuple((sign, 0, i) for sign, f, i in terms if f != 1)

    return [{r: (upper(model), weight, upper(wide))
             for r, (model, weight, wide) in enumerate(_HOPCROFT_KERR)
             if upper(model) and upper(wide)}]


def _combination(terms, side, block):
    total = None
    for sign, a, b in terms:
        if side == _WEIGHT or a < 2:
            total = _accumulate(total, sign, block(a, b))
        else:
            total = _accumulate(total, *_accumulate(
                (sign, block(0, b)), -sign if side == _MODEL else sign, block(1, b)))
    return _value(total)


def _operands(levels, side, block):
    level, *inner = levels
    if not inner:
        block = functools.cache(block)
        return {r: functools.partial(_combination, product[side], side, block)
                for r, product in level.items()}
    operands = {}
    for r, product in level.items():
        def sub_block(a, b, terms=product[side]):
            return _combination(terms, side, lambda f, i: block(2 * f + a, 2 * i + b))

        for n, operand in _operands(inner, side, sub_block).items():
            operands[r * len(inner[0]) + n] = operand
    return operands


def _collect(levels, side, multiply, start, finish, partial_ref=None):
    level, *inner = levels
    terms = [term for product in level.values() for term in product[side]]
    left = {}
    for _, f, i in terms:
        left[f, i] = left.get((f, i), 0) + 1
    for i in sorted({i for _, f, i in terms if f == 2}):
        for f in range(2):
            left[f, i] = left.get((f, i), 0) + 1
    total = {}

    def add(r, f, i, sign, result):
        left[f, i] -= 1
        if f == 2:
            total[f, i] = _accumulate(total.get((f, i)), sign, result)
            if not left[f, i]:
                sign, result = total[f, i]
                add(r, 0, i, sign, result)
                add(r, 1, i, -sign if side == _MODEL else sign, result)
            return
        for (a, b), tile in result.items() if inner else [((0, 0), result)]:
            index = (2 * f + a, 2 * i + b) if inner else (f, i)
            key = f, i, a, b
            if key not in total:
                first = start(*index)
                before = None if first is None else (1, first)
            elif total[key][1] is None:
                before = total[key][0], partial_ref[index]
            else:
                before = total[key]
            total[key] = _accumulate(before, sign, tile)
            if not left[f, i]:
                finish(*index, _value(total[key]))
            elif inner and not any(g in (f, 2) and j == i for _, g, j in level[r + 1][side]):
                partial_ref[index] = total[key][1]
                total[key] = total[key][0], None

    for r, product in level.items():
        if inner:
            result = {}
            _collect(inner, side, lambda n: multiply(r * len(inner[0]) + n), lambda f, i: None,
                     lambda f, i, tile: result.update({(f, i): tile}))
        else:
            result = multiply(r)
        for sign, f, i in product[side]:
            add(r, f, i, sign, result)


@functools.cache
def _operand_slots(groups):
    used = {0: [0]}
    for level in _levels(groups):
        used = {r * len(level) + n: sorted({2 * i + j for i in tiles for _, _, j in terms})
                for r, tiles in used.items() for n, (terms, _, _) in level.items()}
    keys = [(r, tile) for r, tiles in used.items() for tile in [None] + tiles]
    return {key: slot for slot, key in enumerate(keys)}


class _SideJobs:
    def __init__(self, zero):
        self.zero, self.jobs, self.pace, self.due, self.count = zero, [], 0.0, 0.0, -1

    def add(self, source_ref=None, job=None, key=None):
        self.jobs.append((key, source_ref, job))

    def spread(self, products):
        self.pace = len(self.jobs) / products

    def finish(self, *keys):
        while self.jobs and (not keys or any(key in keys for key, _, _ in self.jobs)):
            _, ref, job = self.jobs.pop(0)
            if ref is not None:
                job()

    def dot(self, a, b):
        result = _dot(a, b)
        self.count += 1
        self.due = self.due + self.pace if self.jobs else 0.0
        while self.jobs and self.due >= 1.0:
            self.due -= 1.0
            _, ref, job = self.jobs.pop(0)
            if ref is None:
                continue
            rows = 32 // ref.dtype.itemsize
            first = self.count % 4 * (result.shape[0] // rows) // 4 * rows
            value = jax.lax.slice_in_dim(result, first, first + rows)
            index = (self.zero,) * (ref.ndim - 2) + (
                slice(ref.shape[-2] - rows, None), slice(0, _LANES))
            ref[index] = (pltpu.bitcast(value, ref.dtype) if ref.dtype == jnp.uint32
                          else value.astype(ref.dtype))
            job()
        return result

    def keep_in_memory(self, *refs):
        for ref in refs:
            ref[(self.zero,) * (ref.ndim - 2)] = jnp.zeros(ref.shape[-2:], ref.dtype)


def _store_rows(ref, f, first, x):
    rows = slice(first, first + x.shape[0])
    for i in range(_TILES):
        ref[f, i, rows] = x[:, i * _LANES:(i + 1) * _LANES]
    ref[f, _TILES, rows] = jnp.concatenate([x[:, _TILES * _LANES:]] * 2, axis=1)


def _load_rows(ref, f):
    rest = ref[f, _TILES]
    return jnp.concatenate(
        [ref[f, i] for i in range(_TILES)] + [rest[:, :_CHUNK] + rest[:, _CHUNK:]], axis=1)


def _combination_jobs(ref, groups, side, block, slots):
    def job(batch, rows):
        operands = _operands(_levels(groups), side, lambda a, b: block(a, b, rows))
        for r, slot in batch:
            ref[slot, rows] = jax.lax.convert_element_type(operands[r](), ref.dtype)

    batches = {}
    for r, slot in slots.items():
        key = r // len(_STRASSEN) if groups == 4 else sum(r >= cut for cut in _RUNS) % 4
        batches.setdefault(key, []).append((r, slot))
    step = _SLAB if groups > 1 else ref.shape[1]
    return [functools.partial(job, batch, slice(first, first + step))
            for batch in batches.values() for first in range(0, ref.shape[1], step)]


def _operand_jobs(ref, rows_ref, tile):
    groups = rows_ref.shape[0]
    return _combination_jobs(
        ref, groups, _MODEL, lambda f, i, rows: rows_ref[f, _TILES if i == tile else i, rows],
        {r: slot for (r, replaced), slot in _operand_slots(groups).items() if replaced == tile})


def _operand_loader(ref, groups, part):
    slots = _operand_slots(groups)
    rows = ref.shape[-2] * ref.dtype.itemsize // 4
    lanes = jax.lax.broadcasted_iota(jnp.int32, (rows, _LANES), 1)
    replaced = (lanes & _CHUNK) == (part & 1) * _CHUNK
    if isinstance(part, int):
        others = {r: slot for (r, tile), slot in slots.items() if tile == part // 2}
    else:
        others = {}
        for (r, tile), slot in slots.items():
            others[r] = slot if tile is None else jnp.where(part >> 1 == tile, slot, others[r])

    def load(r, *index):
        words = _load_words(ref, *index, slots[r, None])
        if r in others:
            words = jax.lax.select(replaced, _load_words(ref, *index, others[r]), words)
        return pltpu.bitcast(words, ref.dtype) if words.dtype != ref.dtype else words

    return load


def _attention_masks(n_mem, seg):
    size = n_mem + seg
    shape = (2 * size, _LANES)

    def position(axis):
        r = jax.lax.broadcasted_iota(jnp.int32, shape, axis)
        return r < size, jnp.where(r < seg, r + n_mem, jnp.where(r < size, r - seg, r - size))

    (first_i, i), (first_j, j) = position(0), position(1)
    same = (first_i == first_j) & (j < size)
    fill = jnp.where(same, _MASKED * _LOG2E, -jnp.inf).astype(jnp.float32)
    return same & ((i < n_mem) | (i >= j)), fill


def _start(copies):
    for copy in copies:
        copy.start()


def _wait(copies):
    for copy in copies:
        copy.wait()


def _kernel(xt_hbm, mem0_hbm, wq_hbm, wk_hbm, wv_hbm, wot_hbm, w1_hbm, w2t_hbm, w3_hbm,
            outt_hbm, mem0_ref, tile_ref, x_ref, early_ref, wqkv_ref, wo_ref, w1_ref, w2_ref,
            wplain_ref, stage_ref, stage_sem, mem_sem, tile_sem, *wide_refs, seg):
    d_model, n_tok = xt_hbm.shape
    n_mem = mem0_ref.shape[0]
    d_head = wq_hbm.shape[2]
    n_seg = n_tok // seg
    n_io = n_tok // _LANES
    size = n_mem + seg
    ahead = seg // 2
    width = _TILES * _LANES
    score_scale = d_head ** -0.5 * _LOG2E
    scales = {_W1: -_LOG2E, _W3: -1 / _LOG2E}
    f32, bf16, words = jnp.float32, jnp.bfloat16, jnp.uint32
    shared_slot = 6
    last_slots = {_W1: 2, _W2: shared_slot + 4, _W3: 5}
    wide_refs = list(wide_refs)
    side = _SideJobs(jax.lax.fori_loop(0, 3, lambda i, total: total - i, 3))

    def combine_weights(out_ref, source_ref, block, n_rows, n_tiles):
        wide_refs.reverse()
        wide_ref = wide_refs[0]

        def widen(first, tiles):
            rows = range(first, first + n_rows)
            for j, tile in [(j, block(rows, j)) for j in tiles]:
                wide_ref[first // _LANES, j, pl.ds(first % _LANES, n_rows)] = tile

        jobs = [functools.partial(widen, first, range(j, j + n_tiles))
                for j in range(0, _TILES, n_tiles) for first in range(0, width, n_rows)]
        before = []
        while side.jobs and side.jobs[-1][1] is wide_refs[1]:
            before.insert(0, side.jobs.pop())
        for n, job in enumerate(jobs):
            side.add(source_ref, job)
            if n_rows == _LANES:
                side.add()
            side.jobs += before[n * len(before) // len(jobs):(n + 1) * len(before) // len(jobs)]
        n_products = out_ref.shape[0]
        for job in _combination_jobs(out_ref, 2 if n_products == len(_HOPCROFT_KERR) else 4,
                                     _WEIGHT, lambda i, j, rows: wide_ref[i, j, rows],
                                     {r: r for r in range(n_products)}):
            side.add(wide_ref, job)

    def staged_rows(part, rows, packing):
        count = min(len(rows), _CHUNK)
        for first in rows[::count]:
            c, offset = divmod(first, _CHUNK)
            if isinstance(part, int):
                source = _PARTS if c == part else c
            else:
                source = jnp.where(part == c, _PARTS, c)
            yield _aligned(source * (_CHUNK // packing) + offset // packing, count // packing)

    def block_copies(m, part, slot, rows=pl.ds(0, d_model // 2)):
        src = (wot_hbm, w1_hbm, w2t_hbm, w3_hbm)[m].bitcast(words)
        dst, sem = stage_ref.at[slot], stage_sem.at[slot]
        if m == _WO:
            return [pltpu.make_async_copy(src.at[_TILES * part + j, rows],
                                          dst.at[rows, pl.ds(j * _LANES, _LANES)], sem)
                    for j in range(_TILES)]
        return [pltpu.make_async_copy(src.at[rows, _aligned(part * width, width)],
                                      dst.at[rows], sem)]

    def shared_copies(m):
        return [copy for c in range(_PARTS) for copy in block_copies(
            m, c, shared_slot + m, pl.ds(c * _CHUNK // 2, _CHUNK // 2))]

    def last_copies(m):
        return block_copies(m, _PARTS, last_slots[m])

    def staged(slot, part, rows, j):
        tile = pltpu.bitcast(jnp.concatenate(
            [stage_ref[slot, piece, j * _LANES:(j + 1) * _LANES]
             for piece in staged_rows(part, rows, 2)], axis=0), bf16)
        return (tile.T if len(rows) == _LANES else tile).astype(f32)

    def store_block(m, out_ref, block):
        if m in scales:
            combine_weights(out_ref, stage_ref, lambda *at: block(*at) * scales[m], _SLAB, _TILES)
        else:
            combine_weights(out_ref, stage_ref, block, _LANES, 1)

    def store_part(m, out_ref, part, slot):
        store_block(m, out_ref.at[part], lambda rows, j: (
            staged(slot, part, rows, j) - staged(shared_slot + m, part, rows, j)))

    def store_shared(m, out_ref):
        store_block(m, out_ref.at[out_ref.shape[0] - 1],
                    functools.partial(staged, shared_slot + m, _PARTS))

    def store_last(m, out_ref):
        part = {_W1: 0, _W3: 1, _W2: _PARTS}[m]

        def block(rows, j):
            own = staged(last_slots[m], part, rows, j)
            if m != _W2 and rows[0] // _CHUNK == 1 - part:
                other = _W1 + _W3 - m
                return own - staged(last_slots[other], part, rows, j) * (
                    scales[other] / scales[m])
            return own

        store_block(m, out_ref.at[_PARTS], block)
        for j in range(_TILES):
            rows = range(part * _CHUNK, (part + 1) * _CHUNK)
            wplain_ref[int(m == _W2), j, pl.ds(part % 2 * _CHUNK, _CHUNK)] = (staged(
                last_slots[m], _PARTS, rows, j) * scales.get(m, 1.0)).astype(bf16)

    def first_step_copies(t):
        return [copy for n in range(2) for copy in block_copies(_W3, 2 * t + n, 3 * (t & 1) + n)
                ] + (shared_copies(_W3) + block_copies(_W1, 0, 2) if t == 0
                     else last_copies(_W3) if t == 1 else last_copies(_W1) if t == 2 else [])

    def load_weights(early_in_ref, early_shared_ref, head_ref, head_sem, *rows_refs):
        n_early = n_io - 1
        products = len(_HOPCROFT_KERR)

        def pair_copies(w, part, slot, rows):
            src = (wq_hbm, wk_hbm, wv_hbm)[w].bitcast(words)
            return [pltpu.make_async_copy(src.at[rows, 2 * part + n, :],
                                          head_ref.at[slot, n, rows], head_sem.at[slot])
                    for n in range(2)]

        def head_copies(part, which=range(3)):
            return [copy for w in which
                    for copy in pair_copies(w, part, 3 * w + 2 * (part & 1), pl.ds(0, d_model))]

        def shared_head_copies(w):
            return [copy for c in range(_PARTS)
                    for copy in pair_copies(w, c, 3 * w + 1, pl.ds(c * _CHUNK, _CHUNK))]

        def part_copies(part, which=range(3)):
            return [copy for m in which for copy in block_copies(m, part, 3 * (part & 1) + m)]

        def head(slot, rows, j):
            pair = head_ref[slot, j // 2, rows, :]
            return pltpu.bitcast(pair & words(0xFFFF0000) if j % 2 else pair << 16, f32)

        def store_heads(w, part):
            def block(rows, j):
                rows = next(staged_rows(part, rows, 1))
                tile = head(3 * w + 2 * (part & 1), rows, j) - head(3 * w + 1, rows, j)
                return tile if w else tile * score_scale

            combine_weights(wqkv_ref.at[w, part], head_ref, block, _CHUNK // 2, 2)

        def store_shared_heads(w):
            @pl.loop(0, _LANES // _SLAB)
            def _(n):
                operands = _operands(_levels(2), _WEIGHT, lambda i, j: head(
                    3 * w + 1, _aligned(i * _LANES + n * _SLAB, _SLAB), j) * (
                        1.0 if w else score_scale))
                for r, operand in operands.items():
                    wqkv_ref[w, _PARTS, r, _aligned(n * _SLAB, _SLAB)] = operand().astype(bf16)

        def x_copies(first, last, sem):
            tiles = [(c + 1) % n_io for c in range(first, last)]
            return [pltpu.make_async_copy(xt_hbm.at[:, pl.ds(i * _LANES, _LANES)],
                                          tile_ref.at[i, :d_model], tile_sem.at[sem])
                    for i in tiles]

        def transpose_in(c):
            i = (c + 1) % n_io
            x_ref[i, :_LANES] = _load_packed(tile_ref, i, slice(0, d_model // 2)).T

        def normalize(c):
            for s in range(4):
                _store_rows(rows_refs[c % 3], s // 2, s % 2 * ahead,
                            _layernorm(x_ref[c + 1, s * seg:s * seg + ahead].astype(f32)))

        def fetch(c):
            transpose_in(c)
            if c < n_early:
                normalize(c)

        def prepare(c):
            rows_ref = rows_refs[c % 3]
            for n, job in enumerate(_operand_jobs(early_in_ref.at[c], rows_ref, None)):
                place = 2 * n if c + 2 >= n_early else len(side.jobs)
                side.jobs.insert(place, (c, rows_ref, job))

        def prepare_parts(c):
            for tile in range(_TILES):
                for job in _operand_jobs(early_in_ref.at[c], rows_refs[c % 3], tile):
                    side.add(rows_refs[c % 3], job)

        def project(w, part, c, operand):
            shared = isinstance(part, int) and part == _PARTS

            def keep(f, j, tile):
                early_shared_ref[w, c, f, j] = tile

            def store(f, j, tile):
                early_ref[2 * c + f, w, part, j] = tile.astype(bf16)

            _collect(_levels(2), _WIDE,
                     lambda r: side.dot(operand(r, c), _load_packed(wqkv_ref, w, part, r)),
                     lambda f, j: None if shared else early_shared_ref[w, c, f, j],
                     keep if shared else store)

        def project_shared(pending, first, last):
            operand = _operand_loader(early_in_ref, 2, _PARTS)
            ready = pending + [(w, c) for c in range(first, last) for w in range(3)]
            held = [(w, c) for w, c in ready if w and c + 2 >= last and last < n_early]
            fetch(first)
            side.add(tile_ref, functools.partial(fetch, first + 1))
            prepare(first)
            side.spread(len(pending) * products)
            for w, c in ready:
                if w == 0:
                    side.finish(c)
                    if c + 2 < last + (last == n_early):
                        side.add(tile_ref, functools.partial(fetch, c + 2))
                    if c + 1 < last:
                        prepare(c + 1)
                    prepare_parts(c)
                    if c + 3 == n_early:
                        store_heads(0, 0)
                    side.spread((3 * (n_early - c) - .5 if c + 3 >= n_early
                                 else 1 if (1, c) in held else 3) * products)
                if (w, c) not in held:
                    project(w, _PARTS, c, operand)
            side.finish()
            return held

        def project_part(part, which):
            operand = _operand_loader(early_in_ref, 2, part)
            side.count = 1
            side.spread((len(which) * n_early - .7) * products)
            for w in which:
                for c in range(n_early):
                    project(w, part, c, operand)
            side.finish()

        def store_parts(part, other, which=range(3)):
            for m, out_ref in enumerate((wo_ref, w1_ref, w2_ref)):
                if m in which:
                    store_part(m, out_ref, part, 3 * (part & 1) + m)
                other(m)

        middle = n_io // 2
        _start(x_copies(0, 3, 0) + shared_head_copies(0))
        for w in range(3):
            head_ref[3 * w + 1, :, width:d_model] = jnp.zeros((2, _CHUNK, d_head), words)
        for m in range(4):
            stage_ref[shared_slot + m, width // 2:d_model // 2] = jnp.zeros(
                (_CHUNK // 2, width), words)
        side.keep_in_memory(early_in_ref, early_shared_ref)
        _wait(x_copies(0, 3, 0))
        _start(shared_head_copies(1) + shared_head_copies(2))
        for c in range(3):
            transpose_in(c)
        copies = (x_copies(3, middle, 0), x_copies(middle, middle + 1, 1),
                  x_copies(middle + 1, n_io, 1) + head_copies(0, [0]))
        for w in range(2):
            _wait(shared_head_copies(w))
            _start(copies[w])
            store_shared_heads(w)
            for c in range(3):
                if w:
                    prepare_parts(c)
                else:
                    normalize(c)
                    prepare(c)
            side.spread(2.5 * products)
            for c in range(3):
                side.finish(c)
                project(w, _PARTS, c, _operand_loader(early_in_ref, 2, _PARTS))
            side.finish()
        _wait(shared_head_copies(2) + copies[0])
        _start(copies[2])
        store_shared_heads(2)
        held = project_shared([(2, c) for c in range(3)], 3, middle)
        _wait(copies[1] + copies[2])
        copies = part_copies(0, (_WO, _W2)) + shared_copies(_WO) + shared_copies(_W2)
        _start(head_copies(0, [1, 2]) + copies + head_copies(1))
        project_shared(held, middle, n_early)
        _wait(head_copies(0, [1, 2]))
        _start(shared_copies(_W1))
        store_heads(1, 0)
        store_heads(2, 0)
        project_part(0, [0])
        _wait(copies + head_copies(1))
        _start(part_copies(1) + head_copies(2))
        store_parts(0, lambda w: store_heads(w, 1), (_WO, _W2))
        project_part(0, [1, 2])
        _wait(shared_copies(_W1))

        @pl.loop(1, _PARTS - 1, unroll=True)
        def _(part):
            _wait(part_copies(part) + head_copies(part + 1))
            _start(part_copies(part + 1))
            pl.when(part + 2 < _PARTS)(
                lambda: _start(head_copies(jnp.minimum(part + 2, _PARTS - 1))))
            pl.when(part + 2 == _PARTS)(lambda: _start(last_copies(_W2)))
            store_parts(part, lambda w: store_heads(w, part + 1))
            project_part(part, range(3))

        _wait(part_copies(_PARTS - 1) + last_copies(_W2))
        _start(first_step_copies(0))
        store_parts(_PARTS - 1, lambda m: store_last(_W2, w2_ref) if m == _W1
                    else store_shared(m, w2_ref if m == _W2 else wo_ref))
        project_part(_PARTS - 1, range(3))

    def run_layers(w3_ref, pair_rows_ref, pair_in_ref, solo_rows_ref, solo_in_ref, ffn_rows_ref,
                   ffn_in_ref, attn_shared_ref, ffn_shared_ref, partial_ref, qkv_ref, heads_ref,
                   hidden_ref, attn_sum_ref, ffn_sum_ref, mem_ref, block_ref, second_ref):
        def segment(s):
            return s >> 2, _aligned((s & 3) * seg, seg)

        def transpose_out(i):
            tile_ref.bitcast(words)[i, :d_model // 2] = pltpu.bitcast(x_ref[i, :_LANES].T, words)

        def contract(groups, part, rows_ref, weight_ref, sum_ref, begun):
            operands = _operands(_levels(groups), _WIDE, lambda f, j: rows_ref[part, f, j])

            def targets(i):
                return [_TILES if 2 * i + half == part else i for half in range(2)]

            def start(f, i):
                low, high = (
                    sum_ref[f, n] if (n, half) in begun else None if groups < 4
                    else block_ref[f, :, n * _LANES:(n + 1) * _LANES]
                    for half, n in enumerate(targets(i)))
                if targets(i) == [i, i] and ((i, 0) in begun) == ((i, 1) in begun):
                    return low
                if low is None and high is None:
                    return None
                lanes = jax.lax.broadcasted_iota(jnp.int32, sum_ref.shape[-2:], 1)
                return jnp.where(lanes < _CHUNK, 0.0 if low is None else low,
                                 0.0 if high is None else high)

            def finish(f, i, tile):
                if targets(i) == [i, i]:
                    sum_ref[f, i] = tile
                else:
                    for half, n in enumerate(targets(i)):
                        lanes = slice(half * _CHUNK, (half + 1) * _CHUNK)
                        sum_ref[f, n, :, lanes] = tile[:, lanes]

            _collect(_levels(groups), _MODEL,
                     lambda r: side.dot(operands[r](), _load_packed(weight_ref, part, r)),
                     start, finish, partial_ref.at[part % 2])
            begun.update((n, half) for i in range(_TILES) for half, n in enumerate(targets(i)))

        def keep_and_add(ref, part, f, j, tile):
            total = ref.shape[0] - 1
            ref[part, f, j] = tile
            if 0 < part < _PARTS:
                ref[total, f, j] = ref[total if part > 1 else 0, f, j] + tile

        def project(groups, w, part):
            in_ref = pair_in_ref if groups == 2 else solo_in_ref
            rows = slice(0, in_ref.shape[1])
            side.finish(("P", None), ("P", part // 2))
            operand = _operand_loader(in_ref, groups, part)
            out_ref = qkv_ref.at[w, part % qkv_ref.shape[1]]
            done = {}

            def finish(f, j, tile):
                done[f, j] = tile
                if part == _PARTS:
                    attn_shared_ref[w, f, j, rows] = tile
                elif groups == 2 and (1 - f, j) in done:
                    upper, lower = done[0, j], done[1, j]
                    out_ref[j, :2 * size - ahead] = jnp.concatenate(
                        [upper[n_mem:n_mem + ahead], upper[:n_mem], lower[:n_mem],
                         upper[n_mem + ahead:], lower[n_mem:]], axis=0).astype(bf16)
                elif groups == 1 and (0, j ^ 1) in done:
                    a, b = done[0, j & ~1], done[0, j | 1]
                    out_ref[j | 1] = jnp.concatenate(
                        [a[n_mem:], a[:n_mem], b], axis=0).astype(bf16)

            _collect(_levels(groups), _WIDE,
                     lambda r: side.dot(operand(r), _load_packed(wqkv_ref, w, part, r)),
                     lambda f, j: attn_shared_ref[w, f, j, rows] if part < _PARTS else None,
                     finish)

        def projected(groups, t, place, w, head):
            part, j = divmod(head, _TILES)
            index = w, part % qkv_ref.shape[1], j
            if groups == 1:
                rows = [_load_words(qkv_ref, *index)]
            else:
                rows = [_load_words(early_ref, (t - _LAG) >> 1, w, part, j,
                                    _aligned(place * (ahead // 2), ahead // 2)),
                        _load_words(qkv_ref, *index, slice(0, size - ahead // 2))]
            if w == 1:
                rows.append(jnp.zeros((_CHUNK - size, d_head), words))
            return pltpu.bitcast(jnp.concatenate(rows, axis=0), bf16)

        def by_group(tile):
            return enumerate(tile[f * seg:(f + 1) * seg] for f in range(4))

        def expand(g):
            plain = 2 * _PARTS + 2
            if g == plain:
                x = jnp.concatenate([ffn_rows_ref[f, 0, :seg] for f in range(4)], axis=0)
                for j in range(_TILES):
                    for f, tile in by_group(_dot(x.astype(bf16), _load_packed(wplain_ref, 0, j))):
                        ffn_shared_ref[2, f, j] = tile
                return
            part, up = divmod(g if g < plain else g - 1, 2)
            chunk = up if part == _PARTS else min(part, _PARTS)
            side.finish(("G", None), ("G", chunk // 2))
            operand = _operand_loader(ffn_in_ref, 4, chunk)
            weight_ref = w3_ref if up else w1_ref

            def finish(f, j, tile):
                if part > _PARTS:
                    ffn_shared_ref[up, f, j] = tile
                elif up:
                    keep_and_add(hidden_ref, part, f, j, hidden_ref[part, f, j] * tile)
                else:
                    hidden_ref[part, f, j] = _scaled_silu(tile)

            _collect(_levels(4), _WIDE,
                     lambda r: side.dot(operand(r), _load_packed(weight_ref, part, r)),
                     lambda f, j: None if part > _PARTS else ffn_shared_ref[
                         2 if part == _PARTS else up, f, j],
                     finish, partial_ref.at[g % 2])

        def reduce(g, begun):
            if not begun:
                for f in range(4):
                    rest = block_ref[f, :, width:]
                    ffn_sum_ref[f, _TILES] = jnp.concatenate([rest, jnp.zeros_like(rest)], axis=1)
                begun.update([(_TILES, 0), (_TILES, 1)])
            if g < w2_ref.shape[0]:
                contract(4, g, hidden_ref, w2_ref, ffn_sum_ref, begun)
                return
            total = None
            for j in range(_TILES):
                rows = jnp.concatenate([hidden_ref[_PARTS, f, j] for f in range(4)], axis=0)
                total = _accumulate(total, 1, _dot(
                    _load_packed(wplain_ref, 1, j, slice(0, _CHUNK // 2)), rows.astype(bf16), 1))
            for f, tile in by_group(_value(total).T):
                ffn_sum_ref[f, _TILES, :, :_CHUNK] += tile

        def layer_input(t, place, layer):
            return x_ref[segment(t)].astype(f32) if layer == 0 else second_ref[place]

        def begin_step(t, place, layers):
            h = _layernorm(layer_input(t, place, layers[-1]))
            if len(layers) == 1:
                rows_ref, in_ref = solo_rows_ref, solo_in_ref
                _store_rows(rows_ref, 0, n_mem, h)
            else:
                rows_ref, in_ref, cut = pair_rows_ref, pair_in_ref, ahead // 2
                _store_rows(rows_ref, 0, n_mem, _layernorm(layer_input(t, place, 0)[ahead:]))
                _store_rows(rows_ref, 0, seg - cut, h[:cut])
                _store_rows(rows_ref, 1, n_mem, h[cut:])
            for f, layer in enumerate(layers):
                _store_rows(rows_ref, f, 0, mem_ref[layer])
            for tile in [None, *range(_TILES)]:
                for job in _operand_jobs(in_ref, rows_ref, tile):
                    side.add(rows_ref, job, ("P", tile))

        def close_step(t, place, layers):
            for f, layer in enumerate(layers):
                out = _load_rows(attn_sum_ref, f)
                mem_ref[layer] = out[:n_mem]
                index = 2 * layer + place if len(layers) == 2 else place
                block_ref[index] = layer_input(t, place, layer) + out[n_mem:]

        def run(order, layers=(), t=0, place=0):
            groups, first = len(layers), t
            attn_begun, ffn_begun, probs = set(), set(), {}
            for name in order.split():
                stage, g = name[0], int(name[1:] or 0)
                if stage == "N":
                    begin_step(t, place, layers)
                elif stage == "P":
                    project(groups, g % 3, g // 3)
                elif stage == "S" and (groups == 2 or g % 2):
                    q, k = (projected(groups, first, place, w, g) for w in range(2))
                    s = jnp.where(visible, _dot(q, k, 1), fill)
                    p = jnp.exp2(s - jnp.max(s, axis=-1, keepdims=True))
                    inv = pltpu.reciprocal(jnp.sum(p, axis=-1, keepdims=True), approx=True)
                    probs[g] = p[:, :2 * size].astype(bf16), inv
                elif stage == "V" and (groups == 2 or g % 2):
                    o = _dot(probs[g][0], projected(groups, first, place, 2, g)) * probs[g][1]
                    halves = jnp.concatenate([o[seg:size], o[:seg]], axis=0), o[size:]
                    for f, half in enumerate(halves):
                        index = (f, g % _TILES) if groups == 2 else (0, g % _TILES - 1 + f)
                        keep_and_add(heads_ref, g // _TILES, *index, half)
                elif stage == "O":
                    contract(groups, g, heads_ref, wo_ref, attn_sum_ref, attn_begun)
                elif stage == "A":
                    close_step(t, place, layers)
                    t, place, attn_begun = t + 1, place + 1, set()
                elif stage == "M":
                    _store_rows(ffn_rows_ref, g, 0, _layernorm(block_ref[g]))
                elif stage == "F":
                    tile = g if g < _TILES else None
                    for job in _operand_jobs(ffn_in_ref, ffn_rows_ref, tile):
                        side.add(ffn_rows_ref, job, ("G", tile))
                elif stage == "G":
                    expand(g)
                elif stage == "D":
                    reduce(g, ffn_begun)
                elif stage == "E":
                    for s in range(2):
                        second_ref[g + s] = _load_rows(ffn_sum_ref, s)
                        x_ref[segment(jnp.maximum(first + g - 2 * _LAG, 0) + s)] = _load_rows(
                            ffn_sum_ref, 2 + s).astype(bf16)
                elif stage == "T":
                    side.add(x_ref, functools.partial(transpose_out, g))
                elif stage == "C":
                    _start(out_copies[:n_io - 1])
                elif stage == "Z":
                    for _ in range(g):
                        side.add()
                elif stage == "W":
                    side.spread(g)
                elif stage == "X":
                    side.finish()

        visible, fill = _attention_masks(n_mem, seg)
        side.keep_in_memory(pair_in_ref, solo_rows_ref, solo_in_ref, ffn_in_ref, attn_shared_ref,
                            ffn_shared_ref, partial_ref, qkv_ref, heads_ref, hidden_ref,
                            attn_sum_ref, ffn_sum_ref)
        attn_sum_ref[...] = jnp.zeros_like(attn_sum_ref)
        mem_copy.wait()
        mem_ref[0] = mem0_ref[...].astype(f32)
        for t in range(_LAG):
            run("N", (0,), t, t)
            _wait(first_step_copies(t))
            _start(first_step_copies(t + 1) if t + 1 < _LAG else [mem_copy])
            (store_shared, store_last)[t // 2](*((_W1, w1_ref), (_W3, w3_ref))[t % 2])
            for n in range(2):
                store_part(_W3, w3_ref, 2 * t + n, 3 * (t & 1) + n)
            if t == 0:
                store_part(_W1, w1_ref, 0, 2)
            run("W540 " + _ATTENTION + " X", (0,), t, t)
        mem_copy.wait()
        mem_ref[1] = mem0_ref[...].astype(f32)
        run(_SWIGLU)
        for s in range(2):
            second_ref[s] = _load_rows(ffn_sum_ref, s)
            ffn_sum_ref[s] = ffn_sum_ref[2 + s]
        pl.loop(0, 2, unroll=True)(lambda n: run(_STEP, (0, 1), _LAG + n, n))
        run("M0 M2 M1 M3 G18")

        @pl.loop(_LAG // 2 + 1, n_seg // 2)
        def _(b):
            run(_TWO_STEPS + " X", (0, 1), 2 * b)

        out_copies = [
            pltpu.make_async_copy(tile_ref.at[i, :d_model],
                                  outt_hbm.at[:, pl.ds(i * _LANES, _LANES)], tile_sem.at[0])
            for i in range(n_io)]
        run(_LAST_STEPS, (1,), n_seg)
        pl.loop(2, _LAG, unroll=True)(lambda n: run(_STEP, (1,), n_seg + n, n))
        run(_SWIGLU.replace("W500", " ".join(f"T{i} Z3" for i in range(n_io - 1)) + " W900")
            .replace("D5", "X C D5"))
        for s in range(_LAG):
            x_ref[segment(n_seg - _LAG + s)] = _load_rows(ffn_sum_ref, s).astype(bf16)
        transpose_out(n_io - 1)
        _start(out_copies[n_io - 1:])
        _wait(out_copies)

    spare = 8
    mem_copy = pltpu.make_async_copy(mem0_hbm, mem0_ref, mem_sem)
    mem_copy.start()
    pl.run_scoped(
        load_weights,
        pltpu.VMEM((n_io - 1, len(_operand_slots(2)), seg, _LANES), bf16),
        pltpu.VMEM((3, n_io - 1, 2, _TILES, seg, _LANES), f32),
        pltpu.VMEM((9, 2, d_model + spare, d_head), words),
        pltpu.SemaphoreType.DMA((9,)),
        *[pltpu.VMEM((2, _TILES + 1, seg + spare, _LANES), f32)] * 3)
    pl.run_scoped(
        run_layers,
        pltpu.VMEM(w1_ref.shape, bf16),
        pltpu.VMEM((2, _TILES + 1, seg + spare, _LANES), f32),
        pltpu.VMEM((len(_operand_slots(2)), seg, _LANES), bf16),
        pltpu.VMEM((1, _TILES + 1, size + spare, _LANES), f32),
        pltpu.VMEM((len(_operand_slots(1)), size, _LANES), f32),
        pltpu.VMEM((4, _TILES + 1, seg + spare, _LANES), f32),
        pltpu.VMEM((len(_operand_slots(4)), seg, _LANES), bf16),
        pltpu.VMEM((3, 2, _TILES, size, _LANES), f32),
        pltpu.VMEM((3, 4, _TILES, seg, _LANES), f32),
        pltpu.VMEM((2, 4, _TILES, seg, _LANES), f32),
        pltpu.VMEM((3, 3, _TILES, 2 * size, _LANES), bf16),
        pltpu.VMEM((_PARTS + 1, 2, _TILES, size, _LANES), f32),
        pltpu.VMEM((_PARTS + 2, 4, _TILES, seg, _LANES), f32),
        pltpu.VMEM((2, _TILES + 1, size, _LANES), f32),
        pltpu.VMEM((4, _TILES + 1, seg, _LANES), f32),
        pltpu.VMEM((2, n_mem, d_model), f32),
        pltpu.VMEM((4, seg, d_model), f32),
        pltpu.VMEM((4, seg, d_model), f32))


@functools.partial(jax.jit, static_argnames=("A_seg_len",))
def pallas_interleave_layers__memory_aug_recurrent_mem_tr__glu_gated_swiglu__prompt_kernel(
    A_x: jax.Array,
    A_mem0: jax.Array,
    A_Wq: jax.Array,
    A_Wk: jax.Array,
    A_Wv: jax.Array,
    A_Wo: jax.Array,
    A_seg_len: int,
    B_x: jax.Array,
    B_w1: jax.Array,
    B_w3: jax.Array,
    B_w2: jax.Array,
):
    del B_x
    _, n_tok, d_model = A_x.shape
    n_mem = A_mem0.shape[1]
    _, n_heads, d_head = A_Wq.shape
    seg = A_seg_len
    assert A_x.shape[0] == 1 and _LAG * seg == d_head == _LANES and 4 * n_mem == seg
    assert n_heads == _PARTS * _TILES and d_model == (_PARTS + 1) * _CHUNK
    assert B_w1.shape[1] == (_PARTS + 1) * _TILES * _LANES and n_tok == 16 * _LANES
    bf16 = jnp.bfloat16
    attn_blocks = (_PARTS + 1, len(_HOPCROFT_KERR), _LANES, _LANES)
    ffn_blocks = (_PARTS + 2, len(_STRASSEN) ** 2, _LANES, _LANES)
    hbm = pl.BlockSpec(memory_space=pltpu.HBM)
    out_t = pl.pallas_call(
        functools.partial(_kernel, seg=seg),
        out_shape=jax.ShapeDtypeStruct((d_model, n_tok), A_x.dtype),
        in_specs=[hbm] * 9,
        out_specs=hbm,
        scratch_shapes=[
            pltpu.VMEM((n_mem, d_model), bf16),
            pltpu.VMEM((n_tok // _LANES, d_model + _SLAB, _LANES), bf16),
            pltpu.VMEM((n_tok // _LANES, _LANES + _SLAB, d_model), bf16),
            pltpu.VMEM(((n_tok // seg - _LAG) // 2, 3, _PARTS, _TILES, seg, _LANES), bf16),
            pltpu.VMEM((3, *attn_blocks), bf16),
            pltpu.VMEM(attn_blocks, bf16),
            pltpu.VMEM(ffn_blocks, bf16),
            pltpu.VMEM(ffn_blocks, bf16),
            pltpu.VMEM((2, _TILES, _LANES, _LANES), bf16),
            pltpu.VMEM((11, (d_model + _SLAB) // 2, _TILES * _LANES), jnp.uint32),
            pltpu.SemaphoreType.DMA((11,)),
            pltpu.SemaphoreType.DMA(()),
            pltpu.SemaphoreType.DMA((2,)),
            *[pltpu.VMEM((_TILES, _TILES, _LANES + _SLAB // 2, _LANES), jnp.float32)] * 2,
        ],
        compiler_params=pltpu.CompilerParams(
            vmem_limit_bytes=127 * 1024 * 1024,
            flags={"XLA_TPU_FORCE_LP_LLO_SCHEDULER": True,
                   "XLA_TPU_EVENLY_DISTRIBUTE_CRITICAL_NODES": True}),
    )(A_x.reshape(n_tok, d_model).T, A_mem0.reshape(n_mem, d_model), A_Wq, A_Wk, A_Wv,
      A_Wo.transpose(0, 2, 1), B_w1, B_w2.T, B_w3)
    return out_t.T.reshape(A_x.shape)
```

```python
import functools
import math

import jax
import jax.numpy as jnp
import jax.experimental.pallas as pl
import jax.experimental.pallas.tpu as pltpu

_EPS = 1e-05
_MASKED = -1000000000.0
_LOG2E = math.log2(math.e)
_LANES = 128
_CHUNK = _LANES // 2
_SLAB = 16
_TILES = 4
_PARTS = 2 * _TILES
_LAG = 4
_WO, _W1, _W2, _W3 = range(4)
_MODEL, _WEIGHT, _WIDE = range(3)
_HOPCROFT_KERR = (
    (((1, 1, 2),), ((1, 2, 0), (1, 2, 2), (1, 2, 3), (-1, 1, 2)), ((1, 2, 2),)),
    (((1, 2, 2),), ((1, 2, 1), (1, 2, 2), (-1, 0, 2), (-1, 3, 2)), ((1, 0, 2),)),
    (((1, 0, 2), (1, 0, 3)), ((1, 2, 3),), ((-1, 2, 2), (1, 2, 3))),
    (((1, 2, 2), (1, 0, 3)), ((1, 2, 3), (1, 3, 2)), ((1, 2, 2), (-1, 1, 3))),
    (((1, 2, 2), (1, 2, 3)), ((1, 3, 2),), ((-1, 1, 2), (1, 1, 3))),
    (((1, 0, 0), (1, 0, 2)), ((1, 2, 0),), ((1, 2, 0), (-1, 2, 2))),
    (((1, 0, 0), (1, 2, 2)), ((1, 0, 2), (1, 2, 0)), ((-1, 1, 0), (1, 2, 2))),
    (((1, 2, 0), (1, 2, 2)), ((1, 0, 2),), ((1, 1, 0), (-1, 1, 2))),
    (((1, 0, 1), (1, 0, 2)), ((1, 2, 1),), ((1, 0, 1), (-1, 0, 2))),
    (((1, 0, 1), (1, 1, 2)), ((1, 1, 2), (1, 2, 1)), ((1, 1, 1), (1, 0, 2))),
    (((1, 1, 1), (1, 1, 2)), ((1, 1, 2),), ((-1, 1, 1), (1, 1, 2))),
    (((1, 1, 1), (1, 1, 3)), ((1, 0, 3), (-1, 1, 3)), ((1, 2, 1), (-1, 2, 3))),
    (((1, 0, 0), (1, 0, 1), (1, 0, 3)), ((1, 0, 3),), ((1, 2, 1), (-1, 2, 0), (1, 2, 3))),
    (((1, 2, 0), (1, 2, 1), (1, 0, 3)), ((1, 0, 3), (1, 3, 0)),
     ((1, 2, 0), (-1, 2, 1), (-1, 1, 3))),
    (((1, 2, 0), (1, 2, 1), (1, 2, 3)), ((1, 3, 0),), ((1, 1, 1), (-1, 1, 0), (1, 1, 3))),
    (((1, 1, 3),), ((1, 0, 3), (-1, 1, 3), (1, 3, 0), (1, 3, 2), (1, 3, 3)), ((1, 1, 3),)),
    (((1, 2, 1), (1, 2, 3)), ((1, 3, 0), (1, 3, 1)), ((1, 0, 1), (-1, 0, 3))),
    (((1, 1, 3), (-1, 2, 1)), ((1, 3, 0), (1, 3, 1), (-1, 0, 3), (1, 1, 3)),
     ((1, 2, 1), (-1, 0, 3))),
    (((1, 0, 3),), ((1, 3, 0), (1, 3, 1), (-1, 0, 3), (-1, 2, 3), (1, 3, 3)), ((1, 0, 3),)),
    (((1, 1, 0), (1, 1, 1)), ((1, 0, 3), (1, 1, 0)), ((1, 2, 0), (-1, 2, 1))),
    (((1, 2, 1), (-1, 1, 0)), ((1, 0, 1), (1, 1, 0)), ((1, 0, 0), (-1, 2, 1))),
    (((1, 0, 1),), ((1, 1, 0), (1, 1, 1), (1, 1, 3), (-1, 0, 3), (-1, 2, 1)), ((1, 2, 1),)),
    (((1, 2, 0), (1, 2, 1)), ((1, 0, 1), (1, 3, 0)), ((-1, 0, 0), (1, 0, 1))),
    (((1, 2, 1),), ((1, 3, 0), (1, 3, 1), (1, 0, 1), (-1, 1, 1), (-1, 1, 2)), ((1, 1, 1),)),
    (((1, 0, 0),), ((1, 0, 0), (1, 0, 1), (-1, 2, 0)), ((1, 0, 0),)),
    (((1, 1, 0),), ((1, 0, 0), (1, 0, 2), (-1, 1, 0)), ((1, 1, 0),)),
)
_RUNS = (5, 11, 19, 24, 24)
_STRASSEN = (
    (((-1, 2, 0),), ((1, 0, 0), (1, 0, 1)), ((1, 1, 1),)),
    (((1, 1, 0), (1, 1, 1)), ((1, 0, 0),), ((1, 1, 0), (-1, 1, 1))),
    (((1, 1, 1),), ((1, 1, 0), (-1, 0, 0)), ((1, 2, 0),)),
    (((1, 0, 0), (1, 1, 1)), ((1, 0, 0), (1, 1, 1)), ((1, 0, 0), (1, 1, 1))),
    (((1, 0, 0),), ((1, 0, 1), (-1, 1, 1)), ((1, 2, 1),)),
    (((1, 0, 0), (1, 0, 1)), ((1, 1, 1),), ((-1, 0, 0), (1, 0, 1))),
    (((1, 2, 1),), ((1, 1, 0), (1, 1, 1)), ((1, 0, 0),)),
)
_ATTENTION = (
    "P24 P25 P26 P0 P1 P2 S0 S1 S2 S3 P3 P4 V0 V1 V2 V3 P5 S4 S5 S6 S7 O0 P6 P7 V4 V5 V6 V7 "
    "P8 S8 S9 S10 S11 O1 P9 P10 V8 V9 V10 V11 P11 S12 S13 S14 S15 O2 P12 P13 V12 V13 V14 V15 "
    "P14 S16 S17 S18 S19 O3 P15 P16 V16 V17 V18 V19 P17 S20 S21 S22 S23 P18 P19 V20 V21 V22 "
    "V23 P20 S24 S25 S26 S27 P21 P22 V24 V25 V26 V27 P23 S28 S29 S30 S31 O4 V28 V29 V30 V31 "
    "O5 O6 O7 O8 A")
_STEP = "N W200 " + _ATTENTION
_SWIGLU = (
    "M0 M1 M2 M3 F4 X F0 F1 F2 F3 W500 G18 G19 G20 G16 G17 G0 D8 D10 G1 G2 D0 G3 G4 D1 G5 G6 "
    "D2 G7 G8 D3 G9 G10 D4 G11 G12 G13 G14 D5 G15 D6 D7 D9")
_TWO_STEPS = (
    "E F4 X N Z11 G19 F0 W250 G20 P24 P25 P26 P0 G16 P1 P2 G17 S0 S1 S2 S3 P3 P4 V0 V1 V2 V3 "
    "P5 G0 S4 S5 S6 S7 O0 G1 P6 P7 V4 V5 V6 V7 P8 D8 S8 S9 S10 S11 O1 F1 W200 G2 P9 P10 V8 V9 "
    "V10 V11 P11 S12 S13 S14 S15 O2 D0 P12 P13 V12 V13 V14 V15 P14 S16 S17 S18 S19 O3 G3 P15 "
    "P16 V16 V17 V18 V19 P17 S20 S21 S22 S23 O4 P18 G4 P19 V20 V21 V22 V23 P20 S24 S25 S26 "
    "S27 O5 F2 W160 D1 P21 P22 V24 V25 V26 V27 P23 S28 S29 S30 S31 O6 G5 V28 V29 V30 V31 G6 "
    "O7 O8 A Z4 N W200 D2 G7 D3 P24 P25 P26 G8 P0 P1 P2 S0 S1 S2 S3 P3 P4 V0 V1 V2 V3 P5 G9 "
    "S4 S5 S6 S7 O0 F3 W120 P6 G10 P7 V4 V5 V6 V7 P8 S8 S9 S10 S11 O1 D4 P10 P9 V8 V9 V10 V11 "
    "P11 S12 S13 S14 S15 O2 G11 P12 P13 V12 V13 V14 V15 P14 S16 S17 S18 S19 O3 G12 P15 P16 "
    "V16 V17 V18 V19 P17 S20 S21 S22 S23 O4 P18 P19 V20 V21 V22 V23 P20 S24 S25 S26 S27 O5 "
    "G14 G13 P21 P22 V24 V25 V26 V27 P23 S28 S29 S30 S31 O6 D5 M0 V28 V29 V30 V31 G15 O7 O8 "
    "M2 D9 A D10 M3 D6 M1 D7 G18")
_LAST_STEPS = (
    "E F4 X N F0 F1 W400 G19 G20 " + _ATTENTION.replace("O0", "O0 G16 G17 G0 D8 G1 G2 D0 G3")
    + " N F2 F3 W450 G4 D1 D10 G5 G6 D2 G7 G8 D3 G9 G10 D4 G11 G12 G13 G14 D5 G15 D6 D7 D9 E2 "
    + _ATTENTION)


def _layernorm(x):
    m = jnp.mean(x, axis=-1, keepdims=True)
    d = x - m
    v = jnp.mean(d * d, axis=-1, keepdims=True)
    return d * jax.lax.rsqrt(v + _EPS)


def _scaled_silu(x):
    return x * pltpu.reciprocal(1.0 + jnp.exp2(x), approx=True)


def _dot(a, b, axis=0):
    return jax.lax.dot_general(a, b, (((1,), (axis,)), ((), ())),
                               preferred_element_type=jnp.float32)


def _load_words(ref, *index):
    return ref[index] if ref.dtype == jnp.float32 else ref.bitcast(jnp.uint32)[index]


def _load_packed(ref, *index):
    return pltpu.bitcast(_load_words(ref, *index), ref.dtype)


def _aligned(first, size):
    return pl.ds(first if isinstance(first, int) else pl.multiple_of(first, size), size)


def _accumulate(total, sign, value):
    if total is None:
        return sign, value
    if total[0] == sign:
        return sign, jax.lax.add(total[1], value)
    return 1, jax.lax.sub(*((total[1], value) if sign < 0 else (value, total[1])))


def _value(total):
    return total[1] if total[0] > 0 else -total[1]


def _levels(groups):
    if groups == 4:
        return [dict(enumerate(_STRASSEN))] * 2
    if groups == 2:
        return [dict(enumerate(_HOPCROFT_KERR))]

    def upper(terms):
        return tuple((sign, 0, i) for sign, f, i in terms if f != 1)

    return [{r: (upper(model), weight, upper(wide))
             for r, (model, weight, wide) in enumerate(_HOPCROFT_KERR)
             if upper(model) and upper(wide)}]


def _combination(terms, side, block):
    total = None
    for sign, a, b in terms:
        if side == _WEIGHT or a < 2:
            total = _accumulate(total, sign, block(a, b))
        else:
            total = _accumulate(total, *_accumulate(
                (sign, block(0, b)), -sign if side == _MODEL else sign, block(1, b)))
    return _value(total)


def _operands(levels, side, block):
    level, *inner = levels
    if not inner:
        block = functools.cache(block)
        return {r: functools.partial(_combination, product[side], side, block)
                for r, product in level.items()}
    operands = {}
    for r, product in level.items():
        def sub_block(a, b, terms=product[side]):
            return _combination(terms, side, lambda f, i: block(2 * f + a, 2 * i + b))

        for n, operand in _operands(inner, side, sub_block).items():
            operands[r * len(inner[0]) + n] = operand
    return operands


def _collect(levels, side, multiply, start, finish, partial_ref=None):
    level, *inner = levels
    terms = [term for product in level.values() for term in product[side]]
    left = {}
    for _, f, i in terms:
        left[f, i] = left.get((f, i), 0) + 1
    for i in sorted({i for _, f, i in terms if f == 2}):
        for f in range(2):
            left[f, i] = left.get((f, i), 0) + 1
    total = {}

    def add(r, f, i, sign, result):
        left[f, i] -= 1
        if f == 2:
            total[f, i] = _accumulate(total.get((f, i)), sign, result)
            if not left[f, i]:
                sign, result = total[f, i]
                add(r, 0, i, sign, result)
                add(r, 1, i, -sign if side == _MODEL else sign, result)
            return
        for (a, b), tile in result.items() if inner else [((0, 0), result)]:
            index = (2 * f + a, 2 * i + b) if inner else (f, i)
            key = f, i, a, b
            if key not in total:
                first = start(*index)
                before = None if first is None else (1, first)
            elif total[key][1] is None:
                before = total[key][0], partial_ref[index]
            else:
                before = total[key]
            total[key] = _accumulate(before, sign, tile)
            if not left[f, i]:
                finish(*index, _value(total[key]))
            elif inner and not any(g in (f, 2) and j == i for _, g, j in level[r + 1][side]):
                partial_ref[index] = total[key][1]
                total[key] = total[key][0], None

    for r, product in level.items():
        if inner:
            result = {}
            _collect(inner, side, lambda n: multiply(r * len(inner[0]) + n), lambda f, i: None,
                     lambda f, i, tile: result.update({(f, i): tile}))
        else:
            result = multiply(r)
        for sign, f, i in product[side]:
            add(r, f, i, sign, result)


@functools.cache
def _operand_slots(groups):
    used = {0: [0]}
    for level in _levels(groups):
        used = {r * len(level) + n: sorted({2 * i + j for i in tiles for _, _, j in terms})
                for r, tiles in used.items() for n, (terms, _, _) in level.items()}
    keys = [(r, tile) for r, tiles in used.items() for tile in [None] + tiles]
    return {key: slot for slot, key in enumerate(keys)}


class _SideJobs:
    def __init__(self, zero):
        self.zero, self.jobs, self.pace, self.due, self.count = zero, [], 0.0, 0.0, -1

    def add(self, source_ref=None, job=None, key=None):
        self.jobs.append((key, source_ref, job))

    @staticmethod
    def cost(ref):
        return 0.7 if ref is not None and ref.dtype == jnp.uint32 else 1.0

    def spread(self, products):
        self.pace = sum(self.cost(ref) for _, ref, _ in self.jobs) / products

    def finish(self, *keys):
        while self.jobs and (not keys or any(key in keys for key, _, _ in self.jobs)):
            _, ref, job = self.jobs.pop(0)
            if ref is not None:
                job()

    def dot(self, a, b):
        result = _dot(a, b)
        self.count += 1
        self.due = self.due + self.pace if self.jobs else 0.0
        while self.jobs and self.due >= 1.0:
            _, ref, job = self.jobs.pop(0)
            self.due -= self.cost(ref)
            if ref is None:
                continue
            rows = 32 // ref.dtype.itemsize
            first = self.count % 4 * (result.shape[0] // rows) // 4 * rows
            value = jax.lax.slice_in_dim(result, first, first + rows)
            index = (self.zero,) * (ref.ndim - 2) + (
                slice(ref.shape[-2] - rows, None), slice(0, _LANES))
            ref[index] = (pltpu.bitcast(value, ref.dtype) if ref.dtype == jnp.uint32
                          else value.astype(ref.dtype))
            job()
        return result

    def keep_in_memory(self, *refs):
        for ref in refs:
            ref[(self.zero,) * (ref.ndim - 2)] = jnp.zeros(ref.shape[-2:], ref.dtype)


def _store_rows(ref, f, first, x):
    rows = slice(first, first + x.shape[0])
    for i in range(_TILES):
        ref[f, i, rows] = x[:, i * _LANES:(i + 1) * _LANES]
    ref[f, _TILES, rows] = jnp.concatenate([x[:, _TILES * _LANES:]] * 2, axis=1)


def _load_rows(ref, f):
    rest = ref[f, _TILES]
    return jnp.concatenate(
        [ref[f, i] for i in range(_TILES)] + [rest[:, :_CHUNK] + rest[:, _CHUNK:]], axis=1)


def _combination_jobs(ref, groups, side, block, slots):
    def job(batch, rows):
        operands = _operands(_levels(groups), side, lambda a, b: block(a, b, rows))
        for r, slot in batch:
            ref[slot, rows] = jax.lax.convert_element_type(operands[r](), ref.dtype)

    batches = {}
    for r, slot in slots.items():
        key = r // len(_STRASSEN) if groups == 4 else sum(r >= cut for cut in _RUNS) % 4
        batches.setdefault(key, []).append((r, slot))
    step = _SLAB if groups > 1 else ref.shape[1]
    return [functools.partial(job, batch, slice(first, first + step))
            for batch in batches.values() for first in range(0, ref.shape[1], step)]


def _operand_jobs(ref, rows_ref, tile):
    groups = rows_ref.shape[0]
    return _combination_jobs(
        ref, groups, _MODEL, lambda f, i, rows: rows_ref[f, _TILES if i == tile else i, rows],
        {r: slot for (r, replaced), slot in _operand_slots(groups).items() if replaced == tile})


def _operand_loader(ref, groups, part):
    slots = _operand_slots(groups)
    rows = ref.shape[-2] * ref.dtype.itemsize // 4
    lanes = jax.lax.broadcasted_iota(jnp.int32, (rows, _LANES), 1)
    replaced = (lanes & _CHUNK) == (part & 1) * _CHUNK
    if isinstance(part, int):
        others = {r: slot for (r, tile), slot in slots.items() if tile == part // 2}
    else:
        others = {}
        for (r, tile), slot in slots.items():
            others[r] = slot if tile is None else jnp.where(part >> 1 == tile, slot, others[r])

    def load(r, *index):
        words = _load_words(ref, *index, slots[r, None])
        if r in others:
            words = jax.lax.select(replaced, _load_words(ref, *index, others[r]), words)
        return pltpu.bitcast(words, ref.dtype) if words.dtype != ref.dtype else words

    return load


def _attention_masks(n_mem, seg):
    size = n_mem + seg
    shape = (2 * size, _LANES)

    def position(axis):
        r = jax.lax.broadcasted_iota(jnp.int32, shape, axis)
        return r < size, jnp.where(r < seg, r + n_mem, jnp.where(r < size, r - seg, r - size))

    (first_i, i), (first_j, j) = position(0), position(1)
    same = (first_i == first_j) & (j < size)
    fill = jnp.where(same, _MASKED * _LOG2E, -jnp.inf).astype(jnp.float32)
    return same & ((i < n_mem) | (i >= j)), fill


def _start(copies):
    for copy in copies:
        copy.start()


def _wait(copies):
    for copy in copies:
        copy.wait()


def _kernel(xt_hbm, mem0_hbm, wq_hbm, wk_hbm, wv_hbm, wot_hbm, w1_hbm, w2t_hbm, w3_hbm,
            outt_hbm, mem0_ref, tile_ref, x_ref, early_ref, wqkv_ref, wo_ref, w1_ref, w2_ref,
            wplain_ref, stage_ref, stage_sem, mem_sem, tile_sem, *wide_refs, seg):
    d_model, n_tok = xt_hbm.shape
    n_mem = mem0_ref.shape[0]
    d_head = wq_hbm.shape[2]
    n_seg = n_tok // seg
    n_io = n_tok // _LANES
    size = n_mem + seg
    ahead = seg // 2
    width = _TILES * _LANES
    score_scale = d_head ** -0.5 * _LOG2E
    scales = {_W1: -_LOG2E, _W3: -1 / _LOG2E}
    f32, bf16, words = jnp.float32, jnp.bfloat16, jnp.uint32
    shared_slot = 6
    last_slots = {_W1: 2, _W2: shared_slot + 4, _W3: 5}
    wide_refs = list(wide_refs)
    side = _SideJobs(jax.lax.fori_loop(0, 3, lambda i, total: total - i, 3))

    def combine_weights(out_ref, source_ref, block, n_rows, n_tiles):
        wide_refs.reverse()
        wide_ref = wide_refs[0]

        def widen(first, tiles):
            rows = range(first, first + n_rows)
            for j, tile in [(j, block(rows, j)) for j in tiles]:
                wide_ref[first // _LANES, j, pl.ds(first % _LANES, n_rows)] = tile

        jobs = [functools.partial(widen, first, range(j, j + n_tiles))
                for j in range(0, _TILES, n_tiles) for first in range(0, width, n_rows)]
        before = []
        while side.jobs and side.jobs[-1][1] is wide_refs[1]:
            before.insert(0, side.jobs.pop())
        for n, job in enumerate(jobs):
            side.add(source_ref, job)
            if n_rows == _LANES:
                side.add()
            side.jobs += before[n * len(before) // len(jobs):(n + 1) * len(before) // len(jobs)]
        n_products = out_ref.shape[0]
        for job in _combination_jobs(out_ref, 2 if n_products == len(_HOPCROFT_KERR) else 4,
                                     _WEIGHT, lambda i, j, rows: wide_ref[i, j, rows],
                                     {r: r for r in range(n_products)}):
            side.add(wide_ref, job)

    def staged_rows(part, rows, packing):
        count = min(len(rows), _CHUNK)
        for first in rows[::count]:
            c, offset = divmod(first, _CHUNK)
            if isinstance(part, int):
                source = _PARTS if c == part else c
            else:
                source = jnp.where(part == c, _PARTS, c)
            yield _aligned(source * (_CHUNK // packing) + offset // packing, count // packing)

    def block_copies(m, part, slot, rows=pl.ds(0, d_model // 2)):
        src = (wot_hbm, w1_hbm, w2t_hbm, w3_hbm)[m].bitcast(words)
        dst, sem = stage_ref.at[slot], stage_sem.at[slot]
        if m == _WO:
            return [pltpu.make_async_copy(src.at[_TILES * part + j, rows],
                                          dst.at[rows, pl.ds(j * _LANES, _LANES)], sem)
                    for j in range(_TILES)]
        return [pltpu.make_async_copy(src.at[rows, _aligned(part * width, width)],
                                      dst.at[rows], sem)]

    def shared_copies(m):
        return [copy for c in range(_PARTS) for copy in block_copies(
            m, c, shared_slot + m, pl.ds(c * _CHUNK // 2, _CHUNK // 2))]

    def last_copies(m):
        return block_copies(m, _PARTS, last_slots[m])

    def staged(slot, part, rows, j):
        tile = pltpu.bitcast(jnp.concatenate(
            [stage_ref[slot, piece, j * _LANES:(j + 1) * _LANES]
             for piece in staged_rows(part, rows, 2)], axis=0), bf16)
        return (tile.T if len(rows) == _LANES else tile).astype(f32)

    def store_block(m, out_ref, block):
        if m in scales:
            combine_weights(out_ref, stage_ref, lambda *at: block(*at) * scales[m], _SLAB, 2)
        else:
            combine_weights(out_ref, stage_ref, block, _LANES, 1)

    def store_part(m, out_ref, part, slot):
        store_block(m, out_ref.at[part], lambda rows, j: (
            staged(slot, part, rows, j) - staged(shared_slot + m, part, rows, j)))

    def store_shared(m, out_ref):
        store_block(m, out_ref.at[out_ref.shape[0] - 1],
                    functools.partial(staged, shared_slot + m, _PARTS))

    def store_last(m, out_ref):
        part = {_W1: 0, _W3: 1, _W2: _PARTS}[m]

        def block(rows, j):
            own = staged(last_slots[m], part, rows, j)
            if m != _W2 and rows[0] // _CHUNK == 1 - part:
                other = _W1 + _W3 - m
                return own - staged(last_slots[other], part, rows, j) * (
                    scales[other] / scales[m])
            return own

        store_block(m, out_ref.at[_PARTS], block)
        for j in range(_TILES):
            rows = range(part * _CHUNK, (part + 1) * _CHUNK)
            wplain_ref[int(m == _W2), j, pl.ds(part % 2 * _CHUNK, _CHUNK)] = (staged(
                last_slots[m], _PARTS, rows, j) * scales.get(m, 1.0)).astype(bf16)

    def first_step_copies(t):
        return [copy for n in range(2) for copy in block_copies(_W3, 2 * t + n, 3 * (t & 1) + n)
                ] + (shared_copies(_W3) + block_copies(_W1, 0, 2) if t == 0
                     else last_copies(_W3) if t == 1 else last_copies(_W1) if t == 2 else [])

    def load_weights(early_in_ref, early_shared_ref, head_ref, head_sem, *rows_refs):
        n_early = n_io - 1
        products = len(_HOPCROFT_KERR)

        def pair_copies(w, part, slot, rows):
            src = (wq_hbm, wk_hbm, wv_hbm)[w].bitcast(words)
            return [pltpu.make_async_copy(src.at[rows, 2 * part + n, :],
                                          head_ref.at[slot, n, rows], head_sem.at[slot])
                    for n in range(2)]

        def head_copies(part, which=range(3)):
            return [copy for w in which
                    for copy in pair_copies(w, part, 3 * w + 2 * (part & 1), pl.ds(0, d_model))]

        def shared_head_copies(w):
            return [copy for c in range(_PARTS)
                    for copy in pair_copies(w, c, 3 * w + 1, pl.ds(c * _CHUNK, _CHUNK))]

        def part_copies(part, which=range(3)):
            return [copy for m in which for copy in block_copies(m, part, 3 * (part & 1) + m)]

        def head(slot, rows, j):
            pair = head_ref[slot, j // 2, rows, :]
            return pltpu.bitcast(pair & words(0xFFFF0000) if j % 2 else pair << 16, f32)

        def store_heads(w, part):
            def block(rows, j):
                rows = next(staged_rows(part, rows, 1))
                tile = head(3 * w + 2 * (part & 1), rows, j) - head(3 * w + 1, rows, j)
                return tile if w else tile * score_scale

            combine_weights(wqkv_ref.at[w, part], head_ref, block, _SLAB, 2)

        def store_shared_heads(w):
            @pl.loop(0, _LANES // _SLAB)
            def _(n):
                operands = _operands(_levels(2), _WEIGHT, lambda i, j: head(
                    3 * w + 1, _aligned(i * _LANES + n * _SLAB, _SLAB), j) * (
                        1.0 if w else score_scale))
                for r, operand in operands.items():
                    wqkv_ref[w, _PARTS, r, _aligned(n * _SLAB, _SLAB)] = operand().astype(bf16)

        def x_copies(first, last, sem):
            tiles = [(c + 1) % n_io for c in range(first, last)]
            return [pltpu.make_async_copy(xt_hbm.at[:, pl.ds(i * _LANES, _LANES)],
                                          tile_ref.at[i, :d_model], tile_sem.at[sem])
                    for i in tiles]

        def transpose_in(c):
            i = (c + 1) % n_io
            x_ref[i, :_LANES] = _load_packed(tile_ref, i, slice(0, d_model // 2)).T

        def normalize(c):
            for s in range(4):
                _store_rows(rows_refs[c % 3], s // 2, s % 2 * ahead,
                            _layernorm(x_ref[c + 1, s * seg:s * seg + ahead].astype(f32)))

        def fetch(c):
            transpose_in(c)
            if c < n_early:
                normalize(c)

        def prepare(c):
            rows_ref = rows_refs[c % 3]
            for n, job in enumerate(_operand_jobs(early_in_ref.at[c], rows_ref, None)):
                place = 2 * n if c + 2 >= n_early else len(side.jobs)
                side.jobs.insert(place, (c, rows_ref, job))

        def prepare_parts(c):
            for tile in range(_TILES):
                for job in _operand_jobs(early_in_ref.at[c], rows_refs[c % 3], tile):
                    side.add(rows_refs[c % 3], job)

        def project(w, part, c, operand):
            shared = isinstance(part, int) and part == _PARTS

            def keep(f, j, tile):
                early_shared_ref[w, c, f, j] = tile

            def store(f, j, tile):
                early_ref[2 * c + f, w, part, j] = tile.astype(bf16)

            _collect(_levels(2), _WIDE,
                     lambda r: side.dot(operand(r, c), _load_packed(wqkv_ref, w, part, r)),
                     lambda f, j: None if shared else early_shared_ref[w, c, f, j],
                     keep if shared else store)

        def project_shared(pending, first, last):
            operand = _operand_loader(early_in_ref, 2, _PARTS)
            ready = pending + [(w, c) for c in range(first, last) for w in range(3)]
            held = [(w, c) for w, c in ready if w and c + 2 >= last and last < n_early]
            fetch(first)
            side.add(tile_ref, functools.partial(fetch, first + 1))
            prepare(first)
            side.spread(len(pending) * products)
            for w, c in ready:
                if w == 0:
                    side.finish(c)
                    if c + 2 < last + (last == n_early):
                        side.add(tile_ref, functools.partial(fetch, c + 2))
                    if c + 1 < last:
                        prepare(c + 1)
                    prepare_parts(c)
                    if c + 3 == n_early:
                        store_heads(0, 0)
                    side.spread((3 * (n_early - c) - .5 if c + 3 >= n_early
                                 else 1 if (1, c) in held else 3) * products)
                if (w, c) not in held:
                    project(w, _PARTS, c, operand)
            side.finish()
            return held

        def project_part(part, which):
            operand = _operand_loader(early_in_ref, 2, part)
            side.count = -1
            side.spread((len(which) * n_early - .7) * products)
            for w in which:
                for c in range(n_early):
                    project(w, part, c, operand)
            side.finish()

        def store_parts(part, other, which=range(3)):
            for m, out_ref in enumerate((wo_ref, w1_ref, w2_ref)):
                if m in which:
                    store_part(m, out_ref, part, 3 * (part & 1) + m)
                other(m)

        middle = n_io // 2
        _start(x_copies(0, 3, 0) + shared_head_copies(0))
        for w in range(3):
            head_ref[3 * w + 1, :, width:d_model] = jnp.zeros((2, _CHUNK, d_head), words)
        for m in range(4):
            stage_ref[shared_slot + m, width // 2:d_model // 2] = jnp.zeros(
                (_CHUNK // 2, width), words)
        side.keep_in_memory(early_in_ref, early_shared_ref)
        _wait(x_copies(0, 3, 0))
        _start(shared_head_copies(1) + shared_head_copies(2))
        for c in range(3):
            transpose_in(c)
        copies = (x_copies(3, middle, 0), x_copies(middle, middle + 1, 1),
                  x_copies(middle + 1, n_io, 1) + head_copies(0, [0]))
        for w in range(2):
            _wait(shared_head_copies(w))
            _start(copies[w])
            store_shared_heads(w)
            for c in range(3):
                if w:
                    prepare_parts(c)
                else:
                    normalize(c)
                    prepare(c)
            side.spread(2.5 * products)
            for c in range(3):
                side.finish(c)
                project(w, _PARTS, c, _operand_loader(early_in_ref, 2, _PARTS))
            side.finish()
        _wait(shared_head_copies(2) + copies[0])
        _start(copies[2])
        store_shared_heads(2)
        held = project_shared([(2, c) for c in range(3)], 3, middle)
        _wait(copies[1] + copies[2])
        copies = part_copies(0, (_WO, _W2)) + shared_copies(_WO) + shared_copies(_W2)
        _start(head_copies(0, [1, 2]) + copies + head_copies(1))
        project_shared(held, middle, n_early)
        _wait(head_copies(0, [1, 2]))
        _start(shared_copies(_W1))
        store_heads(1, 0)
        store_heads(2, 0)
        project_part(0, [0])
        _wait(copies + head_copies(1))
        _start(part_copies(1) + head_copies(2))
        store_parts(0, lambda w: store_heads(w, 1), (_WO, _W2))
        project_part(0, [1, 2])
        _wait(shared_copies(_W1))

        @pl.loop(1, _PARTS - 1, unroll=True)
        def _(part):
            _wait(part_copies(part) + head_copies(part + 1))
            _start(part_copies(part + 1))
            pl.when(part + 2 < _PARTS)(
                lambda: _start(head_copies(jnp.minimum(part + 2, _PARTS - 1))))
            pl.when(part + 2 == _PARTS)(lambda: _start(last_copies(_W2)))
            store_parts(part, lambda w: store_heads(w, part + 1))
            project_part(part, range(3))

        _wait(part_copies(_PARTS - 1) + last_copies(_W2))
        _start(first_step_copies(0))
        store_parts(_PARTS - 1, lambda m: store_last(_W2, w2_ref) if m == _W1
                    else store_shared(m, w2_ref if m == _W2 else wo_ref))
        project_part(_PARTS - 1, range(3))

    def run_layers(w3_ref, pair_rows_ref, pair_in_ref, solo_rows_ref, solo_in_ref, ffn_rows_ref,
                   ffn_in_ref, attn_shared_ref, ffn_shared_ref, partial_ref, qkv_ref, heads_ref,
                   hidden_ref, attn_sum_ref, ffn_sum_ref, mem_ref, block_ref, second_ref):
        def segment(s):
            return s >> 2, _aligned((s & 3) * seg, seg)

        def transpose_out(i):
            tile_ref.bitcast(words)[i, :d_model // 2] = pltpu.bitcast(x_ref[i, :_LANES].T, words)

        def contract(groups, part, rows_ref, weight_ref, sum_ref, begun):
            operands = _operands(_levels(groups), _WIDE, lambda f, j: rows_ref[part, f, j])

            def targets(i):
                return [_TILES if 2 * i + half == part else i for half in range(2)]

            def start(f, i):
                low, high = (
                    sum_ref[f, n] if (n, half) in begun else None if groups < 4
                    else block_ref[f, :, n * _LANES:(n + 1) * _LANES]
                    for half, n in enumerate(targets(i)))
                if targets(i) == [i, i] and ((i, 0) in begun) == ((i, 1) in begun):
                    return low
                if low is None and high is None:
                    return None
                lanes = jax.lax.broadcasted_iota(jnp.int32, sum_ref.shape[-2:], 1)
                return jnp.where(lanes < _CHUNK, 0.0 if low is None else low,
                                 0.0 if high is None else high)

            def finish(f, i, tile):
                if targets(i) == [i, i]:
                    sum_ref[f, i] = tile
                else:
                    for half, n in enumerate(targets(i)):
                        lanes = slice(half * _CHUNK, (half + 1) * _CHUNK)
                        sum_ref[f, n, :, lanes] = tile[:, lanes]

            _collect(_levels(groups), _MODEL,
                     lambda r: side.dot(operands[r](), _load_packed(weight_ref, part, r)),
                     start, finish, partial_ref.at[part % 2])
            begun.update((n, half) for i in range(_TILES) for half, n in enumerate(targets(i)))

        def keep_and_add(ref, part, f, j, tile):
            total = ref.shape[0] - 1
            ref[part, f, j] = tile
            if 0 < part < _PARTS:
                ref[total, f, j] = ref[total if part > 1 else 0, f, j] + tile

        def project(groups, w, part):
            in_ref = pair_in_ref if groups == 2 else solo_in_ref
            rows = slice(0, in_ref.shape[1])
            side.finish(("P", None), ("P", part // 2))
            operand = _operand_loader(in_ref, groups, part)
            out_ref = qkv_ref.at[w, part % qkv_ref.shape[1]]
            done = {}

            def finish(f, j, tile):
                done[f, j] = tile
                if part == _PARTS:
                    attn_shared_ref[w, f, j, rows] = tile
                elif groups == 2 and (1 - f, j) in done:
                    upper, lower = done[0, j], done[1, j]
                    out_ref[j, :2 * size - ahead] = jnp.concatenate(
                        [upper[n_mem:n_mem + ahead], upper[:n_mem], lower[:n_mem],
                         upper[n_mem + ahead:], lower[n_mem:]], axis=0).astype(bf16)
                elif groups == 1 and (0, j ^ 1) in done:
                    a, b = done[0, j & ~1], done[0, j | 1]
                    out_ref[j | 1] = jnp.concatenate(
                        [a[n_mem:], a[:n_mem], b], axis=0).astype(bf16)

            _collect(_levels(groups), _WIDE,
                     lambda r: side.dot(operand(r), _load_packed(wqkv_ref, w, part, r)),
                     lambda f, j: attn_shared_ref[w, f, j, rows] if part < _PARTS else None,
                     finish)

        def projected(groups, t, place, w, head):
            part, j = divmod(head, _TILES)
            index = w, part % qkv_ref.shape[1], j
            if groups == 1:
                rows = [_load_words(qkv_ref, *index)]
            else:
                rows = [_load_words(early_ref, (t - _LAG) >> 1, w, part, j,
                                    _aligned(place * (ahead // 2), ahead // 2)),
                        _load_words(qkv_ref, *index, slice(0, size - ahead // 2))]
            if w == 1:
                rows.append(jnp.zeros((_CHUNK - size, d_head), words))
            return pltpu.bitcast(jnp.concatenate(rows, axis=0), bf16)

        def by_group(tile):
            return enumerate(tile[f * seg:(f + 1) * seg] for f in range(4))

        def expand(g):
            plain = 2 * _PARTS + 2
            if g == plain:
                x = jnp.concatenate([ffn_rows_ref[f, 0, :seg] for f in range(4)], axis=0)
                for j in range(_TILES):
                    for f, tile in by_group(_dot(x.astype(bf16), _load_packed(wplain_ref, 0, j))):
                        ffn_shared_ref[2, f, j] = tile
                return
            part, up = divmod(g if g < plain else g - 1, 2)
            chunk = up if part == _PARTS else min(part, _PARTS)
            side.finish(("G", None), ("G", chunk // 2))
            operand = _operand_loader(ffn_in_ref, 4, chunk)
            weight_ref = w3_ref if up else w1_ref

            def finish(f, j, tile):
                if part > _PARTS:
                    ffn_shared_ref[up, f, j] = tile
                elif up:
                    keep_and_add(hidden_ref, part, f, j, hidden_ref[part, f, j] * tile)
                else:
                    hidden_ref[part, f, j] = _scaled_silu(tile)

            _collect(_levels(4), _WIDE,
                     lambda r: side.dot(operand(r), _load_packed(weight_ref, part, r)),
                     lambda f, j: None if part > _PARTS else ffn_shared_ref[
                         2 if part == _PARTS else up, f, j],
                     finish, partial_ref.at[g % 2])

        def reduce(g, begun):
            if not begun:
                for f in range(4):
                    rest = block_ref[f, :, width:]
                    ffn_sum_ref[f, _TILES] = jnp.concatenate([rest, jnp.zeros_like(rest)], axis=1)
                begun.update([(_TILES, 0), (_TILES, 1)])
            if g < w2_ref.shape[0]:
                contract(4, g, hidden_ref, w2_ref, ffn_sum_ref, begun)
                return
            total = None
            for j in range(_TILES):
                rows = jnp.concatenate([hidden_ref[_PARTS, f, j] for f in range(4)], axis=0)
                total = _accumulate(total, 1, _dot(
                    _load_packed(wplain_ref, 1, j, slice(0, _CHUNK // 2)), rows.astype(bf16), 1))
            for f, tile in by_group(_value(total).T):
                ffn_sum_ref[f, _TILES, :, :_CHUNK] += tile

        def layer_input(t, place, layer):
            return x_ref[segment(t)].astype(f32) if layer == 0 else second_ref[place]

        def begin_step(t, place, layers):
            h = _layernorm(layer_input(t, place, layers[-1]))
            if len(layers) == 1:
                rows_ref, in_ref = solo_rows_ref, solo_in_ref
                _store_rows(rows_ref, 0, n_mem, h)
            else:
                rows_ref, in_ref, cut = pair_rows_ref, pair_in_ref, ahead // 2
                _store_rows(rows_ref, 0, n_mem, _layernorm(layer_input(t, place, 0)[ahead:]))
                _store_rows(rows_ref, 0, seg - cut, h[:cut])
                _store_rows(rows_ref, 1, n_mem, h[cut:])
            for f, layer in enumerate(layers):
                _store_rows(rows_ref, f, 0, mem_ref[layer])
            for tile in [None, *range(_TILES)]:
                for job in _operand_jobs(in_ref, rows_ref, tile):
                    side.add(rows_ref, job, ("P", tile))

        def close_step(t, place, layers):
            for f, layer in enumerate(layers):
                out = _load_rows(attn_sum_ref, f)
                mem_ref[layer] = out[:n_mem]
                index = 2 * layer + place if len(layers) == 2 else place
                block_ref[index] = layer_input(t, place, layer) + out[n_mem:]

        def run(order, layers=(), t=0, place=0):
            groups, first = len(layers), t
            attn_begun, ffn_begun, probs = set(), set(), {}
            for name in order.split():
                stage, g = name[0], int(name[1:] or 0)
                if stage == "N":
                    begin_step(t, place, layers)
                elif stage == "P":
                    project(groups, g % 3, g // 3)
                elif stage == "S" and (groups == 2 or g % 2):
                    q, k = (projected(groups, first, place, w, g) for w in range(2))
                    s = jnp.where(visible, _dot(q, k, 1), fill)
                    p = jnp.exp2(s - jnp.max(s, axis=-1, keepdims=True))
                    inv = pltpu.reciprocal(jnp.sum(p, axis=-1, keepdims=True), approx=True)
                    probs[g] = p[:, :2 * size].astype(bf16), inv
                elif stage == "V" and (groups == 2 or g % 2):
                    o = _dot(probs[g][0], projected(groups, first, place, 2, g)) * probs[g][1]
                    halves = jnp.concatenate([o[seg:size], o[:seg]], axis=0), o[size:]
                    for f, half in enumerate(halves):
                        index = (f, g % _TILES) if groups == 2 else (0, g % _TILES - 1 + f)
                        keep_and_add(heads_ref, g // _TILES, *index, half)
                elif stage == "O":
                    contract(groups, g, heads_ref, wo_ref, attn_sum_ref, attn_begun)
                elif stage == "A":
                    close_step(t, place, layers)
                    t, place, attn_begun = t + 1, place + 1, set()
                elif stage == "M":
                    _store_rows(ffn_rows_ref, g, 0, _layernorm(block_ref[g]))
                elif stage == "F":
                    tile = g if g < _TILES else None
                    for job in _operand_jobs(ffn_in_ref, ffn_rows_ref, tile):
                        side.add(ffn_rows_ref, job, ("G", tile))
                elif stage == "G":
                    expand(g)
                elif stage == "D":
                    reduce(g, ffn_begun)
                elif stage == "E":
                    for s in range(2):
                        second_ref[g + s] = _load_rows(ffn_sum_ref, s)
                        x_ref[segment(jnp.maximum(first + g - 2 * _LAG, 0) + s)] = _load_rows(
                            ffn_sum_ref, 2 + s).astype(bf16)
                elif stage == "T":
                    side.add(x_ref, functools.partial(transpose_out, g))
                elif stage == "C":
                    _start(out_copies[:n_io - 1])
                elif stage == "Z":
                    for _ in range(g):
                        side.add()
                elif stage == "W":
                    side.spread(g)
                elif stage == "X":
                    side.finish()

        visible, fill = _attention_masks(n_mem, seg)
        side.keep_in_memory(pair_in_ref, solo_rows_ref, solo_in_ref, ffn_in_ref, attn_shared_ref,
                            ffn_shared_ref, partial_ref, qkv_ref, heads_ref, hidden_ref,
                            attn_sum_ref, ffn_sum_ref)
        attn_sum_ref[...] = jnp.zeros_like(attn_sum_ref)
        mem_copy.wait()
        mem_ref[0] = mem0_ref[...].astype(f32)
        for t in range(_LAG):
            run("N", (0,), t, t)
            _wait(first_step_copies(t))
            _start(first_step_copies(t + 1) if t + 1 < _LAG else [mem_copy])
            (store_shared, store_last)[t // 2](*((_W1, w1_ref), (_W3, w3_ref))[t % 2])
            for n in range(2):
                store_part(_W3, w3_ref, 2 * t + n, 3 * (t & 1) + n)
            if t == 0:
                store_part(_W1, w1_ref, 0, 2)
            side.count = -1
            run("W565 " + _ATTENTION + " X", (0,), t, t)
        mem_copy.wait()
        mem_ref[1] = mem0_ref[...].astype(f32)
        run(_SWIGLU)
        for s in range(2):
            second_ref[s] = _load_rows(ffn_sum_ref, s)
            ffn_sum_ref[s] = ffn_sum_ref[2 + s]
        pl.loop(0, 2, unroll=True)(lambda n: run(_STEP, (0, 1), _LAG + n, n))
        run("M0 M2 M1 M3 G18")

        @pl.loop(_LAG // 2 + 1, n_seg // 2)
        def _(b):
            side.count = 0
            run(_TWO_STEPS + " X", (0, 1), 2 * b)

        out_copies = [
            pltpu.make_async_copy(tile_ref.at[i, :d_model],
                                  outt_hbm.at[:, pl.ds(i * _LANES, _LANES)], tile_sem.at[0])
            for i in range(n_io)]
        run(_LAST_STEPS, (1,), n_seg)
        pl.loop(2, _LAG, unroll=True)(lambda n: run(_STEP, (1,), n_seg + n, n))
        run(_SWIGLU.replace("W500", " ".join(f"T{i} Z3" for i in range(n_io - 1)) + " W900")
            .replace("D5", "X C D5"))
        for s in range(_LAG):
            x_ref[segment(n_seg - _LAG + s)] = _load_rows(ffn_sum_ref, s).astype(bf16)
        transpose_out(n_io - 1)
        _start(out_copies[n_io - 1:])
        _wait(out_copies)

    spare = 8
    mem_copy = pltpu.make_async_copy(mem0_hbm, mem0_ref, mem_sem)
    mem_copy.start()
    pl.run_scoped(
        load_weights,
        pltpu.VMEM((n_io - 1, len(_operand_slots(2)), seg, _LANES), bf16),
        pltpu.VMEM((3, n_io - 1, 2, _TILES, seg, _LANES), f32),
        pltpu.VMEM((9, 2, d_model + spare, d_head), words),
        pltpu.SemaphoreType.DMA((9,)),
        *[pltpu.VMEM((2, _TILES + 1, seg + spare, _LANES), f32)] * 3)
    pl.run_scoped(
        run_layers,
        pltpu.VMEM(w1_ref.shape, bf16),
        pltpu.VMEM((2, _TILES + 1, seg + spare, _LANES), f32),
        pltpu.VMEM((len(_operand_slots(2)), seg, _LANES), bf16),
        pltpu.VMEM((1, _TILES + 1, size + spare, _LANES), f32),
        pltpu.VMEM((len(_operand_slots(1)), size, _LANES), f32),
        pltpu.VMEM((4, _TILES + 1, seg + spare, _LANES), f32),
        pltpu.VMEM((len(_operand_slots(4)), seg, _LANES), bf16),
        pltpu.VMEM((3, 2, _TILES, size, _LANES), f32),
        pltpu.VMEM((3, 4, _TILES, seg, _LANES), f32),
        pltpu.VMEM((2, 4, _TILES, seg, _LANES), f32),
        pltpu.VMEM((3, 3, _TILES, 2 * size, _LANES), bf16),
        pltpu.VMEM((_PARTS + 1, 2, _TILES, size, _LANES), f32),
        pltpu.VMEM((_PARTS + 2, 4, _TILES, seg, _LANES), f32),
        pltpu.VMEM((2, _TILES + 1, size, _LANES), f32),
        pltpu.VMEM((4, _TILES + 1, seg, _LANES), f32),
        pltpu.VMEM((2, n_mem, d_model), f32),
        pltpu.VMEM((4, seg, d_model), f32),
        pltpu.VMEM((4, seg, d_model), f32))


@functools.partial(jax.jit, static_argnames=("A_seg_len",))
def pallas_interleave_layers__memory_aug_recurrent_mem_tr__glu_gated_swiglu__prompt_kernel(
    A_x: jax.Array,
    A_mem0: jax.Array,
    A_Wq: jax.Array,
    A_Wk: jax.Array,
    A_Wv: jax.Array,
    A_Wo: jax.Array,
    A_seg_len: int,
    B_x: jax.Array,
    B_w1: jax.Array,
    B_w3: jax.Array,
    B_w2: jax.Array,
):
    del B_x
    _, n_tok, d_model = A_x.shape
    n_mem = A_mem0.shape[1]
    _, n_heads, d_head = A_Wq.shape
    seg = A_seg_len
    assert A_x.shape[0] == 1 and _LAG * seg == d_head == _LANES and 4 * n_mem == seg
    assert n_heads == _PARTS * _TILES and d_model == (_PARTS + 1) * _CHUNK
    assert B_w1.shape[1] == (_PARTS + 1) * _TILES * _LANES and n_tok == 16 * _LANES
    bf16 = jnp.bfloat16
    attn_blocks = (_PARTS + 1, len(_HOPCROFT_KERR), _LANES, _LANES)
    ffn_blocks = (_PARTS + 2, len(_STRASSEN) ** 2, _LANES, _LANES)
    hbm = pl.BlockSpec(memory_space=pltpu.HBM)
    out_t = pl.pallas_call(
        functools.partial(_kernel, seg=seg),
        out_shape=jax.ShapeDtypeStruct((d_model, n_tok), A_x.dtype),
        in_specs=[hbm] * 9,
        out_specs=hbm,
        scratch_shapes=[
            pltpu.VMEM((n_mem, d_model), bf16),
            pltpu.VMEM((n_tok // _LANES, d_model + _SLAB, _LANES), bf16),
            pltpu.VMEM((n_tok // _LANES, _LANES + _SLAB, d_model), bf16),
            pltpu.VMEM(((n_tok // seg - _LAG) // 2, 3, _PARTS, _TILES, seg, _LANES), bf16),
            pltpu.VMEM((3, *attn_blocks), bf16),
            pltpu.VMEM(attn_blocks, bf16),
            pltpu.VMEM(ffn_blocks, bf16),
            pltpu.VMEM(ffn_blocks, bf16),
            pltpu.VMEM((2, _TILES, _LANES, _LANES), bf16),
            pltpu.VMEM((11, (d_model + _SLAB) // 2, _TILES * _LANES), jnp.uint32),
            pltpu.SemaphoreType.DMA((11,)),
            pltpu.SemaphoreType.DMA(()),
            pltpu.SemaphoreType.DMA((2,)),
            *[pltpu.VMEM((_TILES, _TILES, _LANES + _SLAB // 2, _LANES), jnp.float32)] * 2,
        ],
        compiler_params=pltpu.CompilerParams(
            vmem_limit_bytes=127 * 1024 * 1024,
            flags={"XLA_TPU_FORCE_LP_LLO_SCHEDULER": True,
                   "XLA_TPU_EVENLY_DISTRIBUTE_CRITICAL_NODES": True}),
    )(A_x.reshape(n_tok, d_model).T, A_mem0.reshape(n_mem, d_model), A_Wq, A_Wk, A_Wv,
      A_Wo.transpose(0, 2, 1), B_w1, B_w2.T, B_w3)
    return out_t.T.reshape(A_x.shape)
```
